```python
import os as _os
_os.environ.setdefault('JAX_PLATFORMS', 'cpu')
import jax
import jax.numpy as jnp

def _softmax(x, axis=-1):
    return jax.nn.softmax(x, axis=axis)

def _gelu(x):
    return jax.nn.gelu(x, approximate=True)

def _silu(x):
    return jax.nn.silu(x)

def _sigmoid(x):
    return jax.nn.sigmoid(x)

def _layernorm(x, axis=-1, eps=1e-05):
    m = jnp.mean(x, axis=axis, keepdims=True)
    v = jnp.var(x, axis=axis, keepdims=True)
    return (x - m) / jnp.sqrt(v + eps)

def _scatter_add(tgt, idx, src, axis=0):
    return tgt.at[idx].add(src)

def _segment_sum(src, seg, n):
    return jax.ops.segment_sum(src, seg, n)

class _Rng:

    def __init__(self, key):
        self._k = key

    def _next(self):
        self._k, sub = jax.random.split(self._k)
        return sub

    def normal(self, shape):
        return jax.random.normal(self._next(), shape, dtype=jnp.bfloat16)

    def randint(self, lo, hi, shape):
        return jax.random.randint(self._next(), shape, lo, hi, dtype=jnp.int32)

    def uniform(self, shape, lo=0.0, hi=1.0):
        return jax.random.uniform(self._next(), shape, jnp.bfloat16, lo, hi)

    def permutation(self, n):
        return jax.random.permutation(self._next(), n)
kernel_name = 'standalone__conformer_family_e_branchformer__speech'

def setup_inputs():
    _rng = _Rng(jax.random.key(int.from_bytes(__import__("os").urandom(4), "little")))
    _w = lambda a: (lambda t: t.astype(jnp.bfloat16) if jnp.issubdtype(t.dtype, jnp.floating) else t)(jnp.asarray(a))
    B, T, D, K = (2, 4000, 256, 31)
    return {'x': _w((lambda *s: _rng.normal(s) * 0.05)(B, T, D)), 'w_qkv': _w((lambda *s: _rng.normal(s) * 0.05)(D, 3 * D)), 'w_att_out': _w((lambda *s: _rng.normal(s) * 0.05)(D, D)), 'w_mlp_in': _w((lambda *s: _rng.normal(s) * 0.05)(D, 2 * D)), 'dw_csgu': _w((lambda *s: _rng.normal(s) * 0.05)(K, D)), 'w_mlp_out': _w((lambda *s: _rng.normal(s) * 0.05)(D, D)), 'dw_merge': _w((lambda *s: _rng.normal(s) * 0.05)(K, 2 * D)), 'w_merge': _w((lambda *s: _rng.normal(s) * 0.05)(2 * D, D))}

def reference(x, w_qkv, w_att_out, w_mlp_in, dw_csgu, w_mlp_out, dw_merge, w_merge):
    B, T, D = x.shape
    K = dw_csgu.shape[0]
    pad = K // 2
    xa = _layernorm(x, axis=-1)
    qkv = jnp.einsum('btd,de->bte', xa, w_qkv)
    q, k, v = (qkv[..., :D].copy(), qkv[..., D:2 * D].copy(), qkv[..., 2 * D:].copy())
    scores = jnp.einsum('btd,bsd->bts', q, k) * D ** (-0.5)
    p = _softmax(scores, axis=-1)
    attn = jnp.einsum('bts,bsd->btd', p, v)
    glob = jnp.einsum('btd,de->bte', attn, w_att_out)
    xc = _layernorm(x, axis=-1)
    h = _gelu(jnp.einsum('btd,de->bte', xc, w_mlp_in))
    u, g = (h[..., :D].copy(), h[..., D:].copy())
    g = _layernorm(g, axis=-1)
    gp = jnp.pad(g, ((0, 0), (pad, pad), (0, 0)))
    gc = jnp.zeros_like(g)
    for i in range(K):
        gc = gc + gp[:, i:i + T, :] * dw_csgu[i][None, None, :]
    loc = jnp.einsum('btd,de->bte', u * gc, w_mlp_out)
    m = jnp.concatenate([glob, loc], axis=-1)
    mp = jnp.pad(m, ((0, 0), (pad, pad), (0, 0)))
    mc = jnp.zeros_like(m)
    for i in range(K):
        mc = mc + mp[:, i:i + T, :] * dw_merge[i][None, None, :]
    m = m + mc
    return x + jnp.einsum('btc,cd->btd', m, w_merge)
```

```python
import functools
import math

import jax
import jax.numpy as jnp
from jax import lax
import jax.experimental.pallas as pl
import jax.experimental.pallas.tpu as pltpu

F32 = jnp.float32
BF16 = jnp.bfloat16
EPS = 1e-5
LOG2E = 1.4426950408889634
PADR = 16


def _ln(x):
    m = jnp.mean(x, axis=-1, keepdims=True)
    xc = x - m
    v = jnp.mean(xc * xc, axis=-1, keepdims=True)
    return xc * lax.rsqrt(v + EPS)


def _gelu(x):
    c = math.sqrt(2.0 / math.pi)
    return 0.5 * x * (1.0 + jnp.tanh(c * (x + 0.044715 * (x * x * x))))


def _dot(a, b):
    return jnp.dot(a, b, preferred_element_type=F32)


def _dot_nt(a, b):
    return lax.dot_general(a, b, (((1,), (1,)), ((), ())), preferred_element_type=F32)


def _bf_parts(x):
    return [x[:, l * 128:(l + 1) * 128].astype(BF16) for l in range(x.shape[1] // 128)]


def _cat(parts):
    return jnp.concatenate(parts, axis=-1)


def _conv_block(src_ref, lg, t0, R, w_ref, K):
    acc = None
    for b in range(8):
        win = src_ref[lg, pl.ds(t0 + b, R + 24), :]
        for a in range(4):
            s = 8 * a + b
            if s < 1 or s > K:
                continue
            i = s - 1
            w = w_ref[pl.ds(i, 1), pl.ds(lg * 128, 128)]
            term = win[8 * a:8 * a + R, :] * w
            acc = term if acc is None else acc + term
    return acc


def _kernel(x_ref, wqkv_ref, wao_ref, wmi_ref, dwc_ref, wmo_ref, dwm_ref, wm_ref, o_ref,
            wqk_s, wvo_s, dwc_s, dwm_s, xa_s, v_s, u_s, g_s, m_s, s_s, mx_s,
            *, B, T, D, K, TQ, TP, CK, R):
    step = pl.program_id(0)
    NT = T // TQ
    NTT = B * NT
    TS = T + 2 * PADR
    NLG = D // 128
    nc = TP // CK
    NR = TQ // R

    def split(t):
        if isinstance(t, int):
            return t // NT, (t % NT) * TQ
        b = t // NT
        return b, pl.multiple_of((t - b * NT) * TQ, 16)

    def load_bf(ref, b, r0, n):
        return _cat([ref[b, lg, pl.ds(r0, n), :] for lg in range(NLG)])

    def stage_a1(t):
        b, r0 = split(t)
        xa = _bf_parts(_ln(x_ref[b, pl.ds(r0, TQ), :].astype(F32)))
        v = _bf_parts(_dot(_cat(xa), wvo_s[...]))
        for lg in range(NLG):
            xa_s[b, lg, pl.ds(r0, TQ), :] = xa[lg]
            v_s[b, lg, pl.ds(r0, TQ), :] = v[lg]

    vals = {}

    def a2_mm(t, j):
        b, r0 = split(t)
        vals['a2', j] = _dot(load_bf(xa_s, b, r0 + j * R, R), wmi_ref[...])

    def a2_post(t, j):
        b, r0 = split(t)
        r0 = r0 + j * R
        h = _gelu(vals.pop(('a2', j)))
        u_s[pl.ds(b * T + r0, R), :] = h[:, :D]
        g = _ln(h[:, D:])
        for lg in range(NLG):
            g_s[lg, pl.ds(b * TS + r0 + PADR, R), :] = g[:, lg * 128:(lg + 1) * 128]

    def c1_conv(t, j, lg):
        b, r0 = split(t)
        r0 = r0 + j * R
        gc = _conv_block(g_s, lg, b * TS + r0, R, dwc_s, K)
        vals['c1', j, lg] = (u_s[pl.ds(b * T + r0, R), pl.ds(lg * 128, 128)] * gc).astype(BF16)

    def c1_mm(t, j):
        b, r0 = split(t)
        r0 = r0 + j * R
        loc = _dot(_cat([vals.pop(('c1', j, lg)) for lg in range(NLG)]), wmo_ref[...])
        for lg in range(NLG):
            m_s[NLG + lg, pl.ds(b * TS + r0 + PADR, R), :] = loc[:, lg * 128:(lg + 1) * 128]

    def c2_conv(t, j, lg):
        b, r0 = split(t)
        r0 = r0 + j * R
        mc = _conv_block(m_s, lg, b * TS + r0, R, dwm_s, K)
        vals['c2', j, lg] = (m_s[lg, pl.ds(b * TS + r0 + PADR, R), :] + mc).astype(BF16)

    def c2_mm(t, j):
        b, r0 = split(t)
        r0 = r0 + j * R
        mm = _cat([vals.pop(('c2', j, lg)) for lg in range(2 * NLG)])
        y = _dot(mm, wm_ref[...]) + x_ref[b, pl.ds(r0, R), :].astype(F32)
        o_ref[0, pl.ds(j * R, R), :] = y.astype(o_ref.dtype)

    def q_init(t):
        b, r0 = split(t)
        return b, _cat(_bf_parts(_dot(load_bf(xa_s, b, r0, TQ), wqk_s[...])))

    def q_chunk(b, q, c, mx):
        s = _dot_nt(q, load_bf(xa_s, b, c * CK, CK))
        for l in range(CK // 128):
            sl = s[:, l * 128:(l + 1) * 128]
            c0 = c * CK + l * 128
            if c0 + 128 > T:
                col = lax.broadcasted_iota(jnp.int32, (TQ, 128), 1) + c0
                sl = jnp.where(col < T, sl, -jnp.inf)
            s_s[:, pl.ds(c0, 128)] = sl
            mx = sl if mx is None else jnp.maximum(mx, sl)
        return mx

    def q_fin(mx):
        mx_s[...] = jnp.broadcast_to(jnp.max(mx, axis=-1, keepdims=True), (TQ, 128))

    def p_exp(m, c, ls):
        ps = []
        for l in range(CK // 128):
            p = jnp.exp2(s_s[:, pl.ds(c * CK + l * 128, 128)] - m)
            ls = p if ls is None else ls + p
            ps.append(p.astype(BF16))
        return _cat(ps), ls

    def p_mm(b, p, c, acc):
        pv = _dot(p, load_bf(v_s, b, c * CK, CK))
        return pv if acc is None else acc + pv

    def p_fin(t, ls, acc):
        b, r0 = split(t)
        l = jnp.sum(ls, axis=-1, keepdims=True)
        glob = acc * (1.0 / l)
        for lg in range(NLG):
            m_s[lg, pl.ds(b * TS + r0 + PADR, TQ), :] = glob[:, lg * 128:(lg + 1) * 128]

    def run(tq, tp, pre, slots):
        mx = ls = acc = None
        if tp is not None:
            bp, _ = split(tp)
            m = mx_s[...]
            p, ls = p_exp(m, 0, ls)
        if tq is not None:
            bq, q = q_init(tq)
        for f in pre:
            f()
        for c in range(nc):
            if tp is not None:
                acc = p_mm(bp, p, c, acc)
                if c + 1 < nc:
                    p, ls = p_exp(m, c + 1, ls)
            if tq is not None:
                mx = q_chunk(bq, q, c, mx)
            for f in slots[c]:
                f()
        if tp is not None:
            p_fin(tp, ls, acc)
        if tq is not None:
            q_fin(mx)

    P = functools.partial

    def plan(ta2, tc2, tc1, budget):
        pre = []
        jobs = []
        if ta2 is not None:
            pre += [P(a2_mm, ta2, j) for j in range(NR)]
            jobs += [(700, P(a2_post, ta2, j), None) for j in range(NR)]
        if tc2 is not None:
            for j in range(NR):
                for lg in range(2 * NLG):
                    jobs.append((690, P(c2_conv, tc2, j, lg), P(c2_mm, tc2, j) if lg == 2 * NLG - 1 else None))
        if tc1 is not None:
            for j in range(NR):
                for lg in range(NLG):
                    jobs.append((620, P(c1_conv, tc1, j, lg), P(c1_mm, tc1, j) if lg == NLG - 1 else None))
        valu = [[] for _ in range(nc)]
        mxu = [[] for _ in range(nc)]
        c, used = 0, 0
        for cost, f, g in jobs:
            if used + cost > budget and c < nc - 2:
                c, used = c + 1, 0
            used += cost
            valu[c].append(f)
            if g is not None:
                mxu[c + 1].append(g)
        return pre, [mxu[c] + valu[c] for c in range(nc)]

    @pl.when(step == 0)
    def _():
        wq = wqkv_ref[:, 0:D]
        wk = wqkv_ref[:, D:2 * D]
        wv = wqkv_ref[:, 2 * D:3 * D]
        wqk_s[...] = (_dot_nt(wq, wk) * (D ** -0.5 * LOG2E)).astype(BF16)
        wvo_s[...] = _dot(wv, wao_ref[...]).astype(BF16)
        dwc_s[...] = dwc_ref[...].astype(F32)
        dwm_s[...] = dwm_ref[...].astype(F32)
        for b in range(B):
            for lg in range(NLG):
                xa_s[b, lg, pl.ds(T, TP - T), :] = jnp.zeros((TP - T, 128), BF16)
                v_s[b, lg, pl.ds(T, TP - T), :] = jnp.zeros((TP - T, 128), BF16)
                g_s[lg, pl.ds(b * TS, PADR), :] = jnp.zeros((PADR, 128), F32)
                g_s[lg, pl.ds(b * TS + T + PADR, PADR), :] = jnp.zeros((PADR, 128), F32)
            for lg in range(2 * NLG):
                m_s[lg, pl.ds(b * TS, PADR), :] = jnp.zeros((PADR, 128), F32)
                m_s[lg, pl.ds(b * TS + T + PADR, PADR), :] = jnp.zeros((PADR, 128), F32)
        for t in range(NT):
            stage_a1(t)
        sides = [P(stage_a1, t) for t in range(NT, NTT)]
        for t in range(2):
            for j in range(NR):
                sides += [P(a2_mm, t, j), P(a2_post, t, j)]
        per = -(-len(sides) // nc)
        run(0, None, [], [sides[c * per:(c + 1) * per] for c in range(nc)])

    @pl.when(jnp.logical_and(step >= 1, step < NTT))
    def _():
        tc2 = jnp.maximum(step - 3, 0)
        ta2 = jnp.minimum(step + 1, NTT - 1)
        run(step, step - 1, *plan(ta2, tc2, step - 1, 3600))

    @pl.when(step == NTT)
    def _():
        run(None, NTT - 1, *plan(None, NTT - 3, NTT - 1, 3000))

    @pl.when(step > NTT)
    def _():
        for j in range(NR):
            for lg in range(2 * NLG):
                c2_conv(step - 3, j, lg)
            c2_mm(step - 3, j)


@jax.jit
def pallas_standalone__conformer_family_e_branchformer__speech_kernel(
    x, w_qkv, w_att_out, w_mlp_in, dw_csgu, w_mlp_out, dw_merge, w_merge,
):
    B, T, D = x.shape
    K = dw_csgu.shape[0]
    TQ = 400
    TP = 4096
    CK = 512
    R = 80
    NT = T // TQ
    NTT = B * NT
    TS = T + 2 * PADR
    full = lambda a: pl.BlockSpec(a.shape, lambda s: (0,) * a.ndim)

    def out_map(s):
        t = jnp.maximum(s - 3, 0)
        return (t // NT, t % NT, 0)

    kern = functools.partial(_kernel, B=B, T=T, D=D, K=K, TQ=TQ, TP=TP, CK=CK, R=R)
    return pl.pallas_call(
        kern,
        grid=(NTT + 3,),
        in_specs=[full(x), full(w_qkv), full(w_att_out), full(w_mlp_in), full(dw_csgu),
                  full(w_mlp_out), full(dw_merge), full(w_merge)],
        out_specs=pl.BlockSpec((1, TQ, D), out_map),
        out_shape=jax.ShapeDtypeStruct((B, T, D), x.dtype),
        scratch_shapes=[
            pltpu.VMEM((D, D), BF16),
            pltpu.VMEM((D, D), BF16),
            pltpu.VMEM((K, D), F32),
            pltpu.VMEM((K, 2 * D), F32),
            pltpu.VMEM((B, D // 128, TP, 128), BF16),
            pltpu.VMEM((B, D // 128, TP, 128), BF16),
            pltpu.VMEM((B * T, D), F32),
            pltpu.VMEM((D // 128, B * TS, 128), F32),
            pltpu.VMEM((2 * D // 128, B * TS, 128), F32),
            pltpu.VMEM((TQ, TP), F32),
            pltpu.VMEM((TQ, 128), F32),
        ],
        compiler_params=pltpu.CompilerParams(
            dimension_semantics=("arbitrary",),
            vmem_limit_bytes=100 * 1024 * 1024,
        ),
    )(x, w_qkv, w_att_out, w_mlp_in, dw_csgu, w_mlp_out, dw_merge, w_merge)
```

```python
import functools
import math

import jax
import jax.numpy as jnp
from jax import lax
import jax.experimental.pallas as pl
import jax.experimental.pallas.tpu as pltpu

F32 = jnp.float32
BF16 = jnp.bfloat16
U32 = jnp.uint32
EPS = 1e-5
LOG2E = 1.4426950408889634
PADR = 16
CK = 256
NPV = 20
NACC = 2
ACCB = 0
FIRST = 0
E = lambda k, d: int(d)
PV0, A2A, UA0, UA1, GA0, GA1 = E('PV0', 0), E('A2A', 0), E('UA0', 8), E('UA1', 28), E('GA0', 30), E('GA1', 50)
GLA, GL0, GL1 = E('GLA', 0), E('GL0', 16), E('GL1', 36)
ANCH = 1


def _ln(x):
    m = jnp.mean(x, axis=-1, keepdims=True)
    xc = x - m
    v = jnp.mean(xc * xc, axis=-1, keepdims=True)
    return xc * lax.rsqrt(v + EPS)


def _gelu(x):
    c = math.sqrt(2.0 / math.pi)
    return 0.5 * x * (1.0 + jnp.tanh(c * (x + 0.044715 * (x * x * x))))


def _dot(a, b):
    return jnp.dot(a, b, preferred_element_type=F32)


def _dot_nt(a, b):
    return lax.dot_general(a, b, (((1,), (1,)), ((), ())), preferred_element_type=F32)


def _cat(parts, axis=-1):
    return jnp.concatenate(parts, axis=axis)


def _pk(x):
    return pltpu.bitcast(x, U32)


def _upk(x):
    return pltpu.bitcast(x, BF16)


def _conv_block(src_ref, slot, lg, R, w_ref, K):
    accs = [None] * NACC
    for b in range(8):
        win = src_ref[slot, lg, pl.ds(b, R + 24), :]
        for a in range(4):
            s = 8 * a + b
            if s < 1 or s > K:
                continue
            i = s - 1
            w = w_ref[pl.ds(i, 1), pl.ds(lg * 128, 128)]
            term = win[8 * a:8 * a + R, :] * w
            j = (b * NACC) // 8 if ACCB else a % NACC
            accs[j] = term if accs[j] is None else accs[j] + term
    while len(accs) > 1:
        accs = [accs[j] + accs[j + 1] for j in range(0, len(accs), 2)]
    return accs[0]


def _kernel(x_hbm, wqkv_hbm, wao_hbm, wmi_hbm, dwc_ref, wmo_hbm, dwm_ref, wm_hbm, o_ref,
            x_ref, wqkv_ref, wao_ref, wmi_ref, wmo_ref, wm_ref, sems,
            wqk_s, wvo_s, wmi_s, wmo_s, wm_s, dwc_s, dwm_s, xa_s, v_s, u_s, g_s, m_s, s_s, mx_s, z_s,
            *, B, T, D, K, R, U, TP):
    step = pl.program_id(0)
    NK = T // R
    NKT = B * NK
    NS = NKT // U
    NLG = D // 128
    TA = 400
    NC = TP // CK

    def split(k):
        if isinstance(k, int):
            return k // NK, k % NK
        b = k // NK
        return b, k - b * NK

    def rows(i, n):
        r = i * n
        return pl.ds(r if isinstance(r, int) else pl.multiple_of(r, 8), n)

    def halo_store(ref, k, kmod, lg, val):
        ref[kmod, lg, pl.ds(PADR, R), :] = val
        top, bot = val[:PADR], val[R - PADR:]
        if kmod == 0:
            first = (k % NK == 0)
            top = jnp.where(first, 0.0, top) if not isinstance(first, bool) else (jnp.zeros_like(top) if first else top)
        if kmod == U - 1:
            last = (k % NK == NK - 1)
            bot = jnp.where(last, 0.0, bot) if not isinstance(last, bool) else (jnp.zeros_like(bot) if last else bot)
        ref[(kmod - 1) % U, lg, pl.ds(PADR + R, PADR), :] = top
        ref[(kmod + 1) % U, lg, pl.ds(0, PADR), :] = bot

    def vregs(a):
        return [a[8 * r:8 * r + 8, l * 128:(l + 1) * 128] for r in range(a.shape[0] // 8) for l in range(a.shape[1] // 128)]

    def stage_a1(b, t):
        xa = _ln(x_ref[b, pl.ds(t * TA, TA), :].astype(F32))
        v = _dot(xa.astype(BF16), _upk(wvo_s[...]))
        xa_s[b, rows(t, TA // 2), :] = _pk(xa.astype(BF16))
        v_s[b, rows(t, TA // 2), :] = _pk(v.astype(BF16))

    def stage_a2(k, kmod):
        b, i = split(k)
        h = _gelu(_dot(_upk(xa_s[b, rows(i, R // 2), :]), _upk(wmi_s[...])))
        u_s[kmod] = h[:, :D]
        g = _ln(h[:, D:])
        for lg in range(NLG):
            halo_store(g_s, k, kmod, lg, g[:, lg * 128:(lg + 1) * 128])
        return vregs(h[:, :D]), vregs(g)

    def c1_conv(kmod):
        return [u_s[kmod, :, pl.ds(lg * 128, 128)] * _conv_block(g_s, kmod, lg, R, dwc_s, K) for lg in range(NLG)]

    def c1_mm(k, kmod, parts):
        loc = _dot(_cat(parts).astype(BF16), _upk(wmo_s[...]))
        for lg in range(NLG):
            halo_store(m_s, k, kmod, NLG + lg, loc[:, lg * 128:(lg + 1) * 128])

    def c2_conv(kmod):
        return [m_s[kmod, lg, pl.ds(PADR, R), :] + _conv_block(m_s, kmod, lg, R, dwm_s, K) for lg in range(2 * NLG)]

    def c2_mm(k, kmod, parts):
        b, i = split(k)
        r0 = i * R
        r0 = r0 if isinstance(r0, int) else pl.multiple_of(r0, 16)
        y = _dot(_cat(parts).astype(BF16), _upk(wm_s[...])) + x_ref[b, pl.ds(r0, R), :].astype(F32)
        o_ref[0, pl.ds(kmod * R, R), :] = y.astype(o_ref.dtype)

    def q_proj(k):
        b, i = split(k)
        return _dot(_upk(xa_s[b, rows(i, R // 2), :]), _upk(wqk_s[...])).astype(BF16)

    def kv_chunk(ref, b, c, never, deps):
        blks = []
        for kt in range(CK // 128):
            parts = []
            for lg in range(NLG):
                t = ref[b, pl.ds(c * CK // 2 + kt * 64, 64), pl.ds(lg * 128, 128)]
                dd = deps[(c * (CK // 128) + kt) * NLG + lg]
                if dd:
                    pieces = [t[8 * j:8 * j + 8] for j in range(8)]
                    for j, d in enumerate(dd):
                        jj = 7 - j if FIRST else j
                        pieces[jj] = jnp.where(never, pltpu.bitcast(d, U32), pieces[jj])
                    t = _cat(pieces, axis=0)
                parts.append(t)
            blks.append(_cat(parts))
        return _upk(_cat(blks, axis=0))

    def stage_q(k, kmod, q, never, deps):
        b, _ = split(k)
        mx = None
        for c in range(NC):
            s = _dot_nt(q, kv_chunk(xa_s, b, c, never, deps))
            for l in range(CK // 128):
                sl = s[:, l * 128:(l + 1) * 128]
                c0 = c * CK + l * 128
                if c0 + 128 > T:
                    col = lax.broadcasted_iota(jnp.int32, (R, 128), 1) + c0
                    sl = jnp.where(col < T, sl, -jnp.inf)
                s_s[kmod, :, pl.ds(c0, 128)] = sl
                mx = sl if mx is None else jnp.maximum(mx, sl)
        mx_s[kmod] = jnp.broadcast_to(jnp.max(mx, axis=-1, keepdims=True), (R, 128))

    def stage_p(k, kmod, never, deps):
        b, _ = split(k)
        m = mx_s[kmod]
        ls = acc = None
        for c in range(NC):
            ps = []
            for l in range(CK // 128):
                p = jnp.exp2(s_s[kmod, :, pl.ds(c * CK + l * 128, 128)] - m)
                ls = p if ls is None else ls + p
                ps.append(p)
            pv = _dot(_cat(ps).astype(BF16), kv_chunk(v_s, b, c, never, deps))
            acc = pv if acc is None else acc + pv
        l = jnp.sum(ls, axis=-1, keepdims=True)
        glob = acc * (1.0 / l)
        for lg in range(NLG):
            halo_store(m_s, k, kmod, lg, glob[:, lg * 128:(lg + 1) * 128])
        return vregs(glob)

    NTILE = (TP // 128) * NLG

    def place(slots, items, lo, hi):
        for j, it in enumerate(items):
            slots[lo + (j * (hi - lo)) // len(items)].append(it)

    def micro(n, nmod):
        ok = lambda k: (not isinstance(k, int)) or 0 <= k < NKT
        never = z_s[...] != 0
        c1p = c2p = None
        conv = []
        if ok(n):
            if isinstance(n, int) and n == NKT - 1:
                for lg in range(2 * NLG):
                    m_s[nmod, lg, pl.ds(PADR + R, PADR), :] = jnp.zeros((PADR, 128), F32)
            c2p = c2_conv(nmod)
            conv += [p[8 * r:8 * r + 8] for p in c2p for r in range(R // 8)]
        if ok(n + 2):
            if isinstance(n, int) and n + 2 == NKT - 1:
                for lg in range(NLG):
                    g_s[(nmod + 2) % U, lg, pl.ds(PADR + R, PADR), :] = jnp.zeros((PADR, 128), F32)
            c1p = c1_conv((nmod + 2) % U)
            conv += [p[8 * r:8 * r + 8] for p in c1p for r in range(R // 8)]
        hasp, hasq = ok(n + 2), ok(n + 3)
        dp = [[] for _ in range(NTILE)]
        dq = [[] for _ in range(NTILE)]
        if hasp and hasq:
            npv = min(NPV, len(conv))
        elif hasp:
            npv = len(conv)
        else:
            npv = 0
        if npv:
            place(dp, conv[:npv], PV0, NTILE)
        if hasq and conv[npv:]:
            place(dq, conv[npv:], 0, NTILE)
        if hasq:
            q = q_proj(n + 3)
        if ok(n + 4):
            uu, gg = stage_a2(n + 4, (nmod + 4) % U)
            if A2A and (hasp or hasq):
                dd = dp if hasp else dq
                place(dd, uu, UA0, UA1)
                place(dd, gg, GA0, GA1)
        if hasp:
            gl = stage_p(n + 2, (nmod + 2) % U, never, dp)
            if hasq and GLA:
                place(dq, gl, GL0, GL1)
        if hasq:
            stage_q(n + 3, (nmod + 3) % U, q, never, dq)
        if c2p is not None:
            c2_mm(n, nmod, c2p)
        if c1p is not None:
            c1_mm(n + 2, (nmod + 2) % U, c1p)

    @pl.when(step == 0)
    @jax.named_scope("prologue")
    def _():
        nt1 = T // TA
        xgroups = [(0, 0, 2), (0, 2, 6), (0, 6, nt1), (1, 0, nt1)]
        cw = [pltpu.make_async_copy(src, dst, sems.at[j]) for j, (src, dst) in enumerate(
            [(wqkv_hbm, wqkv_ref), (wao_hbm, wao_ref), (wmi_hbm, wmi_ref), (wmo_hbm, wmo_ref), (wm_hbm, wm_ref)])]
        cx = [pltpu.make_async_copy(x_hbm.at[b, pl.ds(t0 * TA, (t1 - t0) * TA), :],
                                    x_ref.at[b, pl.ds(t0 * TA, (t1 - t0) * TA), :], sems.at[5 + j])
              for j, (b, t0, t1) in enumerate(xgroups)]
        for c in [cw[0], cw[1], cx[0], cx[1], cx[2], cw[2], cw[3], cw[4], cx[3]]:
            c.start()
        z_s[...] = jnp.zeros(z_s.shape, z_s.dtype)
        dwc_s[...] = dwc_ref[...].astype(F32)
        dwm_s[...] = dwm_ref[...].astype(F32)
        for b in range(B):
            xa_s[b, pl.ds(T // 2, (TP - T) // 2), :] = jnp.zeros(((TP - T) // 2, D), U32)
            v_s[b, pl.ds(T // 2, (TP - T) // 2), :] = jnp.zeros(((TP - T) // 2, D), U32)
        for lg in range(NLG):
            g_s[0, lg, pl.ds(0, PADR), :] = jnp.zeros((PADR, 128), F32)
        for lg in range(2 * NLG):
            m_s[0, lg, pl.ds(0, PADR), :] = jnp.zeros((PADR, 128), F32)
        cw[0].wait()
        cw[1].wait()
        wq = wqkv_ref[:, 0:D]
        wk = wqkv_ref[:, D:2 * D]
        wv = wqkv_ref[:, 2 * D:3 * D]
        wvo_s[...] = _pk(_dot(wv, wao_ref[...]).astype(BF16))
        wqk_s[...] = _pk((_dot_nt(wq, wk) * (D ** -0.5 * LOG2E)).astype(BF16))
        for j in range(3):
            cx[j].wait()
            for t in range(xgroups[j][1], xgroups[j][2]):
                stage_a1(0, t)
        cw[2].wait()
        cw[3].wait()
        cw[4].wait()
        cx[3].wait()
        wmi_s[...] = _pk(wmi_ref[...])
        wmo_s[...] = _pk(wmo_ref[...])
        wm_s[...] = _pk(wm_ref[...])
        for n in range(-4, 0):
            micro(n, n % U)
            for t in range(nt1):
                if t * 4 // nt1 == n + 4:
                    stage_a1(1, t)

    @pl.when(step < NS - 1)
    @jax.named_scope("steady")
    def _():
        for i in range(U):
            micro(step * U + i, i)

    @pl.when(step == NS - 1)
    @jax.named_scope("last")
    def _():
        for i in range(U):
            micro((NS - 1) * U + i, i)


@jax.jit
def pallas_standalone__conformer_family_e_branchformer__speech_kernel(
    x, w_qkv, w_att_out, w_mlp_in, dw_csgu, w_mlp_out, dw_merge, w_merge,
):
    B, T, D = x.shape
    K = dw_csgu.shape[0]
    R = 80
    U = 5
    TP = 4096
    NSB = T // (R * U)
    TH = -(-(R + 2 * PADR) // 32) * 32
    full = lambda a: pl.BlockSpec(a.shape, lambda s: (0,) * a.ndim)

    hbm = pl.BlockSpec(memory_space=pl.ANY)
    kern = functools.partial(_kernel, B=B, T=T, D=D, K=K, R=R, U=U, TP=TP)
    return pl.pallas_call(
        kern,
        grid=(B * NSB,),
        in_specs=[hbm, hbm, hbm, hbm, full(dw_csgu), hbm, full(dw_merge), hbm],
        out_specs=pl.BlockSpec((1, R * U, D), lambda s: (s // NSB, s % NSB, 0)),
        out_shape=jax.ShapeDtypeStruct((B, T, D), x.dtype),
        scratch_shapes=[
            pltpu.VMEM(x.shape, BF16),
            pltpu.VMEM(w_qkv.shape, BF16),
            pltpu.VMEM(w_att_out.shape, BF16),
            pltpu.VMEM(w_mlp_in.shape, BF16),
            pltpu.VMEM(w_mlp_out.shape, BF16),
            pltpu.VMEM(w_merge.shape, BF16),
            pltpu.SemaphoreType.DMA((9,)),
            pltpu.VMEM((D // 2, D), U32),
            pltpu.VMEM((D // 2, D), U32),
            pltpu.VMEM((D // 2, 2 * D), U32),
            pltpu.VMEM((D // 2, D), U32),
            pltpu.VMEM((D, D), U32),
            pltpu.VMEM((K, D), F32),
            pltpu.VMEM((K, 2 * D), F32),
            pltpu.VMEM((B, TP // 2, D), U32),
            pltpu.VMEM((B, TP // 2, D), U32),
            pltpu.VMEM((U, R, D), F32),
            pltpu.VMEM((U, D // 128, TH, 128), F32),
            pltpu.VMEM((U, 2 * D // 128, TH, 128), F32),
            pltpu.VMEM((U, R, TP), F32),
            pltpu.VMEM((U, R, 128), F32),
            pltpu.VMEM((8, 128), jnp.int32),
        ],
        compiler_params=pltpu.CompilerParams(
            dimension_semantics=("arbitrary",),
            vmem_limit_bytes=100 * 1024 * 1024,
        ),
    )(x, w_qkv, w_att_out, w_mlp_in, dw_csgu, w_mlp_out, dw_merge, w_merge)
```

```python
import functools
import math

import jax
import jax.numpy as jnp
from jax import lax
import jax.experimental.pallas as pl
import jax.experimental.pallas.tpu as pltpu

F32 = jnp.float32
BF16 = jnp.bfloat16
U32 = jnp.uint32
EPS = 1e-5
LOG2E = 1.4426950408889634
PADR = 16
CK = 256
NPV = 20
NACC = 2
ACCB = 0
FIRST = 1
E = lambda k, d: int(d)
PV0, A2A, UA0, UA1, GA0, GA1 = E('PV0', 0), E('A2A', 0), E('UA0', 8), E('UA1', 28), E('GA0', 30), E('GA1', 50)
GLA, GL0, GW = E('GLA', 0), E('GL0', 12), E('GW', 10)
PO = [int(c) for c in '1113130']
ZS = E('ZS', 0)
DS0, DS1 = E('DS0', 9), E('DS1', 9)
UN = E('UN', 5)
THR, THS, GRP = E('THR', 0), E('THS', 1), E('GRP', 1)
HA0, AW, AD, QK0, CORD = E('HA0', 8), E('AW', 20), E('AD', 10), E('QK0', 0), E('CORD', 0)
ANCH = 1


def _ln(x):
    m = jnp.mean(x, axis=-1, keepdims=True)
    xc = x - m
    v = jnp.mean(xc * xc, axis=-1, keepdims=True)
    return xc * lax.rsqrt(v + EPS)


def _gelu(x):
    c = math.sqrt(2.0 / math.pi)
    return 0.5 * x * (1.0 + jnp.tanh(c * (x + 0.044715 * (x * x * x))))


def _dot(a, b):
    return jnp.dot(a, b, preferred_element_type=F32)


def _dot_nt(a, b):
    return lax.dot_general(a, b, (((1,), (1,)), ((), ())), preferred_element_type=F32)


def _cat(parts, axis=-1):
    return jnp.concatenate(parts, axis=axis)


def _pk(x):
    return pltpu.bitcast(x, U32)


def _upk(x):
    return pltpu.bitcast(x, BF16)


def _conv_block(src_ref, lg, R, w_ref, K, zs):
    accs = [None] * NACC
    for b in range(8):
        for a in range(4):
            s = 8 * a + b
            if s < 1 or s > K:
                continue
            i = s - 1
            win = src_ref[lg, pl.ds(zs[a] + s, R), :]
            w = w_ref[pl.ds(i, 1), pl.ds(lg * 128, 128)]
            term = win * w
            j = (b * NACC) // 8 if ACCB else a % NACC
            accs[j] = term if accs[j] is None else accs[j] + term
    while len(accs) > 1:
        accs = [accs[j] + accs[j + 1] for j in range(0, len(accs), 2)]
    return accs[0]


def _kernel(x_hbm, wqkv_hbm, wao_hbm, wmi_hbm, dwc_ref, wmo_hbm, dwm_ref, wm_hbm, o_ref,
            x_ref, wqkv_ref, wao_ref, wmi_ref, wmo_ref, wm_ref, sems,
            wqk_s, wvo_s, wmi_s, wmo_s, wm_s, dwc_s, dwm_s, xa_s, v_s, u_s, s_s, mx_s, z_s, zs_s, *rings,
            B, T, D, K, R, U, TP):
    g_s, m_s = rings[:U], rings[U:]
    step = pl.program_id(0)
    NK = T // R
    NKT = B * NK
    NS = NKT // UN
    NLG = D // 128
    TA = 400
    NC = TP // CK

    def split(k):
        if isinstance(k, int):
            return k // NK, k % NK
        b = k // NK
        return b, k - b * NK

    def rows(i, n):
        r = i * n
        return pl.ds(r if isinstance(r, int) else pl.multiple_of(r, 8), n)

    def halo_store(ref, k, kmod, lg, val):
        ref[kmod][lg, pl.ds(PADR, R), :] = val
        top, bot = val[:PADR], val[R - PADR:]
        if kmod == 0:
            first = (k % NK == 0)
            top = jnp.where(first, 0.0, top) if not isinstance(first, bool) else (jnp.zeros_like(top) if first else top)
        if kmod == U - 1:
            last = (k % NK == NK - 1)
            bot = jnp.where(last, 0.0, bot) if not isinstance(last, bool) else (jnp.zeros_like(bot) if last else bot)
        ref[(kmod - 1) % U][lg, pl.ds(PADR + R, PADR), :] = top
        ref[(kmod + 1) % U][lg, pl.ds(0, PADR), :] = bot

    def vregs(a):
        return [a[8 * r:8 * r + 8, l * 128:(l + 1) * 128] for r in range(a.shape[0] // 8) for l in range(a.shape[1] // 128)]

    def stage_a1(b, t):
        xa = _ln(x_ref[b, pl.ds(t * TA, TA), :].astype(F32))
        v = _dot(xa.astype(BF16), _upk(wvo_s[...]))
        xa_s[b, rows(t, TA // 2), :] = _pk(xa.astype(BF16))
        v_s[b, rows(t, TA // 2), :] = _pk(v.astype(BF16))

    def bc(a):
        return jnp.broadcast_to(a, (a.shape[0], 128))

    def stage_a2(k, kmod):
        b, i = split(k)
        h = _gelu(_dot(_upk(xa_s[b, rows(i, R // 2), :]), _upk(wmi_s[...])))
        u_s[kmod] = h[:, :D]
        hg = h[:, D:]
        mu = jnp.mean(hg, axis=-1, keepdims=True)
        xc = hg - mu
        rs = lax.rsqrt(jnp.mean(xc * xc, axis=-1, keepdims=True) + EPS)
        g = xc * rs
        for lg in range(NLG):
            halo_store(g_s, k, kmod, lg, g[:, lg * 128:(lg + 1) * 128])
        return vregs(h[:, :D]), vregs(hg), vregs(bc(mu)), vregs(bc(rs)), vregs(g)

    def c1_conv(kmod, zs):
        return [u_s[kmod, :, pl.ds(lg * 128, 128)] * _conv_block(g_s[kmod], lg, R, dwc_s, K, zs) for lg in range(NLG)]

    def c1_mm(k, kmod, parts):
        loc = _dot(_cat(parts).astype(BF16), _upk(wmo_s[...]))
        for lg in range(NLG):
            halo_store(m_s, k, kmod, NLG + lg, loc[:, lg * 128:(lg + 1) * 128])

    def c2_conv(kmod, zs):
        return [m_s[kmod][lg, pl.ds(PADR, R), :] + _conv_block(m_s[kmod], lg, R, dwm_s, K, zs) for lg in range(2 * NLG)]

    def c2_mm(k, pos, parts):
        b, i = split(k)
        r0 = i * R
        r0 = r0 if isinstance(r0, int) else pl.multiple_of(r0, 16)
        y = _dot(_cat(parts).astype(BF16), _upk(wm_s[...])) + x_ref[b, pl.ds(r0, R), :].astype(F32)
        o_ref[0, pl.ds(pos * R, R), :] = y.astype(o_ref.dtype)

    def q_proj(k):
        b, i = split(k)
        return _dot(_upk(xa_s[b, rows(i, R // 2), :]), _upk(wqk_s[...])).astype(BF16)

    def kv_chunk(ref, b, c, never, deps):
        blks = []
        for kt in range(CK // 128):
            parts = []
            for lg in range(NLG):
                t = ref[b, pl.ds(c * CK // 2 + kt * 64, 64), pl.ds(lg * 128, 128)]
                dd = deps[(c * (CK // 128) + kt) * NLG + lg]
                if dd:
                    pieces = [t[8 * j:8 * j + 8] for j in range(8)]
                    for j, d in enumerate(dd):
                        jj = 7 - j if FIRST else j
                        pieces[jj] = jnp.where(never, pltpu.bitcast(d, U32), pieces[jj])
                    t = _cat(pieces, axis=0)
                parts.append(t)
            blks.append(_cat(parts))
        return _upk(_cat(blks, axis=0))

    def q_chunks(k, kmod, q, never, deps, mx, ca, cb):
        b, _ = split(k)
        for c in range(ca, cb):
            s = _dot_nt(q, kv_chunk(xa_s, b, c, never, deps))
            for l in range(CK // 128):
                sl = s[:, l * 128:(l + 1) * 128]
                c0 = c * CK + l * 128
                if c0 + 128 > T:
                    col = lax.broadcasted_iota(jnp.int32, (R, 128), 1) + c0
                    sl = jnp.where(col < T, sl, -jnp.inf)
                s_s[kmod, :, pl.ds(c0, 128)] = sl
                mx = sl if mx is None else jnp.maximum(mx, sl)
        if cb == NC:
            mx_s[kmod] = jnp.broadcast_to(jnp.max(mx, axis=-1, keepdims=True), (R, 128))
        return mx

    def stage_q(k, kmod, q, never, deps):
        q_chunks(k, kmod, q, never, deps, None, 0, NC)

    def stage_p(k, kmod, never, deps):
        b, _ = split(k)
        m = mx_s[kmod]
        ls = acc = None
        pvs = []
        neverr = _cat([never] * (R // 8), axis=0)
        for c in range(NC):
            ps = []
            if THR and c >= THR and (c % THS == 0):
                m = jnp.where(neverr, pvs[c - THR][:, :128], m)
            for l in range(CK // 128):
                p = jnp.exp2(s_s[kmod, :, pl.ds(c * CK + l * 128, 128)] - m)
                ls = p if ls is None else ls + p
                ps.append(p)
            pv = _dot(_cat(ps).astype(BF16), kv_chunk(v_s, b, c, never, deps))
            pvs.append(pv)
            acc = pv if acc is None else acc + pv
        l = jnp.sum(ls, axis=-1, keepdims=True)
        rinv = 1.0 / l
        glob = acc * rinv
        for lg in range(NLG):
            halo_store(m_s, k, kmod, lg, glob[:, lg * 128:(lg + 1) * 128])
        return vregs(bc(rinv)), vregs(glob)

    NTILE = (TP // 128) * NLG

    def place(slots, items, lo, hi, grp=1):
        ng = -(-len(items) // grp)
        for j, it in enumerate(items):
            pos = lo + (((j // grp) * 2 + 1) * (hi - lo)) // (2 * ng) if grp > 1 else lo + (j * (hi - lo)) // len(items)
            while len(slots[pos]) >= 8:
                pos += 1
            slots[pos].append(it)

    def micro(n, pos):
        nmod = pos % U
        ok = lambda k: (not isinstance(k, int)) or 0 <= k < NKT
        never = z_s[...] != 0
        zs = [zs_s[a] if ZS else 0 for a in range(4)]
        c1p = c2p = None
        conv = []
        if ok(n):
            if isinstance(n, int) and n == NKT - 1:
                for lg in range(2 * NLG):
                    m_s[nmod][lg, pl.ds(PADR + R, PADR), :] = jnp.zeros((PADR, 128), F32)
            c2p = c2_conv(nmod, zs)
            conv += [p[8 * r:8 * r + 8] for p in c2p for r in range(R // 8)]
        if ok(n + 2):
            if isinstance(n, int) and n + 2 == NKT - 1:
                for lg in range(NLG):
                    g_s[(nmod + 2) % U][lg, pl.ds(PADR + R, PADR), :] = jnp.zeros((PADR, 128), F32)
            c1p = c1_conv((nmod + 2) % U, zs)
            conv += [p[8 * r:8 * r + 8] for p in c1p for r in range(R // 8)]
        hasp, hasq = ok(n + 2), ok(n + 3)
        slots = [[] for _ in range(2 * NTILE)]
        lo = 0 if hasp else NTILE
        hi = 2 * NTILE if hasq else NTILE

        def put(items, a, b, grp=1):
            a, b = max(a, lo), min(b, hi)
            if items and b > a:
                place(slots, items, a, b, grp)

        if CORD == 1 and c1p is not None and c2p is not None:
            conv = conv[4 * (R // 8):] + conv[:4 * (R // 8)]
        if hasp and hasq:
            npv = min(NPV, len(conv))
        elif hasp:
            npv = len(conv)
        else:
            npv = 0
        put(conv[:npv], PV0, NTILE, GRP)
        put(conv[npv:], NTILE + QK0, 2 * NTILE, GRP)
        if hasq:
            q = q_proj(n + 3)
        if ok(n + 4):
            uu, hh, mu, rs, gg = stage_a2(n + 4, (nmod + 4) % U)
            if A2A:
                off = 0 if hasp else NTILE
                if UA1 > UA0:
                    put(uu, off + UA0, off + UA1)
                put(hh, off + HA0, off + HA0 + AW)
                put(mu, off + HA0 + AD, off + HA0 + AD + AW)
                put(rs, off + HA0 + 2 * AD, off + HA0 + 2 * AD + AW)
                put(gg, off + HA0 + 2 * AD + 4, off + HA0 + 2 * AD + 4 + AW)
        if hasp:
            ri, gl = stage_p(n + 2, (nmod + 2) % U, never, slots[:NTILE])
            if hasq and GLA:
                put(ri, NTILE + GL0, NTILE + GL0 + GW)
                put(gl, NTILE + GL0 + 4, NTILE + GL0 + 4 + GW)
        if hasq:
            stage_q(n + 3, (nmod + 3) % U, q, never, slots[NTILE:])
        if c2p is not None:
            c2_mm(n, pos, c2p)
        if c1p is not None:
            c1_mm(n + 2, (nmod + 2) % U, c1p)

    @pl.when(step == 0)
    @jax.named_scope("prologue")
    def _():
        nt1 = T // TA
        xgroups = [(0, 0, 2), (0, 2, 6), (0, 6, nt1), (1, 0, nt1)]
        cw = [pltpu.make_async_copy(src, dst, sems.at[j]) for j, (src, dst) in enumerate(
            [(wqkv_hbm, wqkv_ref), (wao_hbm, wao_ref), (wmi_hbm, wmi_ref), (wmo_hbm, wmo_ref), (wm_hbm, wm_ref)])]
        cx = [pltpu.make_async_copy(x_hbm.at[b, pl.ds(t0 * TA, (t1 - t0) * TA), :],
                                    x_ref.at[b, pl.ds(t0 * TA, (t1 - t0) * TA), :], sems.at[5 + j])
              for j, (b, t0, t1) in enumerate(xgroups)]
        dma_order = [cx[0], cw[0], cw[1], cx[1], cw[2], cx[2], cw[3], cw[4], cx[3]]
        for c in dma_order[:DS0]:
            c.start()
        z_s[...] = jnp.zeros(z_s.shape, z_s.dtype)
        for a in range(4):
            zs_s[a] = 0
        dwc_s[...] = dwc_ref[...].astype(F32)
        dwm_s[...] = dwm_ref[...].astype(F32)
        for b in range(B):
            xa_s[b, pl.ds(T // 2, (TP - T) // 2), :] = jnp.zeros(((TP - T) // 2, D), U32)
            v_s[b, pl.ds(T // 2, (TP - T) // 2), :] = jnp.zeros(((TP - T) // 2, D), U32)
        for lg in range(NLG):
            g_s[0][lg, pl.ds(0, PADR), :] = jnp.zeros((PADR, 128), F32)
        for lg in range(2 * NLG):
            m_s[0][lg, pl.ds(0, PADR), :] = jnp.zeros((PADR, 128), F32)
        nodeps = [[] for _ in range(NTILE)]

        def weave(a1_tiles, jobs):
            n = len(a1_tiles)
            for j, (b, t) in enumerate(a1_tiles):
                for f in jobs[(j * len(jobs)) // n:((j + 1) * len(jobs)) // n]:
                    f()
                stage_a1(b, t)

        cx[0].wait()
        cw[0].wait()
        cw[1].wait()
        for c in dma_order[DS0:DS1]:
            c.start()
        wq = wqkv_ref[:, 0:D]
        wk = wqkv_ref[:, D:2 * D]
        wv = wqkv_ref[:, 2 * D:3 * D]
        wvo_s[...] = _pk(_dot(wv, wao_ref[...]).astype(BF16))
        wqk_s[...] = _pk((_dot_nt(wq, wk) * (D ** -0.5 * LOG2E)).astype(BF16))
        for t in range(xgroups[0][1], xgroups[0][2]):
            stage_a1(0, t)
        cx[1].wait()
        cw[2].wait()
        for c in dma_order[DS1:]:
            c.start()
        wmi_s[...] = _pk(wmi_ref[...])
        qs, mxs = {}, {0: None, 1: None, 2: None}

        def jq(k):
            qs[k] = q_proj(k)

        def jc(k, ca, cb):
            mxs[k] = q_chunks(k, k % U, qs[k], None, nodeps, mxs[k], ca, cb)

        P = functools.partial
        c1 = (xgroups[0][2] * TA) // CK
        c2 = (xgroups[1][2] * TA) // CK
        jobs = [P(jq, k) for k in range(3)] + [P(stage_a2, k, k % U) for k in range(4)]
        jobs += [P(jc, k, 0, c1) for k in range(3)]
        weave([(0, t) for t in range(xgroups[1][1], xgroups[1][2])], jobs)
        cx[2].wait()
        jobs = [P(jc, k, c, c + 1) for c in range(c1, c2) for k in range(3)]
        weave([(0, t) for t in range(xgroups[2][1], xgroups[2][2])], jobs)
        cw[3].wait()
        cw[4].wait()
        cx[3].wait()
        wmo_s[...] = _pk(wmo_ref[...])
        wm_s[...] = _pk(wm_ref[...])
        zs = [zs_s[a] if ZS else 0 for a in range(4)]

        def jp(k):
            stage_p(k, k % U, z_s[...] != 0, nodeps)

        def jl(k):
            c1_mm(k, k % U, c1_conv(k % U, zs))

        jobs = [P(jc, k, c2, NC) for k in range(3)] + [P(jp, 0), P(jl, 0), P(jp, 1), P(jl, 1)]
        order = PO
        tiles = [(1, t) for t in range(nt1)]
        ti = 0
        for j, f in enumerate(jobs):
            f()
            for _ in range(order[j]):
                stage_a1(*tiles[ti])
                ti += 1
        assert ti == nt1

    @pl.when(step < NS - 1)
    @jax.named_scope("steady")
    def _():
        for i in range(UN):
            micro(step * UN + i, i)

    @pl.when(step == NS - 1)
    @jax.named_scope("last")
    def _():
        for i in range(UN):
            micro((NS - 1) * UN + i, i)


@jax.jit
def pallas_standalone__conformer_family_e_branchformer__speech_kernel(
    x, w_qkv, w_att_out, w_mlp_in, dw_csgu, w_mlp_out, dw_merge, w_merge,
):
    B, T, D = x.shape
    K = dw_csgu.shape[0]
    R = 80
    U = 5
    TP = 4096
    NSB = T // (R * UN)
    TH = -(-(R + 2 * PADR) // 32) * 32
    full = lambda a: pl.BlockSpec(a.shape, lambda s: (0,) * a.ndim)

    hbm = pl.BlockSpec(memory_space=pl.ANY)
    kern = functools.partial(_kernel, B=B, T=T, D=D, K=K, R=R, U=U, TP=TP)
    return pl.pallas_call(
        kern,
        grid=(B * NSB,),
        in_specs=[hbm, hbm, hbm, hbm, full(dw_csgu), hbm, full(dw_merge), hbm],
        out_specs=pl.BlockSpec((1, R * UN, D), lambda s: (s // NSB, s % NSB, 0)),
        out_shape=jax.ShapeDtypeStruct((B, T, D), x.dtype),
        scratch_shapes=[
            pltpu.VMEM(x.shape, BF16),
            pltpu.VMEM(w_qkv.shape, BF16),
            pltpu.VMEM(w_att_out.shape, BF16),
            pltpu.VMEM(w_mlp_in.shape, BF16),
            pltpu.VMEM(w_mlp_out.shape, BF16),
            pltpu.VMEM(w_merge.shape, BF16),
            pltpu.SemaphoreType.DMA((9,)),
            pltpu.VMEM((D // 2, D), U32),
            pltpu.VMEM((D // 2, D), U32),
            pltpu.VMEM((D // 2, 2 * D), U32),
            pltpu.VMEM((D // 2, D), U32),
            pltpu.VMEM((D, D), U32),
            pltpu.VMEM((K, D), F32),
            pltpu.VMEM((K, 2 * D), F32),
            pltpu.VMEM((B, TP // 2, D), U32),
            pltpu.VMEM((B, TP // 2, D), U32),
            pltpu.VMEM((U, R, D), F32),
            pltpu.VMEM((U, R, TP), F32),
            pltpu.VMEM((U, R, 128), F32),
            pltpu.VMEM((8, 128), jnp.int32),
            pltpu.SMEM((4,), jnp.int32),
        ] + [pltpu.VMEM((D // 128, TH, 128), F32)] * U + [pltpu.VMEM((2 * D // 128, TH, 128), F32)] * U,
        compiler_params=pltpu.CompilerParams(
            dimension_semantics=("arbitrary",),
            vmem_limit_bytes=100 * 1024 * 1024,
        ),
    )(x, w_qkv, w_att_out, w_mlp_in, dw_csgu, w_mlp_out, dw_merge, w_merge)
```

```python
import functools
import math

import jax
import jax.numpy as jnp
from jax import lax
import jax.experimental.pallas as pl
import jax.experimental.pallas.tpu as pltpu

F32 = jnp.float32
BF16 = jnp.bfloat16
U32 = jnp.uint32
EPS = 1e-5
LOG2E = 1.4426950408889634
PADR = 16
CK = 256
NPV = 12
NACC = 2
ACCB = 0
FIRST = 1
E = lambda k, d: int(d)
PV0, A2A, UA0, UA1, GA0, GA1 = E('PV0', 38), E('A2A', 1), E('UA0', 34), E('UA1', 54), E('GA0', 30), E('GA1', 50)
GLA, GL0, GW = E('GLA', 0), E('GL0', 12), E('GW', 10)
PO = [int(c) for c in '1113130']
ZS = E('ZS', 0)
DS0, DS1 = E('DS0', 9), E('DS1', 9)
UN = E('UN', 5)
WIN, ZW, THL = E('WIN', 6), E('ZW', 0), E('THL', 5)
A2L = E('A2L', 99)
ZM = E('ZM', 64)
NCP = E('NCP', 4)
ONLY = E('ONLY', 0)
PVL = E('PVL', 0)
CP = 512
LSP, LSD, LSW = E('LSP', 0), E('LSD', 1), E('LSW', 8)
WBC = E('WBC', 1)
PSPLIT, LSUM = E('PSPLIT', 0), E('LSUM', 0)
THR, THS, GRP = E('THR', 3), E('THS', 1), E('GRP', 1)
HA0, AW, AD, QK0, CORD = E('HA0', 40), E('AW', 20), E('AD', 10), E('QK0', 0), E('CORD', 0)
ANCH = 1


def _ln(x):
    m = jnp.mean(x, axis=-1, keepdims=True)
    xc = x - m
    v = jnp.mean(xc * xc, axis=-1, keepdims=True)
    return xc * lax.rsqrt(v + EPS)


def _gelu(x):
    c = math.sqrt(2.0 / math.pi)
    return 0.5 * x * (1.0 + jnp.tanh(c * (x + 0.044715 * (x * x * x))))


def _dot(a, b):
    return jnp.dot(a, b, preferred_element_type=F32)


def _dot_nt(a, b):
    return lax.dot_general(a, b, (((1,), (1,)), ((), ())), preferred_element_type=F32)


def _cat(parts, axis=-1):
    return jnp.concatenate(parts, axis=axis)


def _pk(x):
    return pltpu.bitcast(x, U32)


def _upk(x):
    return pltpu.bitcast(x, BF16)


def _conv_block(src_ref, lg, R, w_ref, K, zs):
    accs = [None] * NACC
    for b in range(8):
        for a in range(4):
            s = 8 * a + b
            if s < 1 or s > K:
                continue
            i = s - 1
            win = src_ref[a % NCP, lg, pl.ds(s, R), :]
            w = w_ref[lg, pl.ds(8 * i, 1), :]
            term = win * w
            j = (b * NACC) // 8 if ACCB else a % NACC
            accs[j] = term if accs[j] is None else accs[j] + term
    while len(accs) > 1:
        accs = [accs[j] + accs[j + 1] for j in range(0, len(accs), 2)]
    return accs[0]


def _conv_rows(src_ref, lg, r0, n, w_ref, K, zs, zw, never, rel):
    accs = [None] * NACC
    for b in range(8):
        for a in range(4):
            s = 8 * a + b
            if s < 1 or s > K:
                continue
            i = s - 1
            win = src_ref[a % NCP, lg, pl.ds(r0 + s, n), :]
            w = w_ref[lg, pl.ds(8 * i, 8), :] if WBC else w_ref[lg, pl.ds(8 * i, 1), :]
            j = (b * NACC) // 8 if ACCB else a % NACC
            if accs[j] is None:
                if rel is not None:
                    win = jnp.where(never, rel, win)
                accs[j] = win * w
            else:
                accs[j] = accs[j] + win * w
    while len(accs) > 1:
        accs = [accs[j] + accs[j + 1] for j in range(0, len(accs), 2)]
    return accs[0]


def _kernel(x_hbm, wqkv_hbm, wao_hbm, wmi_hbm, dwc_ref, wmo_hbm, dwm_ref, wm_hbm, o_ref,
            x_ref, wqkv_ref, wao_ref, wmi_ref, wmo_ref, wm_ref, sems,
            wqk_s, wvo_s, wmi_s, wmo_s, wm_s, dwc_s, dwm_s, xa_s, v_s, u_s, s_s, mx_s, z_s, zs_s, *rings,
            B, T, D, K, R, U, TP):
    g_s, m_s = rings[:U], rings[U:]
    step = pl.program_id(0)
    NK = T // R
    NKT = B * NK
    NS = NKT // UN
    NLG = D // 128
    TA = 400
    NC = TP // CK

    def split(k):
        if isinstance(k, int):
            return k // NK, k % NK
        b = k // NK
        return b, k - b * NK

    def rows(i, n):
        r = i * n
        return pl.ds(r if isinstance(r, int) else pl.multiple_of(r, 8), n)

    def ring_put(ref, lg, r0, val):
        n = val.shape[0]
        for cp in range(NCP):
            aa = [a for a in range(4) if a % NCP == cp]
            lo, hi = max(r0, 8 * min(aa)), min(r0 + n, 8 * max(aa) + R + 8)
            if hi > lo:
                ref[cp, lg, pl.ds(lo, hi - lo), :] = val[lo - r0:hi - r0]

    def halo_store(ref, k, kmod, lg, val):
        ring_put(ref[kmod], lg, PADR, val)
        top, bot = val[:PADR], val[R - PADR:]
        if kmod == 0:
            first = (k % NK == 0)
            top = jnp.where(first, 0.0, top) if not isinstance(first, bool) else (jnp.zeros_like(top) if first else top)
        if kmod == U - 1:
            last = (k % NK == NK - 1)
            bot = jnp.where(last, 0.0, bot) if not isinstance(last, bool) else (jnp.zeros_like(bot) if last else bot)
        ring_put(ref[(kmod - 1) % U], lg, PADR + R, top)
        ring_put(ref[(kmod + 1) % U], lg, 0, bot)

    def vregs(a):
        return [a[8 * r:8 * r + 8, l * 128:(l + 1) * 128] for r in range(a.shape[0] // 8) for l in range(a.shape[1] // 128)]

    def stage_a1(b, t):
        xa = _ln(x_ref[b, pl.ds(t * TA, TA), :].astype(F32))
        v = _dot(xa.astype(BF16), _upk(wvo_s[...]))
        xa_s[b, rows(t, TA // 2), :] = _pk(xa.astype(BF16))
        v_s[b, rows(t, TA // 2), :] = _pk(v.astype(BF16))

    def bc(a):
        return jnp.broadcast_to(a, (a.shape[0], 128))

    def stage_a2(k, kmod):
        b, i = split(k)
        h = _gelu(_dot(_upk(xa_s[b, rows(i, R // 2), :]), _upk(wmi_s[...])))
        u_s[kmod] = h[:, :D]
        hg = h[:, D:]
        mu = jnp.mean(hg, axis=-1, keepdims=True)
        xc = hg - mu
        rs = lax.rsqrt(jnp.mean(xc * xc, axis=-1, keepdims=True) + EPS)
        g = xc * rs
        for lg in range(NLG):
            halo_store(g_s, k, kmod, lg, g[:, lg * 128:(lg + 1) * 128])
        return vregs(h[:, :D]), vregs(hg), vregs(bc(mu)), vregs(bc(rs)), vregs(g)

    def c1_conv(kmod, zs):
        return [u_s[kmod, :, pl.ds(lg * 128, 128)] * _conv_block(g_s[kmod], lg, R, dwc_s, K, zs) for lg in range(NLG)]

    def c1_mm(k, kmod, parts):
        loc = _dot(_cat(parts).astype(BF16), _upk(wmo_s[...]))
        for lg in range(NLG):
            halo_store(m_s, k, kmod, NLG + lg, loc[:, lg * 128:(lg + 1) * 128])

    def c2_conv(kmod, zs):
        return [m_s[kmod][lg, pl.ds(PADR, R), :] + _conv_block(m_s[kmod], lg, R, dwm_s, K, zs) for lg in range(2 * NLG)]

    def c2_mm(k, pos, parts):
        b, i = split(k)
        r0 = i * R
        r0 = r0 if isinstance(r0, int) else pl.multiple_of(r0, 16)
        y = _dot(_cat(parts).astype(BF16), _upk(wm_s[...])) + x_ref[b, pl.ds(r0, R), :].astype(F32)
        o_ref[0, pl.ds(pos * R, R), :] = y.astype(o_ref.dtype)

    def q_proj(k):
        b, i = split(k)
        return _dot(_upk(xa_s[b, rows(i, R // 2), :]), _upk(wqk_s[...])).astype(BF16)

    def kv_chunk(ref, b, c, never, deps):
        blks = []
        for kt in range(CK // 128):
            parts = []
            for lg in range(NLG):
                t = ref[b, pl.ds(c * CK // 2 + kt * 64, 64), pl.ds(lg * 128, 128)]
                dd = deps[(c * (CK // 128) + kt) * NLG + lg]
                if dd:
                    pieces = [t[8 * j:8 * j + 8] for j in range(8)]
                    for j, d in enumerate(dd):
                        jj = 7 - j if FIRST else j
                        pieces[jj] = jnp.where(never, pltpu.bitcast(d, U32), pieces[jj])
                    t = _cat(pieces, axis=0)
                parts.append(t)
            blks.append(_cat(parts))
        return _upk(_cat(blks, axis=0))

    def q_chunks(k, kmod, q, never, deps, mx, ca, cb, hook=None):
        b, _ = split(k)
        for c in range(ca, cb):
            s = _dot_nt(q, kv_chunk(xa_s, b, c, never, deps))
            if hook is not None:
                hook(NC + c, s)
            for l in range(CK // 128):
                sl = s[:, l * 128:(l + 1) * 128]
                c0 = c * CK + l * 128
                if c0 + 128 > T:
                    col = lax.broadcasted_iota(jnp.int32, (R, 128), 1) + c0
                    sl = jnp.where(col < T, sl, -jnp.inf)
                s_s[kmod, :, pl.ds(c0, 128)] = sl
                mx = sl if mx is None else jnp.maximum(mx, sl)
        if cb == NC:
            mx_s[kmod] = jnp.broadcast_to(jnp.max(mx, axis=-1, keepdims=True), (R, 128))
        return mx

    def stage_q(k, kmod, q, never, deps, hook=None):
        q_chunks(k, kmod, q, never, deps, None, 0, NC, hook)

    def v_tiles(b, c, lg, never, deps):
        blks = []
        for kt in range(CP // 128):
            t = v_s[b, pl.ds(c * CP // 2 + kt * 64, 64), pl.ds(lg * 128, 128)]
            dd = deps[kt]
            if dd:
                pieces = [t[8 * j:8 * j + 8] for j in range(8)]
                for j, d in enumerate(dd):
                    jj = 7 - j if FIRST else j
                    pieces[jj] = jnp.where(never, pltpu.bitcast(d, U32), pieces[jj])
                t = _cat(pieces, axis=0)
            blks.append(t)
        return _upk(_cat(blks, axis=0))

    def stage_p(k, kmod, never, deps, hook=None, thr=0, lshook=None):
        b, _ = split(k)
        m = mx_s[kmod]
        neverr = _cat([never] * (R // 8), axis=0)
        NCP_ = TP // CP
        TPC = CP // 128
        ls = None
        pbs, pvs, accs = [], [], []
        for lg in range(NLG):
            acc = None
            for c in range(NCP_):
                gc = lg * NCP_ + c
                if lg == 0:
                    ps = []
                    if thr and c >= thr and (c % THS == 0):
                        m = jnp.where(neverr, pvs[c - thr], m)
                    for l in range(TPC):
                        p = jnp.exp2(s_s[kmod, :, pl.ds(c * CP + l * 128, 128)] - m)
                        ps.append(p)
                    if LSUM:
                        t = (ps[0] + ps[1]) + (ps[2] + ps[3])
                        ls = t if ls is None else ls + t
                    else:
                        for p in ps:
                            ls = p if ls is None else ls + p
                    pbs.append(_cat(ps).astype(BF16))
                    if lshook is not None:
                        lshook(c, ls)
                pv = _dot(pbs[c], v_tiles(b, c, lg, never, deps[gc * TPC:(gc + 1) * TPC]))
                if hook is not None:
                    hook(gc, pv)
                pvs.append(pv)
                acc = pv if acc is None else acc + pv
            accs.append(acc)
        acc = _cat(accs)
        l = jnp.sum(ls, axis=-1, keepdims=True)
        rinv = 1.0 / l
        glob = acc * rinv
        for lg in range(NLG):
            halo_store(m_s, k, kmod, lg, glob[:, lg * 128:(lg + 1) * 128])
        return vregs(bc(rinv)), vregs(glob)

    NTILE = (TP // 128) * NLG

    def place(slots, items, lo, hi, grp=1):
        ng = -(-len(items) // grp)
        for j, it in enumerate(items):
            pos = lo + (((j // grp) * 2 + 1) * (hi - lo)) // (2 * ng) if grp > 1 else lo + (j * (hi - lo)) // len(items)
            while len(slots[pos]) >= 8:
                pos += 1
            slots[pos].append(it)

    def micro(n, pos):
        nmod = pos % U
        ok = lambda k: (not isinstance(k, int)) or 0 <= k < NKT
        never = z_s[...] != 0
        zs = [pl.multiple_of(zs_s[a], ZM) if ZS else 0 for a in range(4)]
        NV = R // 8
        TPC = NTILE // NC
        hasp, hasq = ok(n + 2), ok(n + 3)
        lo = 0 if hasp else NTILE
        hi = 2 * NTILE if hasq else NTILE
        res = {}
        jobs = []

        def zw(r):
            return zs_s[4 + (pos % 5) * NV + r] if ZW else 0

        if ok(n):
            if isinstance(n, int) and n == NKT - 1:
                for lg in range(2 * NLG):
                    ring_put(m_s[nmod], lg, PADR + R, jnp.zeros((PADR, 128), F32))
            for lg in range(2 * NLG):
                for r in range(NV):
                    jobs.append((('c2', lg, r), lambda rel, lg=lg, r=r: _conv_rows(
                        m_s[nmod], lg, 8 * r, 8, dwm_s, K, zs, zw(r), never, rel)))
        if ok(n + 2):
            km = (nmod + 2) % U
            if isinstance(n, int) and n + 2 == NKT - 1:
                for lg in range(NLG):
                    ring_put(g_s[km], lg, PADR + R, jnp.zeros((PADR, 128), F32))
            j1 = []
            for lg in range(NLG):
                for r in range(NV):
                    j1.append((('c1', lg, r), lambda rel, lg=lg, r=r: u_s[km, pl.ds(8 * r, 8), pl.ds(lg * 128, 128)] * _conv_rows(
                        g_s[km], lg, 8 * r, 8, dwc_s, K, zs, zw(r), never, rel)))
            jobs = j1 + jobs if CORD else jobs + j1
        if hasp and hasq:
            npv = min(NPV, len(jobs))
        elif hasp:
            npv = len(jobs)
        else:
            npv = 0
        pv0 = PV0 if hasq else PVL
        dls = [pv0 + (j * (NTILE - pv0)) // max(npv, 1) for j in range(npv)]
        nq = len(jobs) - npv
        dls += [NTILE + QK0 + (j * (NTILE - QK0)) // nq if hasq else None for j in range(nq)]
        slots = [[] for _ in range(2 * NTILE)]
        pending = {}
        for (key, fn), dl in zip(jobs, dls):
            rc = None if dl is None else dl // TPC - WIN
            if rc is None or rc < lo // TPC or not WIN:
                res[key] = fn(None)
                if dl is not None:
                    slots[dl].append(res[key])
            else:
                pending.setdefault(rc, []).append((key, fn, dl))

        def hook(gc, val):
            for j, (key, fn, dl) in enumerate(pending.pop(gc, [])):
                res[key] = fn(val[8 * (j % NV):8 * (j % NV) + 8, :128])
                slots[dl].append(res[key])

        def put(items, a, b, grp=1):
            a, b = max(a, lo), min(b, hi)
            if items and b > a:
                place(slots, items, a, b, grp)

        if hasq:
            q = q_proj(n + 3)
        if ok(n + 4):
            uu, hh, mu, rs, gg = stage_a2(n + 4, (nmod + 4) % U)
            if A2A and pos >= UN - A2L:
                off = 0 if hasp else NTILE
                if UA1 > UA0:
                    put(uu, off + UA0, off + UA1)
                put(hh, off + HA0, off + HA0 + AW)
                if A2A == 1:
                    put(mu, off + HA0 + AD, off + HA0 + AD + AW)
                    put(rs, off + HA0 + 2 * AD, off + HA0 + 2 * AD + AW)
                    put(gg, off + HA0 + 2 * AD + 4, off + HA0 + 2 * AD + 4 + AW)
        if hasp:
            def lshook(c, ls):
                if LSP and (c + 1) % LSP == 0:
                    a = (c + 1 + LSD) * TPC
                    put(vregs(ls), a, a + LSW)
            ri, gl = stage_p(n + 2, (nmod + 2) % U, never, slots[:NTILE], hook, THR if (pos >= UN - THL) else 0, lshook)
            if hasq and GLA and pos >= UN - A2L:
                put(ri, NTILE + GL0, NTILE + GL0 + GW)
                put(gl, NTILE + GL0 + 4, NTILE + GL0 + 4 + GW)
        if hasq:
            stage_q(n + 3, (nmod + 3) % U, q, never, slots[NTILE:], hook)
        assert not pending
        if ok(n):
            c2_mm(n, pos, [_cat([res['c2', lg, r] for r in range(NV)], axis=0) for lg in range(2 * NLG)])
        if ok(n + 2):
            c1_mm(n + 2, (nmod + 2) % U, [_cat([res['c1', lg, r] for r in range(NV)], axis=0) for lg in range(NLG)])

    @pl.when(step == 0)
    @jax.named_scope("prologue")
    def _():
        if ONLY:
            return
        nt1 = T // TA
        xgroups = [(0, 0, 2), (0, 2, 6), (0, 6, nt1), (1, 0, nt1)]
        cw = [pltpu.make_async_copy(src, dst, sems.at[j]) for j, (src, dst) in enumerate(
            [(wqkv_hbm, wqkv_ref), (wao_hbm, wao_ref), (wmi_hbm, wmi_ref), (wmo_hbm, wmo_ref), (wm_hbm, wm_ref)])]
        cx = [pltpu.make_async_copy(x_hbm.at[b, pl.ds(t0 * TA, (t1 - t0) * TA), :],
                                    x_ref.at[b, pl.ds(t0 * TA, (t1 - t0) * TA), :], sems.at[5 + j])
              for j, (b, t0, t1) in enumerate(xgroups)]
        dma_order = [cx[0], cw[0], cw[1], cx[1], cw[2], cx[2], cw[3], cw[4], cx[3]]
        for c in dma_order[:DS0]:
            c.start()
        z_s[...] = jnp.zeros(z_s.shape, z_s.dtype)
        for a in range(64):
            zs_s[a] = 0
        for lg in range(NLG):
            wl = dwc_ref[:, pl.ds(lg * 128, 128)].astype(F32)
            for i in range(K):
                dwc_s[lg, pl.ds(8 * i, 8), :] = jnp.broadcast_to(wl[i:i + 1], (8, 128))
        for lg in range(2 * NLG):
            wl = dwm_ref[:, pl.ds(lg * 128, 128)].astype(F32)
            for i in range(K):
                wi = wl[i:i + 1] + 1.0 if i == K // 2 else wl[i:i + 1]
                dwm_s[lg, pl.ds(8 * i, 8), :] = jnp.broadcast_to(wi, (8, 128))
        for b in range(B):
            xa_s[b, pl.ds(T // 2, (TP - T) // 2), :] = jnp.zeros(((TP - T) // 2, D), U32)
            v_s[b, pl.ds(T // 2, (TP - T) // 2), :] = jnp.zeros(((TP - T) // 2, D), U32)
        for lg in range(NLG):
            ring_put(g_s[0], lg, 0, jnp.zeros((PADR, 128), F32))
        for lg in range(2 * NLG):
            ring_put(m_s[0], lg, 0, jnp.zeros((PADR, 128), F32))
        nodeps = [[] for _ in range(NTILE)]

        def weave(a1_tiles, jobs):
            n = len(a1_tiles)
            for j, (b, t) in enumerate(a1_tiles):
                for f in jobs[(j * len(jobs)) // n:((j + 1) * len(jobs)) // n]:
                    f()
                stage_a1(b, t)

        cx[0].wait()
        cw[0].wait()
        cw[1].wait()
        for c in dma_order[DS0:DS1]:
            c.start()
        wq = wqkv_ref[:, 0:D]
        wk = wqkv_ref[:, D:2 * D]
        wv = wqkv_ref[:, 2 * D:3 * D]
        wvo_s[...] = _pk(_dot(wv, wao_ref[...]).astype(BF16))
        wqk_s[...] = _pk((_dot_nt(wq, wk) * (D ** -0.5 * LOG2E)).astype(BF16))
        for t in range(xgroups[0][1], xgroups[0][2]):
            stage_a1(0, t)
        cx[1].wait()
        cw[2].wait()
        for c in dma_order[DS1:]:
            c.start()
        wmi_s[...] = _pk(wmi_ref[...])
        qs, mxs = {}, {0: None, 1: None, 2: None}

        def jq(k):
            qs[k] = q_proj(k)

        def jc(k, ca, cb):
            mxs[k] = q_chunks(k, k % U, qs[k], None, nodeps, mxs[k], ca, cb)

        P = functools.partial
        c1 = (xgroups[0][2] * TA) // CK
        c2 = (xgroups[1][2] * TA) // CK
        jobs = [P(jq, k) for k in range(3)] + [P(stage_a2, k, k % U) for k in range(4)]
        jobs += [P(jc, k, 0, c1) for k in range(3)]
        weave([(0, t) for t in range(xgroups[1][1], xgroups[1][2])], jobs)
        cx[2].wait()
        jobs = [P(jc, k, c, c + 1) for c in range(c1, c2) for k in range(3)]
        weave([(0, t) for t in range(xgroups[2][1], xgroups[2][2])], jobs)
        cw[3].wait()
        cw[4].wait()
        cx[3].wait()
        wmo_s[...] = _pk(wmo_ref[...])
        wm_s[...] = _pk(wm_ref[...])
        zs = [pl.multiple_of(zs_s[a], ZM) if ZS else 0 for a in range(4)]

        def jp(k):
            stage_p(k, k % U, z_s[...] != 0, nodeps)

        def jl(k):
            c1_mm(k, k % U, c1_conv(k % U, zs))

        jobs = [P(jc, k, c2, NC) for k in range(3)] + [P(jp, 0), P(jl, 0), P(jp, 1), P(jl, 1)]
        order = PO
        tiles = [(1, t) for t in range(nt1)]
        ti = 0
        for j, f in enumerate(jobs):
            f()
            for _ in range(order[j]):
                stage_a1(*tiles[ti])
                ti += 1
        assert ti == nt1

    @pl.when(step < NS - 1)
    @jax.named_scope("steady")
    def _():
        for i in range(UN):
            micro(step * UN + i, i)

    @pl.when(step == NS - 1)
    @jax.named_scope("last")
    def _():
        if ONLY:
            return
        for i in range(UN):
            micro((NS - 1) * UN + i, i)


@jax.jit
def pallas_standalone__conformer_family_e_branchformer__speech_kernel(
    x, w_qkv, w_att_out, w_mlp_in, dw_csgu, w_mlp_out, dw_merge, w_merge,
):
    B, T, D = x.shape
    K = dw_csgu.shape[0]
    R = 80
    U = 5
    TP = 4096
    NSB = T // (R * UN)
    TH = -(-(R + 2 * PADR) // 32) * 32
    full = lambda a: pl.BlockSpec(a.shape, lambda s: (0,) * a.ndim)

    hbm = pl.BlockSpec(memory_space=pl.ANY)
    kern = functools.partial(_kernel, B=B, T=T, D=D, K=K, R=R, U=U, TP=TP)
    return pl.pallas_call(
        kern,
        grid=(B * NSB,),
        in_specs=[hbm, hbm, hbm, hbm, full(dw_csgu), hbm, full(dw_merge), hbm],
        out_specs=pl.BlockSpec((1, R * UN, D), lambda s: (s // NSB, s % NSB, 0)),
        out_shape=jax.ShapeDtypeStruct((B, T, D), x.dtype),
        scratch_shapes=[
            pltpu.VMEM(x.shape, BF16),
            pltpu.VMEM(w_qkv.shape, BF16),
            pltpu.VMEM(w_att_out.shape, BF16),
            pltpu.VMEM(w_mlp_in.shape, BF16),
            pltpu.VMEM(w_mlp_out.shape, BF16),
            pltpu.VMEM(w_merge.shape, BF16),
            pltpu.SemaphoreType.DMA((9,)),
            pltpu.VMEM((D // 2, D), U32),
            pltpu.VMEM((D // 2, D), U32),
            pltpu.VMEM((D // 2, 2 * D), U32),
            pltpu.VMEM((D // 2, D), U32),
            pltpu.VMEM((D, D), U32),
            pltpu.VMEM((D // 128, 256, 128), F32),
            pltpu.VMEM((2 * D // 128, 256, 128), F32),
            pltpu.VMEM((B, TP // 2, D), U32),
            pltpu.VMEM((B, TP // 2, D), U32),
            pltpu.VMEM((U, R, D), F32),
            pltpu.VMEM((U, R, TP), F32),
            pltpu.VMEM((U, R, 128), F32),
            pltpu.VMEM((8, 128), jnp.int32),
            pltpu.SMEM((64,), jnp.int32),
        ] + [pltpu.VMEM((NCP, D // 128, TH, 128), F32)] * U + [pltpu.VMEM((NCP, 2 * D // 128, TH, 128), F32)] * U,
        compiler_params=pltpu.CompilerParams(
            dimension_semantics=("arbitrary",),
            vmem_limit_bytes=100 * 1024 * 1024,
        ),
    )(x, w_qkv, w_att_out, w_mlp_in, dw_csgu, w_mlp_out, dw_merge, w_merge)
```

```python
import functools
import math

import jax
import jax.numpy as jnp
from jax import lax
import jax.experimental.pallas as pl
import jax.experimental.pallas.tpu as pltpu

F32 = jnp.float32
BF16 = jnp.bfloat16
U32 = jnp.uint32
EPS = 1e-5
LOG2E = 1.4426950408889634
PADR = 16
CK = 256
NPV = 6
NACC = 2
ACCB = 0
FIRST = 1
E = lambda k, d: int(d)
PV0, A2A, UA0, UA1, GA0, GA1 = E('PV0', 40), E('A2A', 1), E('UA0', 10), E('UA1', 54), E('GA0', 30), E('GA1', 50)
GLA, GL0, GW = E('GLA', 0), E('GL0', 12), E('GW', 10)
PO = [int(c) for c in '12133']
ZS = E('ZS', 0)
DS0, DS1 = E('DS0', 9), E('DS1', 9)
UN = E('UN', 5)
WIN, ZW, THL = E('WIN', 5), E('ZW', 0), E('THL', 1)
A2L = E('A2L', 99)
ZM = E('ZM', 64)
NCP = E('NCP', 1)
ONLY = E('ONLY', 0)
RR = E('RR', 56)
JG = E('JG', 5)
ONLYP = E('ONLYP', 0)
DEC = E('DEC', 1)
MORD = E('MORD', 1)
PLANS = {
 1: ([(0, 0, 2), (0, 2, 4), (0, 4, 6), (0, 6, 10), (1, 0, 5), (1, 5, 10)],
     'x0 w0 w1 x1 w2 x2 x3 w3 w4 x4 x5',
     '!x0 L0 L1 '
     '!w0 !w1 F V0 V1 Q0 Q1 Q2 C0-3 '
     '!x1 !w2 !x2 W2 L2 A0 A1 L3 A2 A3 L4 L5 V2 V3 V4 '
     '!x3 L6 V5 C3-5 L7 C5-7 L8 C7-9 L9 V6 V7 V8 '
     '!w3 !w4 !x4 W3 W4 V9 L10 C9-12 L11 C12-14 L12 C14-16 L13 L14 V10 V11 V12 V13 '
     '!x5 V14 L15 P0 L16 V15 L17 V16 P1 L18 V17 L19 V18 V19'),
 2: ([(0, 0, 2), (0, 2, 6), (0, 6, 10), (1, 0, 5), (1, 5, 10)],
     'x0 w0 w1 w2 x1 x2 w3 w4 x3 x4',
     '!x0 L0 L1 '
     '!w0 !w1 F V0 Q0 Q1 Q2 C0-3 '
     '!w2 !x1 W2 V1 L2 A0 A1 L3 A2 A3 L4 L5 V2 V3 '
     '!x2 V4 L6 V5 C3-5 L7 C5-7 L8 C7-9 L9 V6 V7 V8 '
     '!w3 !w4 !x3 W3 W4 V9 L10 C9-12 L11 C12-14 L12 C14-16 L13 L14 V10 V11 V12 V13 '
     '!x4 V14 L15 P0 L16 V15 L17 V16 P1 L18 V17 L19 V18 V19'),
 3: ([(0, 0, 2), (0, 2, 6), (0, 6, 10), (1, 0, 3), (1, 3, 10)],
     'x0 w0 w1 w2 x1 x2 x3 w3 w4 x4',
     '!x0 L0 L1 '
     '!w0 !w1 F V0 Q0 Q1 Q2 C0-3 '
     '!w2 !x1 W2 V1 L2 A0 A1 L3 A2 A3 L4 L5 V2 V3 '
     '!x2 !x3 V4 L6 V5 C3-5 L7 C5-7 L8 C7-9 L9 V6 V7 L10 V8 V9 L11 C9-12 L12 C12-14 '
     '!w3 !w4 !x4 W3 W4 C14-16 L13 V10 V11 L14 V12 L15 V13 P0 L16 V14 L17 V15 V16 P1 L18 V17 L19 V18 V19'),
 4: ([(0, 0, 3), (0, 3, 6), (0, 6, 10), (1, 0, 3), (1, 3, 10)],
     'x0 w0 w1 w2 x1 x2 x3 w3 w4 x4',
     '!x0 L0 L1 L2 '
     '!w0 !w1 !w2 W2 F V0 V1 Q0 Q1 Q2 A0 A1 A2 A3 C0-4 '
     '!x1 !x2 V2 L3 L4 V3 L5 V4 L6 C4-7 V5 L7 C7-9 L8 V6 L9 V7 V8 '
     '!x3 V9 L10 C9-12 L11 C12-14 L12 C14-16 V10 V11 '
     '!w3 !w4 !x4 W3 W4 V12 L13 L14 P0 L15 V13 L16 V14 L17 V15 V16 P1 L18 V17 L19 V18 V19'),
 5: ([(0, 0, 2), (0, 2, 6), (0, 6, 10), (1, 0, 4), (1, 4, 10)],
     'x0 w0 w1 w2 x1 x2 x3 w3 w4 x4',
     '!x0 L0 L1 '
     '!w0 !w1 !w2 W2 F V0 V1 Q0 Q1 Q2 A0 A1 A2 A3 C0-3 '
     '!x1 !x2 L2 L3 V2 L4 V3 L5 C3-6 V4 L6 V5 C6-9 L7 L8 V6 L9 V7 V8 '
     '!x3 V9 L10 C9-12 L11 C12-14 L12 C14-16 L13 V10 V11 V12 '
     '!w3 !w4 !x4 W3 W4 V13 L14 P0 L15 V14 L16 V15 L17 V16 P1 L18 V17 L19 V18 V19'),
}
XG, DORD, PLAN = PLANS[E('PL', 1)]
DORD = DORD.split()
NPVF = E('NPVF', 34)
TORD = E('TORD', 1)
PVL = E('PVL', 0)
CP = 512
LSP, LSD, LSW = E('LSP', 0), E('LSD', 1), E('LSW', 8)
WBC = E('WBC', 1)
PSPLIT, LSUM = E('PSPLIT', 0), E('LSUM', 0)
THR, THS, GRP = E('THR', 0), E('THS', 2), E('GRP', 1)
HA0, AW, AD, QK0, CORD = E('HA0', 40), E('AW', 14), E('AD', 8), E('QK0', 8), E('CORD', 0)
ANCH = 1


def _ln(x):
    m = jnp.mean(x, axis=-1, keepdims=True)
    xc = x - m
    v = jnp.mean(xc * xc, axis=-1, keepdims=True)
    return xc * lax.rsqrt(v + EPS)


def _ln_mxu_var(x):
    d = x.shape[-1]
    m = jnp.mean(x, axis=-1, keepdims=True)
    xc = x - m
    sq = xc * xc
    q = sq[:, :128]
    for l in range(1, d // 128):
        q = q + sq[:, l * 128:(l + 1) * 128]
    v = jnp.dot(q.astype(BF16), jnp.ones((128, 128), BF16), preferred_element_type=F32) * (1.0 / d)
    r = lax.rsqrt(v + EPS)
    return xc * jnp.concatenate([r] * (d // 128), axis=-1)


def _gelu(x):
    c = math.sqrt(2.0 / math.pi)
    return 0.5 * x * (1.0 + jnp.tanh(c * (x + 0.044715 * (x * x * x))))


def _dot(a, b):
    return jnp.dot(a, b, preferred_element_type=F32)


def _dot_nt(a, b):
    return lax.dot_general(a, b, (((1,), (1,)), ((), ())), preferred_element_type=F32)


def _cat(parts, axis=-1):
    return jnp.concatenate(parts, axis=axis)


def _pk(x):
    return pltpu.bitcast(x, U32)


def _upk(x):
    return pltpu.bitcast(x, BF16)


def _even_odd(xb):
    xu = _pk(xb)
    return pltpu.bitcast(xu << 16, F32), pltpu.bitcast(xu & jnp.uint32(0xFFFF0000), F32)


def _interleave_bf16(e, o):
    rb = lambda a: pltpu.bitcast(a.astype(BF16).astype(F32), U32)
    return _upk((rb(e) >> 16) | (rb(o) & jnp.uint32(0xFFFF0000)))


def _ffa_pair(ring, lg, j, w_ref, never, rel):
    outs = []
    for q, nt in enumerate((16, 16, 15)):
        acc = None
        ks = list(range(nt))
        if TORD == 1:
            ks = [k for pair in zip(range(8), range(8, 16)) for k in pair if k < nt]
        for k in ks:
            o = k + 1
            win = ring[lg, 2 * q + ((o // 8) % 2 if NCP > 1 else 0), pl.ds(8 * j + o, 8), :]
            w = w_ref[lg, pl.ds(8 * (16 * q + k), 8), :]
            if acc is None:
                if rel is not None:
                    win = jnp.where(never, rel, win)
                acc = win * w
            else:
                acc = acc + win * w
        outs.append(acc)
    return outs[0] + outs[1], outs[0] + outs[2]


def _ffa_chain(ring, lg, q, j0, nj, w_ref, never, rel, init):
    nt = (16, 16, 15)[q]
    acc = init
    ks = list(range(nt))
    if TORD == 1:
        ks = [k for pair in zip(range(8), range(8, 16)) for k in pair if k < nt]
    for n_, k in enumerate(ks):
        o = k + 1
        win = ring[lg, 2 * q + ((o // 8) % 2 if NCP > 1 else 0), pl.ds(8 * j0 + o, 8 * nj), :]
        w = w_ref[lg, pl.ds(8 * (16 * q + k), 8), :]
        if n_ == 0 and rel is not None:
            w = jnp.where(never, rel, w)
        w = _cat([w] * nj, axis=0)
        acc = win * w if acc is None else acc + win * w
    return acc


def _kernel(x_hbm, wqkv_hbm, wao_hbm, wmi_hbm, dwc_ref, wmo_hbm, dwm_ref, wm_hbm, o_ref,
            x_ref, wqkv_ref, wao_ref, wmi_ref, wmo_ref, wm_ref, sems,
            wqk_s, wvo_s, wmi_s, wmo_s, wm_s, dwc_s, dwm_s, xa_s, v_s, u_s, s_s, mx_s, z_s, *rings,
            B, T, D, K, R, U, TP):
    g_s, m_s = rings[:U], rings[U:]
    xa_b, v_b = xa_s, v_s
    xa_s, v_s = xa_b.bitcast(U32), v_b.bitcast(U32)
    step = pl.program_id(0)
    NK = T // R
    NKT = B * NK
    NS = NKT // UN
    NLG = D // 128
    TA = 400
    NC = TP // CK

    def split(k):
        if isinstance(k, int):
            return k // NK, k % NK
        b = sum((k >= j * NK).astype(jnp.int32) for j in range(1, B))
        return b, k - b * NK

    def rows(i, n):
        r = i * n
        return pl.ds(r if isinstance(r, int) else pl.multiple_of(r, 8), n)

    H = R // 2
    NH = H // 8

    def seq_put(ref, q, lg, r0, val):
        n = val.shape[0]
        if NCP == 1:
            ref[lg, 2 * q, pl.ds(r0, n), :] = val
            return
        if not (q == 2 and r0 >= 8 + H):
            ref[lg, 2 * q, pl.ds(r0, n), :] = val
        if r0 >= 8:
            ref[lg, 2 * q + 1, pl.ds(r0, n), :] = val

    def halo_store(ref, k, kmod, lg, val):
        cur, prv, nxt = ref[kmod], ref[(kmod - 1) % U], ref[(kmod + 1) % U]
        xe, xo = val[:H], val[H:]
        row0 = lax.broadcasted_iota(jnp.int32, (8, 128), 0) == 0
        rot = [pltpu.roll(xo[8 * i:8 * i + 8], 1, 0) for i in range(NH)]
        nxt[lg, 6, pl.ds(0, 8), :] = rot[-1]
        rot = [cur[lg, 6, pl.ds(0, 8), :]] + rot
        sh = _cat([jnp.where(row0, rot[i], rot[i + 1]) for i in range(NH)], axis=0)
        zero = jnp.zeros((8, 128), F32)
        first = (split(k)[1] == 0) if kmod == 0 else False
        last = (split(k)[1] == NK - 1) if kmod == U - 1 else False
        sh0 = sh[:8]
        if first is not False:
            cut = row0 if first is True else jnp.logical_and(row0, first)
            sh = _cat([jnp.where(cut, 0.0, sh0), sh[8:]], axis=0)
        seqs = [xe, sh - xe, xo - xe]
        for q, v in enumerate(seqs):
            seq_put(cur, q, lg, 8, v)
            top, bot = v[:8], v[H - 8:]
            if first is not False:
                edge = jnp.where(row0, sh0, 0.0) if q == 1 else zero
                top = None if (first is True and k == 0) else (edge if first is True else jnp.where(first, edge, top))
            if last is not False:
                bot = zero if last is True else jnp.where(last, 0.0, bot)
            if top is not None:
                seq_put(prv, q, lg, 8 + H, top)
            seq_put(nxt, q, lg, 0, bot)
        if isinstance(k, int) and k == NKT - 1:
            e = rot[-1]
            for q in range(3):
                seq_put(cur, q, lg, 8 + H, jnp.where(row0, e, 0.0) if q == 1 else zero)

    def vregs(a):
        return [a[8 * r:8 * r + 8, l * 128:(l + 1) * 128] for r in range(a.shape[0] // 8) for l in range(a.shape[1] // 128)]

    def xa_rows(b, r):
        return _upk(_cat([xa_s[b, lg, r, :] for lg in range(NLG)]))

    def ln_tile(b, t):
        eo = _even_odd(x_ref[b, pl.ds(t * TA, TA), :])
        xa = _ln(_cat([eo[par][i * H:(i + 1) * H] for i in range(TA // R) for par in range(2)], axis=0))
        for lg in range(NLG):
            xa_b[b, lg, pl.ds(t * TA, TA), :] = xa[:, lg * 128:(lg + 1) * 128].astype(BF16)

    def v_tile(b, t):
        v = _dot(xa_rows(b, rows(t, TA // 2)), _upk(wvo_s[...]))
        for lg in range(NLG):
            v_b[b, lg, pl.ds(t * TA, TA), :] = v[:, lg * 128:(lg + 1) * 128].astype(BF16)

    def stage_a1(b, t):
        ln_tile(b, t)
        v_tile(b, t)

    def bc(a):
        return jnp.broadcast_to(a, (a.shape[0], 128))

    def stage_a2(k, kmod):
        b, i = split(k)
        h = _gelu(_dot(xa_rows(b, rows(i, R // 2)), _upk(wmi_s[...])))
        u_s[kmod] = h[:, :D]
        hg = h[:, D:]
        mu = jnp.mean(hg, axis=-1, keepdims=True)
        xc = hg - mu
        rs = lax.rsqrt(jnp.mean(xc * xc, axis=-1, keepdims=True) + EPS)
        g = xc * rs
        for lg in range(NLG):
            halo_store(g_s, k, kmod, lg, g[:, lg * 128:(lg + 1) * 128])
        return vregs(h[:, :D]), vregs(hg), vregs(bc(mu)), vregs(bc(rs)), vregs(g)

    def c1_job(km, lg, j, never, rel):
        ye, yo = _ffa_pair(g_s[km], lg, j, dwc_s, never, rel)
        lanes = pl.ds(lg * 128, 128)
        return u_s[km, pl.ds(8 * j, 8), lanes] * ye, u_s[km, pl.ds(H + 8 * j, 8), lanes] * yo

    def gather(res, name, nlg):
        return [_cat([res[name, lg, j][0] for j in range(NH)] + [res[name, lg, j][1] for j in range(NH)], axis=0)
                for lg in range(nlg)]

    def c1_mm(k, kmod, parts):
        loc = _dot(_cat(parts).astype(BF16), _upk(wmo_s[...]))
        for lg in range(NLG):
            halo_store(m_s, k, kmod, NLG + lg, loc[:, lg * 128:(lg + 1) * 128])

    def c2_mm(k, pos, parts):
        b, i = split(k)
        r0 = i * R
        r0 = r0 if isinstance(r0, int) else pl.multiple_of(r0, 16)
        y = _dot(_cat(parts).astype(BF16), _upk(wm_s[...]))
        xe, xo = _even_odd(x_ref[b, pl.ds(r0, R), :])
        o_ref[pl.ds(pos * R, R), :] = _interleave_bf16(y[:H] + xe, y[H:] + xo)

    def q_proj(k):
        b, i = split(k)
        return _dot(xa_rows(b, rows(i, R // 2)), _upk(wqk_s[...])).astype(BF16)

    def kv_chunk(ref, b, c, never, deps):
        blks = []
        for kt in range(CK // 128):
            parts = []
            for lg in range(NLG):
                t = ref[b, lg, pl.ds(c * CK // 2 + kt * 64, 64), :]
                dd = deps[(c * (CK // 128) + kt) * NLG + lg]
                if dd:
                    pieces = [t[8 * j:8 * j + 8] for j in range(8)]
                    for j, d in enumerate(dd):
                        jj = 7 - j if FIRST else j
                        pieces[jj] = jnp.where(never, pltpu.bitcast(d, U32), pieces[jj])
                    t = _cat(pieces, axis=0)
                parts.append(t)
            blks.append(_cat(parts))
        return _upk(_cat(blks, axis=0))

    def q_chunks(k, kmod, q, never, deps, mx, ca, cb, hook=None):
        b, _ = split(k)
        for c in range(ca, cb):
            s = _dot_nt(q, kv_chunk(xa_s, b, c, never, deps))
            if hook is not None:
                hook(NC + c, s)
            for l in range(CK // 128):
                sl = s[:, l * 128:(l + 1) * 128]
                c0 = c * CK + l * 128
                if c0 + 128 > T:
                    col = lax.broadcasted_iota(jnp.int32, (R, 128), 1) + c0
                    sl = jnp.where(col < T, sl, -jnp.inf)
                s_s[kmod, :, pl.ds(c0, 128)] = sl
                mx = sl if mx is None else jnp.maximum(mx, sl)
        if cb == NC:
            mx_s[kmod] = jnp.broadcast_to(jnp.max(mx, axis=-1, keepdims=True), (R, 128))
        return mx

    def stage_q(k, kmod, q, never, deps, hook=None):
        q_chunks(k, kmod, q, never, deps, None, 0, NC, hook)

    def v_tiles(b, c, lg, never, deps):
        blks = []
        for kt in range(CP // 128):
            t = v_s[b, lg, pl.ds(c * CP // 2 + kt * 64, 64), :]
            dd = deps[kt]
            if dd:
                pieces = [t[8 * j:8 * j + 8] for j in range(8)]
                for j, d in enumerate(dd):
                    jj = 7 - j if FIRST else j
                    pieces[jj] = jnp.where(never, pltpu.bitcast(d, U32), pieces[jj])
                t = _cat(pieces, axis=0)
            blks.append(t)
        return _upk(_cat(blks, axis=0))

    def stage_p(k, kmod, never, deps, hook=None, thr=0, lshook=None):
        b, _ = split(k)
        m = mx_s[kmod]
        neverr = _cat([never] * (R // 8), axis=0)
        NCP_ = TP // CP
        TPC = CP // 128
        ls = None
        pbs, pvs, accs = [], [], []
        for lg in range(NLG):
            acc = None
            for c in range(NCP_):
                gc = lg * NCP_ + c
                if lg == 0:
                    ps = []
                    if thr and c >= thr and (c % THS == 0):
                        m = jnp.where(neverr, pvs[c - thr], m)
                    for l in range(TPC):
                        p = jnp.exp2(s_s[kmod, :, pl.ds(c * CP + l * 128, 128)] - m)
                        ps.append(p)
                    if LSUM:
                        t = (ps[0] + ps[1]) + (ps[2] + ps[3])
                        ls = t if ls is None else ls + t
                    else:
                        for p in ps:
                            ls = p if ls is None else ls + p
                    pbs.append(_cat(ps).astype(BF16))
                    if lshook is not None:
                        lshook(c, ls)
                pv = _dot(pbs[c], v_tiles(b, c, lg, never, deps[gc * TPC:(gc + 1) * TPC]))
                if hook is not None:
                    hook(gc, pv)
                pvs.append(pv)
                acc = pv if acc is None else acc + pv
            accs.append(acc)
        acc = _cat(accs)
        l = jnp.sum(ls, axis=-1, keepdims=True)
        rinv = 1.0 / l
        glob = acc * rinv
        for lg in range(NLG):
            halo_store(m_s, k, kmod, lg, glob[:, lg * 128:(lg + 1) * 128])
        return vregs(bc(rinv)), vregs(glob)

    NTILE = (TP // 128) * NLG

    def place(slots, items, lo, hi, grp=1):
        ng = -(-len(items) // grp)
        for j, it in enumerate(items):
            pos = lo + (((j // grp) * 2 + 1) * (hi - lo)) // (2 * ng) if grp > 1 else lo + (j * (hi - lo)) // len(items)
            while len(slots[pos]) >= 8:
                pos += 1
            slots[pos].append(it)

    def micro(n, pos):
        nmod = pos % U
        ok = lambda k: (not isinstance(k, int)) or 0 <= k < NKT
        never = z_s[...] != 0
        NV = R // 8
        TPC = NTILE // NC
        hasp, hasq = ok(n + 2), ok(n + 3)
        lo = 0 if hasp else NTILE
        hi = 2 * NTILE if hasq else NTILE
        res = {}
        jobs = []
        def chain_jobs(name, ring, nlg, w_ref, fin):
            out = []
            for lg in range(nlg):
                for j0 in range(0, NH, JG):
                    nj = min(JG, NH - j0)
                    for q in range(3):
                        def fn(rel, lg=lg, q=q, j0=j0, nj=nj):
                            init = None if q == 0 else _cat(res[name, lg, 0, j0], axis=0)
                            y = _ffa_chain(ring, lg, q, j0, nj, w_ref, never, rel, init)
                            if q > 0:
                                y = fin(lg, q - 1, j0, nj, y)
                            return [y[8 * i:8 * i + 8] for i in range(nj)]
                        out.append(((name, lg, q, j0), fn))
            return out

        if ok(n):
            jobs += chain_jobs('c2', m_s[nmod], 2 * NLG, dwm_s, lambda lg, par, j0, nj, y: y)
        if ok(n + 2):
            km = (nmod + 2) % U
            j1 = chain_jobs('c1', g_s[km], NLG, dwc_s, lambda lg, par, j0, nj, y: y * u_s[km, pl.ds(par * H + 8 * j0, 8 * nj), pl.ds(lg * 128, 128)])
            jobs = j1 + jobs if CORD else jobs + j1

        def gather2(name, nlg):
            return [_cat([v for q in (1, 2) for j0 in range(0, NH, JG) for v in res[name, lg, q, j0]], axis=0) for lg in range(nlg)]

        if hasp and hasq:
            npv = (NPVF * len(jobs)) // 100
        elif hasp:
            npv = len(jobs)
        else:
            npv = 0
        pv0 = PV0 if hasq else PVL
        dls = [pv0 + (j * (NTILE - pv0)) // max(npv, 1) for j in range(npv)]
        nq = len(jobs) - npv
        dls += [NTILE + QK0 + (j * (NTILE - QK0)) // nq if hasq else None for j in range(nq)]
        slots = [[] for _ in range(2 * NTILE)]
        pending = {}

        def addslot(dl, vals):
            for v in vals:
                while len(slots[dl]) >= 8:
                    dl += 1
                slots[dl].append(v)

        for (key, fn), dl in zip(jobs, dls):
            rc = None if dl is None else dl // TPC - WIN
            if rc is None or rc < lo // TPC or not WIN:
                res[key] = fn(None)
                if dl is not None:
                    addslot(dl, res[key])
            else:
                pending.setdefault(rc, []).append((key, fn, dl))

        def hook(gc, val):
            for j, (key, fn, dl) in enumerate(pending.pop(gc, [])):
                res[key] = fn(val[8 * (j % NV):8 * (j % NV) + 8, :128])
                addslot(dl, res[key])

        def put(items, a, b, grp=1):
            a, b = max(a, lo), min(b, hi)
            if items and b > a:
                place(slots, items, a, b, grp)

        if hasq:
            q = q_proj(n + 3)
        if ok(n + 4):
            uu, hh, mu, rs, gg = stage_a2(n + 4, (nmod + 4) % U)
            if A2A and pos >= UN - A2L:
                off = 0 if hasp else NTILE
                if UA1 > UA0:
                    put(uu, off + UA0, off + UA1)
                put(hh, off + HA0, off + HA0 + AW)
                if A2A == 1:
                    put(mu, off + HA0 + AD, off + HA0 + AD + AW)
                    put(rs, off + HA0 + 2 * AD, off + HA0 + 2 * AD + AW)
                    put(gg, off + HA0 + 2 * AD + 4, off + HA0 + 2 * AD + 4 + AW)
        if hasp:
            def lshook(c, ls):
                if LSP and (c + 1) % LSP == 0:
                    a = (c + 1 + LSD) * TPC
                    put(vregs(ls), a, a + LSW)
            ri, gl = stage_p(n + 2, (nmod + 2) % U, never, slots[:NTILE], hook, THR if (pos >= UN - THL) else 0, lshook)
            if hasq and GLA and pos >= UN - A2L:
                put(ri, NTILE + GL0, NTILE + GL0 + GW)
                put(gl, NTILE + GL0 + 4, NTILE + GL0 + 4 + GW)
        if hasq:
            stage_q(n + 3, (nmod + 3) % U, q, never, slots[NTILE:], hook)
        assert not pending
        tail = []
        if ok(n):
            tail.append(lambda: c2_mm(n, pos, gather2('c2', 2 * NLG)))
        if ok(n + 2):
            tail.append(lambda: c1_mm(n + 2, (nmod + 2) % U, gather2('c1', NLG)))
        if MORD == 1 or (MORD == 2 and pos == UN - 1):
            tail = tail[::-1]
        for f in tail:
            f()

    @pl.when(step == 0)
    @jax.named_scope("prologue")
    def _():
        if ONLY:
            return
        nt1 = T // TA
        xgroups = XG
        cw = [pltpu.make_async_copy(src, dst, sems.at[j]) for j, (src, dst) in enumerate(
            [(wqkv_hbm, wqkv_ref), (wao_hbm, wao_ref), (wmi_hbm, wmi_ref), (wmo_hbm, wmo_ref), (wm_hbm, wm_ref)])]
        cx = [pltpu.make_async_copy(x_hbm.at[b, pl.ds(t0 * TA, (t1 - t0) * TA), :],
                                    x_ref.at[b, pl.ds(t0 * TA, (t1 - t0) * TA), :], sems.at[5 + j])
              for j, (b, t0, t1) in enumerate(xgroups)]
        dmas = {'w%d' % j: c for j, c in enumerate(cw)}
        dmas.update({'x%d' % j: c for j, c in enumerate(cx)})
        for name in DORD:
            dmas[name].start()
        z_s[...] = jnp.zeros(z_s.shape, z_s.dtype)
        for src, dst, nlg, centre in ((dwc_ref, dwc_s, NLG, 0.0), (dwm_ref, dwm_s, 2 * NLG, 1.0)):
            for lg in range(nlg):
                wl = src[:, pl.ds(lg * 128, 128)].astype(F32)
                w = [wl[i:i + 1] for i in range(K)]
                if centre:
                    w[K // 2] = w[K // 2] + centre
                wa, wb = w[1::2], w[0::2]
                ws = [wa[i] + wb[i] if i < len(wa) else wb[i] for i in range(len(wb))]
                for q, ww in enumerate((ws, wb, wa)):
                    for i, wi in enumerate(ww):
                        dst[lg, pl.ds(8 * (16 * q + i), 8), :] = jnp.broadcast_to(wi, (8, 128))
        for b in range(B):
            for lg in range(NLG):
                xa_b[b, lg, pl.ds(T, TP - T), :] = jnp.zeros((TP - T, 128), BF16)
                v_b[b, lg, pl.ds(T, TP - T), :] = jnp.zeros((TP - T, 128), BF16)
        for q in range(3):
            for lg in range(NLG):
                seq_put(g_s[0], q, lg, 0, jnp.zeros((8, 128), F32))
            for lg in range(2 * NLG):
                seq_put(m_s[0], q, lg, 0, jnp.zeros((8, 128), F32))
        nodeps = [[] for _ in range(NTILE)]

        qs, mxs = {}, {0: None, 1: None, 2: None}

        def fold():
            wq = wqkv_ref[:, 0:D]
            wk = wqkv_ref[:, D:2 * D]
            wv = wqkv_ref[:, 2 * D:3 * D]
            wvo_s[...] = _pk(_dot(wv, wao_ref[...]).astype(BF16))
            wqk_s[...] = _pk((_dot_nt(wq, wk) * (D ** -0.5 * LOG2E)).astype(BF16))

        def jq(k):
            qs[k] = q_proj(k)

        def jc(ca, cb):
            for k in range(3):
                mxs[k] = q_chunks(k, k % U, qs[k], None, nodeps, mxs[k], ca, cb)

        def jp(k):
            never = z_s[...] != 0
            res = {('c1', lg, j): c1_job(k % U, lg, j, None, None) for lg in range(NLG) for j in range(NH)}
            deps = [[] for _ in range(NTILE)]
            place(deps, [v for key in res for v in res[key]], NTILE // 2, NTILE)
            stage_p(k, k % U, never, deps)
            c1_mm(k, k % U, gather(res, 'c1', NLG))

        for tok in PLAN.split():
            op, arg = tok[0], tok[1:]
            if op == '!':
                dmas[arg].wait()
            elif op == 'W':
                src, dst = {'2': (wmi_ref, wmi_s), '3': (wmo_ref, wmo_s), '4': (wm_ref, wm_s)}[arg]
                dst[...] = _pk(src[...])
            elif op == 'F':
                fold()
            elif op == 'L':
                ln_tile(int(arg) // nt1, int(arg) % nt1)
            elif op == 'V':
                v_tile(int(arg) // nt1, int(arg) % nt1)
            elif op == 'Q':
                jq(int(arg))
            elif op == 'A':
                stage_a2(int(arg), int(arg) % U)
            elif op == 'C':
                ca, cb = arg.split('-')
                jc(int(ca), int(cb))
            elif op == 'P':
                jp(int(arg))
            else:
                raise ValueError(tok)

    @pl.when(step < NS - 1)
    @jax.named_scope("steady")
    def _():
        if ONLYP:
            return
        for i in range(UN):
            micro(step * UN + i, i)

    @pl.when(step == NS - 1)
    @jax.named_scope("last")
    def _():
        if ONLY or ONLYP:
            return
        for i in range(UN):
            micro((NS - 1) * UN + i, i)


@jax.jit
def pallas_standalone__conformer_family_e_branchformer__speech_kernel(
    x, w_qkv, w_att_out, w_mlp_in, dw_csgu, w_mlp_out, dw_merge, w_merge,
):
    B, T, D = x.shape
    K = dw_csgu.shape[0]
    R = 80
    U = 5
    TP = 4096
    NSB = T // (R * UN)
    TH = -(-(R + 2 * PADR) // 32) * 32
    full = lambda a: pl.BlockSpec(a.shape, lambda s: (0,) * a.ndim)

    hbm = pl.BlockSpec(memory_space=pl.ANY)
    kern = functools.partial(_kernel, B=B, T=T, D=D, K=K, R=R, U=U, TP=TP)
    return pl.pallas_call(
        kern,
        grid=(B * NSB,),
        in_specs=[hbm, hbm, hbm, hbm, full(dw_csgu), hbm, full(dw_merge), hbm],
        out_specs=pl.BlockSpec((R * UN, D), lambda s: (s, 0)),
        out_shape=jax.ShapeDtypeStruct((B * T, D), x.dtype),
        scratch_shapes=[
            pltpu.VMEM(x.shape, BF16),
            pltpu.VMEM(w_qkv.shape, BF16),
            pltpu.VMEM(w_att_out.shape, BF16),
            pltpu.VMEM(w_mlp_in.shape, BF16),
            pltpu.VMEM(w_mlp_out.shape, BF16),
            pltpu.VMEM(w_merge.shape, BF16),
            pltpu.SemaphoreType.DMA((5 + len(XG),)),
            pltpu.VMEM((D // 2, D), U32),
            pltpu.VMEM((D // 2, D), U32),
            pltpu.VMEM((D // 2, 2 * D), U32),
            pltpu.VMEM((D // 2, D), U32),
            pltpu.VMEM((D, D), U32),
            pltpu.VMEM((D // 128, 384, 128), F32),
            pltpu.VMEM((2 * D // 128, 384, 128), F32),
            pltpu.VMEM((B, D // 128, TP, 128), BF16),
            pltpu.VMEM((B, D // 128, TP, 128), BF16),
            pltpu.VMEM((U, R, D), F32),
            pltpu.VMEM((U, R, TP), F32),
            pltpu.VMEM((U, R, 128), F32),
            pltpu.VMEM((8, 128), jnp.int32),
        ] + [pltpu.VMEM((D // 128, 7, RR, 128), F32)] * U + [pltpu.VMEM((2 * D // 128, 7, RR, 128), F32)] * U,
        compiler_params=pltpu.CompilerParams(
            dimension_semantics=("arbitrary",),
            vmem_limit_bytes=100 * 1024 * 1024,
        ),
    )(x, w_qkv, w_att_out, w_mlp_in, dw_csgu, w_mlp_out, dw_merge, w_merge).reshape(B, T, D)
```

```python
import functools
import math

import jax
import jax.numpy as jnp
from jax import lax
import jax.experimental.pallas as pl
import jax.experimental.pallas.tpu as pltpu

F32 = jnp.float32
BF16 = jnp.bfloat16
U32 = jnp.uint32
EPS = 1e-5
LOG2E = 1.4426950408889634
PADR = 16
CK = 256
NPV = 6
NACC = 2
ACCB = 0
FIRST = 1
E = lambda k, d: int(d)
PV0, A2A, UA0, UA1, GA0, GA1 = E('PV0', 40), E('A2A', 1), E('UA0', 16), E('UA1', 54), E('GA0', 30), E('GA1', 50)
GLA, GL0, GW = E('GLA', 0), E('GL0', 12), E('GW', 10)
PO = [int(c) for c in '12133']
ZS = E('ZS', 0)
DS0, DS1 = E('DS0', 9), E('DS1', 9)
UN = E('UN', 12)
UR = E('UR', 6)
WIN, ZW, THL = E('WIN', 5), E('ZW', 0), E('THL', 1)
A2L = E('A2L', 99)
ZM = E('ZM', 64)
NCP = E('NCP', 1)
ONLY = E('ONLY', 0)
RR = E('RR', 72)
JG = E('JG', 5)
ONLYP = E('ONLYP', 0)
DEC = E('DEC', 1)
MORD = E('MORD', 1)
PLANS = {
 1: ([(0, 0, 2), (0, 2, 4), (0, 4, 6), (0, 6, 10), (1, 0, 5), (1, 5, 10)],
     'x0 w5 w6 w0 w1 x1 w2 x2 x3 w3 w4 x4 x5',
     '!x0 L0 L1 '
     '!w5 !w6 !w0 !w1 D F V0 V1 Q0 Q1 Q2 C0-3 '
     '!x1 !w2 !x2 W2 L2 A0 A1 L3 A2 A3 L4 L5 V2 V3 V4 '
     '!x3 L6 V5 C3-5 L7 C5-7 L8 C7-9 L9 V6 V7 V8 '
     '!w3 !w4 !x4 W3 W4 V9 L10 C9-12 L11 C12-14 L12 C14-16 L13 L14 V10 V11 V12 V13 '
     '!x5 V14 L15 P0 L16 V15 L17 V16 P1 L18 V17 L19 V18 V19'),
 7: ([(0, 0, 1), (0, 1, 4), (0, 4, 6), (0, 6, 10), (1, 0, 5), (1, 5, 10)],
     'x0 w2 w5 w6 w0 w1 x1 x2 x3 w3 w4 x4 x5',
     '!x0 !w2 !w5 !w6 L0 W2 D A0 A1 A2 A3 '
     '!w0 !w1 F V0 Q0 Q1 Q2 C0-1 '
     '!x1 !x2 L1 L2 V1 L3 C1-3 V2 L4 C3-4 L5 V3 C4-6 V4 '
     '!x3 L6 V5 C6-8 L7 C8-9 L8 V6 L9 V7 V8 '
     '!w3 !w4 !x4 W3 W4 V9 L10 C9-12 L11 C12-14 L12 C14-16 L13 L14 V10 V11 V12 V13 '
     '!x5 V14 L15 P0 L16 V15 L17 V16 P1 L18 V17 L19 V18 V19'),
 8: ([(0, 0, 2), (0, 2, 6), (0, 6, 10), (1, 0, 5), (1, 5, 10)],
     'x0 w2 w5 w6 w0 w1 x1 x2 w3 w4 x3 x4',
     '!x0 !w2 !w5 !w6 L0 W2 D L1 A0 A1 A2 A3 '
     '!w0 !w1 F V0 V1 Q0 Q1 Q2 C0-3 '
     '!x1 L2 L3 V2 L4 V3 C3-6 L5 V4 '
     '!x2 L6 V5 C6-8 L7 C8-9 L8 V6 L9 V7 V8 '
     '!w3 !w4 !x3 W3 W4 V9 L10 C9-12 L11 C12-14 L12 C14-16 L13 L14 V10 V11 V12 V13 '
     '!x4 V14 L15 P0 L16 V15 L17 V16 P1 L18 V17 L19 V18 V19'),
 9: ([(0, 0, 2), (0, 2, 4), (0, 4, 6), (0, 6, 10), (1, 0, 4), (1, 4, 10)],
     'x0 w5 w6 w0 w1 x1 w2 x2 x3 x4 w3 w4 x5',
     '!x0 L0 L1 '
     '!w5 !w6 !w0 !w1 D F V0 V1 Q0 Q1 Q2 C0-3 '
     '!x1 !w2 !x2 W2 L2 A0 A1 L3 A2 A3 L4 L5 V2 V3 V4 '
     '!x3 !x4 L6 V5 C3-5 L7 C5-7 L8 C7-9 L9 V6 V7 L10 V8 V9 L11 C9-12 L12 C12-14 L13 C14-16 V10 V11 V12 '
     '!w3 !w4 !x5 W3 W4 V13 L14 P0 L15 V14 L16 V15 L17 V16 P1 L18 V17 L19 V18 V19'),
 10: ([(0, 0, 2), (0, 2, 4), (0, 4, 6), (0, 6, 10), (1, 0, 5), (1, 5, 10)],
     'x0 w5 w6 w0 w1 x1 w2 x2 x3 w3 w4 x4 x5',
     '!x0 L0 L1 '
     '!w5 !w6 !w0 !w1 D F V0 V1 Q0 Q1 Q2 C0-2 '
     '!x1 !w2 !x2 W2 C2-3 L2 A0 A1 L3 A2 A3 L4 L5 V2 V3 '
     '!x3 V4 L6 V5 C3-5 L7 C5-7 L8 C7-9 L9 V6 V7 '
     '!w3 !w4 !x4 W3 W4 V8 V9 L10 C9-12 L11 C12-14 L12 C14-16 L13 L14 V10 V11 V12 '
     '!x5 V13 V14 L15 P0 L16 L17 V15 V16 P1 L18 V17 L19 V18 V19'),
}
XG, DORD, PLAN = PLANS[E('PL', 1)]
DORD = DORD.split()
NPVF = E('NPVF', 28)
TORD = E('TORD', 1)
PVL = E('PVL', 0)
CP = 512
LSP, LSD, LSW = E('LSP', 0), E('LSD', 1), E('LSW', 8)
WBC = E('WBC', 1)
PSPLIT, LSUM = E('PSPLIT', 0), E('LSUM', 0)
THR, THS, GRP = E('THR', 3), E('THS', 1), E('GRP', 1)
HA0, AW, AD, QK0, CORD = E('HA0', 36), E('AW', 20), E('AD', 8), E('QK0', 12), E('CORD', 0)
ANCH = 1


def _ln(x):
    m = jnp.mean(x, axis=-1, keepdims=True)
    xc = x - m
    v = jnp.mean(xc * xc, axis=-1, keepdims=True)
    return xc * lax.rsqrt(v + EPS)


def _ln_mxu_var(x):
    d = x.shape[-1]
    m = jnp.mean(x, axis=-1, keepdims=True)
    xc = x - m
    sq = xc * xc
    q = sq[:, :128]
    for l in range(1, d // 128):
        q = q + sq[:, l * 128:(l + 1) * 128]
    v = jnp.dot(q.astype(BF16), jnp.ones((128, 128), BF16), preferred_element_type=F32) * (1.0 / d)
    r = lax.rsqrt(v + EPS)
    return xc * jnp.concatenate([r] * (d // 128), axis=-1)


def _gelu(x):
    c = math.sqrt(2.0 / math.pi)
    return 0.5 * x * (1.0 + jnp.tanh(c * (x + 0.044715 * (x * x * x))))


def _dot(a, b):
    return jnp.dot(a, b, preferred_element_type=F32)


def _dot_nt(a, b):
    return lax.dot_general(a, b, (((1,), (1,)), ((), ())), preferred_element_type=F32)


def _cat(parts, axis=-1):
    return jnp.concatenate(parts, axis=axis)


def _pk(x):
    return pltpu.bitcast(x, U32)


def _upk(x):
    return pltpu.bitcast(x, BF16)


def _even_odd(xb):
    xu = _pk(xb)
    return pltpu.bitcast(xu << 16, F32), pltpu.bitcast(xu & jnp.uint32(0xFFFF0000), F32)


def _interleave_bf16(e, o):
    rb = lambda a: pltpu.bitcast(a.astype(BF16).astype(F32), U32)
    return _upk((rb(e) >> 16) | (rb(o) & jnp.uint32(0xFFFF0000)))


def _ffa_pair(ring, lg, j, w_ref, never, rel):
    outs = []
    for q, nt in enumerate((16, 16, 15)):
        acc = None
        ks = list(range(nt))
        if TORD == 1:
            ks = [k for pair in zip(range(8), range(8, 16)) for k in pair if k < nt]
        for k in ks:
            o = k + 1
            win = ring[lg, 2 * q + ((o // 8) % 2 if NCP > 1 else 0), pl.ds(8 * j + o, 8), :]
            w = w_ref[lg, pl.ds(8 * (16 * q + k), 8), :]
            if acc is None:
                if rel is not None:
                    win = jnp.where(never, rel, win)
                acc = win * w
            else:
                acc = acc + win * w
        outs.append(acc)
    return outs[0] + outs[1], outs[0] + outs[2]


def _ffa_chain(ring, lg, q, j0, nj, w_ref, never, rel, init):
    nt = (16, 16, 15)[q]
    acc = init
    ks = list(range(nt))
    if TORD == 1:
        ks = [k for pair in zip(range(8), range(8, 16)) for k in pair if k < nt]
    for n_, k in enumerate(ks):
        o = k + 1
        win = ring[lg, 2 * q + ((o // 8) % 2 if NCP > 1 else 0), pl.ds(8 * j0 + o, 8 * nj), :]
        w = w_ref[lg, pl.ds(8 * (16 * q + k), 8), :]
        if n_ == 0 and rel is not None:
            w = jnp.where(never, rel, w)
        w = _cat([w] * nj, axis=0)
        acc = win * w if acc is None else acc + win * w
    return acc


def _kernel(x_hbm, wqkv_hbm, wao_hbm, wmi_hbm, dwc_hbm, wmo_hbm, dwm_hbm, wm_hbm, o_ref,
            x_ref, wqkv_ref, wao_ref, wmi_ref, wmo_ref, wm_ref, dwc_ref, dwm_ref, sems,
            wqk_s, wvo_s, wmi_s, wmo_s, wm_s, dwc_s, dwm_s, xa_s, v_s, u_s, s_s, mx_s, z_s, *rings,
            B, T, D, K, R, U, TP):
    g_s, m_s = rings[:U], rings[U:]
    xa_b, v_b = xa_s, v_s
    xa_s, v_s = xa_b.bitcast(U32), v_b.bitcast(U32)
    step = pl.program_id(0)
    NK = T // R
    NKT = B * NK
    NS = -(-NKT // UN)
    assert (NS - 1) * UN <= NKT - 4 and UN % U == 0
    NLG = D // 128
    TA = 400
    NC = TP // CK

    def split(k):
        if isinstance(k, int):
            return k // NK, k % NK
        b = sum((k >= j * NK).astype(jnp.int32) for j in range(1, B))
        return b, k - b * NK

    def rows(i, n):
        r = i * n
        return pl.ds(r if isinstance(r, int) else pl.multiple_of(r, 8), n)

    H = R // 2
    NH = H // 8

    def seq_put(ref, q, lg, r0, val):
        n = val.shape[0]
        if NCP == 1:
            ref[lg, 2 * q, pl.ds(r0, n), :] = val
            return
        if not (q == 2 and r0 >= 8 + H):
            ref[lg, 2 * q, pl.ds(r0, n), :] = val
        if r0 >= 8:
            ref[lg, 2 * q + 1, pl.ds(r0, n), :] = val

    def halo_store(ref, k, kmod, lg, val):
        cur, prv, nxt = ref[kmod % U], ref[(kmod - 1) % U], ref[(kmod + 1) % U]
        xe, xo = val[:H], val[H:]
        row0 = lax.broadcasted_iota(jnp.int32, (8, 128), 0) == 0
        rot = [pltpu.roll(xo[8 * i:8 * i + 8], 1, 0) for i in range(NH)]
        nxt[lg, 6, pl.ds(0, 8), :] = rot[-1]
        rot = [cur[lg, 6, pl.ds(0, 8), :]] + rot
        sh = _cat([jnp.where(row0, rot[i], rot[i + 1]) for i in range(NH)], axis=0)
        zero = jnp.zeros((8, 128), F32)
        if isinstance(k, int):
            first, last = k % NK == 0, k % NK == NK - 1
        else:
            first = (split(k)[1] == 0) if any((j * NK) % UN == kmod for j in range(B)) else False
            last = (split(k)[1] == NK - 1) if any((j * NK - 1) % UN == kmod for j in range(1, B + 1)) else False
        sh0 = sh[:8]
        if first is not False:
            cut = row0 if first is True else jnp.logical_and(row0, first)
            sh = _cat([jnp.where(cut, 0.0, sh0), sh[8:]], axis=0)
        seqs = [xe, sh - xe, xo - xe]
        for q, v in enumerate(seqs):
            seq_put(cur, q, lg, 8, v)
            top, bot = v[:8], v[H - 8:]
            if first is not False:
                edge = jnp.where(row0, sh0, 0.0) if q == 1 else zero
                top = None if (first is True and k == 0) else (edge if first is True else jnp.where(first, edge, top))
            if last is not False:
                bot = zero if last is True else jnp.where(last, 0.0, bot)
            if top is not None:
                seq_put(prv, q, lg, 8 + H, top)
            seq_put(nxt, q, lg, 0, bot)

    def tail_store(ref, nlg):
        row0 = lax.broadcasted_iota(jnp.int32, (8, 128), 0) == 0
        for lg in range(nlg):
            e = ref[NKT % U][lg, 6, pl.ds(0, 8), :]
            for q in range(3):
                seq_put(ref[(NKT - 1) % U], q, lg, 8 + H, jnp.where(row0, e, 0.0) if q == 1 else jnp.zeros((8, 128), F32))

    def vregs(a):
        return [a[8 * r:8 * r + 8, l * 128:(l + 1) * 128] for r in range(a.shape[0] // 8) for l in range(a.shape[1] // 128)]

    def xa_rows(b, r):
        return _upk(_cat([xa_s[b, lg, r, :] for lg in range(NLG)]))

    def ln_tile(b, t):
        eo = _even_odd(x_ref[b, pl.ds(t * TA, TA), :])
        xa = _ln(_cat([eo[par][i * H:(i + 1) * H] for i in range(TA // R) for par in range(2)], axis=0))
        for lg in range(NLG):
            xa_b[b, lg, pl.ds(t * TA, TA), :] = xa[:, lg * 128:(lg + 1) * 128].astype(BF16)

    def v_tile(b, t):
        v = _dot(xa_rows(b, rows(t, TA // 2)), _upk(wvo_s[...]))
        for lg in range(NLG):
            v_b[b, lg, pl.ds(t * TA, TA), :] = v[:, lg * 128:(lg + 1) * 128].astype(BF16)

    def stage_a1(b, t):
        ln_tile(b, t)
        v_tile(b, t)

    def bc(a):
        return jnp.broadcast_to(a, (a.shape[0], 128))

    def stage_a2(k, kmod):
        b, i = split(k)
        h = _gelu(_dot(xa_rows(b, rows(i, R // 2)), _upk(wmi_s[...])))
        u_s[kmod % U] = h[:, :D]
        hg = h[:, D:]
        mu = jnp.mean(hg, axis=-1, keepdims=True)
        xc = hg - mu
        rs = lax.rsqrt(jnp.mean(xc * xc, axis=-1, keepdims=True) + EPS)
        g = xc * rs
        for lg in range(NLG):
            halo_store(g_s, k, kmod, lg, g[:, lg * 128:(lg + 1) * 128])
        return vregs(h[:, :D]), vregs(hg), vregs(bc(mu)), vregs(bc(rs)), vregs(g)

    def c1_job(km, lg, j, never, rel):
        ye, yo = _ffa_pair(g_s[km], lg, j, dwc_s, never, rel)
        lanes = pl.ds(lg * 128, 128)
        return u_s[km, pl.ds(8 * j, 8), lanes] * ye, u_s[km, pl.ds(H + 8 * j, 8), lanes] * yo

    def gather(res, name, nlg):
        return [_cat([res[name, lg, j][0] for j in range(NH)] + [res[name, lg, j][1] for j in range(NH)], axis=0)
                for lg in range(nlg)]

    def c1_mm(k, kmod, parts):
        loc = _dot(_cat(parts).astype(BF16), _upk(wmo_s[...]))
        for lg in range(NLG):
            halo_store(m_s, k, kmod, NLG + lg, loc[:, lg * 128:(lg + 1) * 128])

    def c2_mm(k, pos, parts):
        b, i = split(k)
        r0 = i * R
        r0 = r0 if isinstance(r0, int) else pl.multiple_of(r0, 16)
        y = _dot(_cat(parts).astype(BF16), _upk(wm_s[...]))
        xe, xo = _even_odd(x_ref[b, pl.ds(r0, R), :])
        o_ref[pl.ds(pos * R, R), :] = _interleave_bf16(y[:H] + xe, y[H:] + xo)

    def q_proj(k):
        b, i = split(k)
        return _dot(xa_rows(b, rows(i, R // 2)), _upk(wqk_s[...])).astype(BF16)

    def kv_chunk(ref, b, c, never, deps):
        blks = []
        for kt in range(CK // 128):
            parts = []
            for lg in range(NLG):
                t = ref[b, lg, pl.ds(c * CK // 2 + kt * 64, 64), :]
                dd = deps[(c * (CK // 128) + kt) * NLG + lg]
                if dd:
                    pieces = [t[8 * j:8 * j + 8] for j in range(8)]
                    for j, d in enumerate(dd):
                        jj = 7 - j if FIRST else j
                        pieces[jj] = jnp.where(never, pltpu.bitcast(d, U32), pieces[jj])
                    t = _cat(pieces, axis=0)
                parts.append(t)
            blks.append(_cat(parts))
        return _upk(_cat(blks, axis=0))

    def q_chunks(k, kmod, q, never, deps, mx, ca, cb, hook=None):
        b, _ = split(k)
        for c in range(ca, cb):
            s = _dot_nt(q, kv_chunk(xa_s, b, c, never, deps))
            if hook is not None:
                hook(NC + c, s)
            for l in range(CK // 128):
                sl = s[:, l * 128:(l + 1) * 128]
                c0 = c * CK + l * 128
                if c0 + 128 > T:
                    col = lax.broadcasted_iota(jnp.int32, (R, 128), 1) + c0
                    sl = jnp.where(col < T, sl, -jnp.inf)
                s_s[kmod % U, :, pl.ds(c0, 128)] = sl
                mx = sl if mx is None else jnp.maximum(mx, sl)
        if cb == NC:
            mx_s[kmod % U] = jnp.broadcast_to(jnp.max(mx, axis=-1, keepdims=True), (R, 128))
        return mx

    def stage_q(k, kmod, q, never, deps, hook=None):
        q_chunks(k, kmod, q, never, deps, None, 0, NC, hook)

    def v_tiles(b, c, lg, never, deps):
        blks = []
        for kt in range(CP // 128):
            t = v_s[b, lg, pl.ds(c * CP // 2 + kt * 64, 64), :]
            dd = deps[kt]
            if dd:
                pieces = [t[8 * j:8 * j + 8] for j in range(8)]
                for j, d in enumerate(dd):
                    jj = 7 - j if FIRST else j
                    pieces[jj] = jnp.where(never, pltpu.bitcast(d, U32), pieces[jj])
                t = _cat(pieces, axis=0)
            blks.append(t)
        return _upk(_cat(blks, axis=0))

    def stage_p(k, kmod, never, deps, hook=None, thr=0, lshook=None):
        b, _ = split(k)
        m = mx_s[kmod % U]
        neverr = _cat([never] * (R // 8), axis=0)
        NCP_ = TP // CP
        TPC = CP // 128
        ls = None
        pbs, pvs, accs = [], [], []
        for lg in range(NLG):
            acc = None
            for c in range(NCP_):
                gc = lg * NCP_ + c
                if lg == 0:
                    ps = []
                    if thr and c >= thr and (c % THS == 0):
                        m = jnp.where(neverr, pvs[c - thr], m)
                    for l in range(TPC):
                        p = jnp.exp2(s_s[kmod % U, :, pl.ds(c * CP + l * 128, 128)] - m)
                        ps.append(p)
                    if LSUM:
                        t = (ps[0] + ps[1]) + (ps[2] + ps[3])
                        ls = t if ls is None else ls + t
                    else:
                        for p in ps:
                            ls = p if ls is None else ls + p
                    pbs.append(_cat(ps).astype(BF16))
                    if lshook is not None:
                        lshook(c, ls)
                pv = _dot(pbs[c], v_tiles(b, c, lg, never, deps[gc * TPC:(gc + 1) * TPC]))
                if hook is not None:
                    hook(gc, pv)
                pvs.append(pv)
                acc = pv if acc is None else acc + pv
            accs.append(acc)
        acc = _cat(accs)
        l = jnp.sum(ls, axis=-1, keepdims=True)
        rinv = 1.0 / l
        glob = acc * rinv
        for lg in range(NLG):
            halo_store(m_s, k, kmod, lg, glob[:, lg * 128:(lg + 1) * 128])
        return vregs(bc(rinv)), vregs(glob)

    NTILE = (TP // 128) * NLG

    def place(slots, items, lo, hi, grp=1):
        ng = -(-len(items) // grp)
        for j, it in enumerate(items):
            pos = lo + (((j // grp) * 2 + 1) * (hi - lo)) // (2 * ng) if grp > 1 else lo + (j * (hi - lo)) // len(items)
            while len(slots[pos]) >= 8:
                pos += 1
            slots[pos].append(it)

    def micro(n, pos):
        nmod = pos % U
        ok = lambda k: (not isinstance(k, int)) or 0 <= k < NKT
        never = z_s[...] != 0
        NV = R // 8
        TPC = NTILE // NC
        hasp, hasq = ok(n + 2), ok(n + 3)
        lo = 0 if hasp else NTILE
        hi = 2 * NTILE if hasq else NTILE
        res = {}
        jobs = []
        if isinstance(n, int) and n + 4 == NKT:
            tail_store(g_s, NLG)
        if isinstance(n, int) and n + 2 == NKT:
            tail_store(m_s, 2 * NLG)
        def chain_jobs(name, ring, nlg, w_ref, fin):
            out = []
            for lg in range(nlg):
                for j0 in range(0, NH, JG):
                    nj = min(JG, NH - j0)
                    for q in range(3):
                        def fn(rel, lg=lg, q=q, j0=j0, nj=nj):
                            init = None if q == 0 else _cat(res[name, lg, 0, j0], axis=0)
                            y = _ffa_chain(ring, lg, q, j0, nj, w_ref, never, rel, init)
                            if q > 0:
                                y = fin(lg, q - 1, j0, nj, y)
                            return [y[8 * i:8 * i + 8] for i in range(nj)]
                        out.append(((name, lg, q, j0), fn))
            return out

        if ok(n):
            jobs += chain_jobs('c2', m_s[nmod], 2 * NLG, dwm_s, lambda lg, par, j0, nj, y: y)
        if ok(n + 2):
            km = (nmod + 2) % U
            j1 = chain_jobs('c1', g_s[km], NLG, dwc_s, lambda lg, par, j0, nj, y: y * u_s[km, pl.ds(par * H + 8 * j0, 8 * nj), pl.ds(lg * 128, 128)])
            jobs = j1 + jobs if CORD else jobs + j1

        def gather2(name, nlg):
            return [_cat([v for q in (1, 2) for j0 in range(0, NH, JG) for v in res[name, lg, q, j0]], axis=0) for lg in range(nlg)]

        if hasp and hasq:
            npv = (NPVF * len(jobs)) // 100
        elif hasp:
            npv = len(jobs)
        else:
            npv = 0
        pv0 = PV0 if hasq else PVL
        dls = [pv0 + (j * (NTILE - pv0)) // max(npv, 1) for j in range(npv)]
        nq = len(jobs) - npv
        dls += [NTILE + QK0 + (j * (NTILE - QK0)) // nq if hasq else None for j in range(nq)]
        slots = [[] for _ in range(2 * NTILE)]
        pending = {}

        def addslot(dl, vals):
            for v in vals:
                while len(slots[dl]) >= 8:
                    dl += 1
                slots[dl].append(v)

        for (key, fn), dl in zip(jobs, dls):
            rc = None if dl is None else dl // TPC - WIN
            if rc is None or rc < lo // TPC or not WIN:
                res[key] = fn(None)
                if dl is not None:
                    addslot(dl, res[key])
            else:
                pending.setdefault(rc, []).append((key, fn, dl))

        def hook(gc, val):
            for j, (key, fn, dl) in enumerate(pending.pop(gc, [])):
                res[key] = fn(val[8 * (j % NV):8 * (j % NV) + 8, :128])
                addslot(dl, res[key])

        def put(items, a, b, grp=1):
            a, b = max(a, lo), min(b, hi)
            if items and b > a:
                place(slots, items, a, b, grp)

        if hasq:
            q = q_proj(n + 3)
        if ok(n + 4):
            uu, hh, mu, rs, gg = stage_a2(n + 4, (pos + 4) % UN)
            if A2A and pos >= UN - A2L:
                off = 0 if hasp else NTILE
                if UA1 > UA0:
                    put(uu, off + UA0, off + UA1)
                put(hh, off + HA0, off + HA0 + AW)
                if A2A == 1:
                    put(mu, off + HA0 + AD, off + HA0 + AD + AW)
                    put(rs, off + HA0 + 2 * AD, off + HA0 + 2 * AD + AW)
                    put(gg, off + HA0 + 2 * AD + 4, off + HA0 + 2 * AD + 4 + AW)
        if hasp:
            def lshook(c, ls):
                if LSP and (c + 1) % LSP == 0:
                    a = (c + 1 + LSD) * TPC
                    put(vregs(ls), a, a + LSW)
            ri, gl = stage_p(n + 2, (pos + 2) % UN, never, slots[:NTILE], hook, THR if (pos >= UN - THL) else 0, lshook)
            if hasq and GLA and pos >= UN - A2L:
                put(ri, NTILE + GL0, NTILE + GL0 + GW)
                put(gl, NTILE + GL0 + 4, NTILE + GL0 + 4 + GW)
        if hasq:
            stage_q(n + 3, (pos + 3) % UN, q, never, slots[NTILE:], hook)
        assert not pending
        tail = []
        if ok(n):
            tail.append(lambda: c2_mm(n, pos, gather2('c2', 2 * NLG)))
        if ok(n + 2):
            tail.append(lambda: c1_mm(n + 2, (pos + 2) % UN, gather2('c1', NLG)))
        if MORD == 1 or (MORD == 2 and pos == UN - 1):
            tail = tail[::-1]
        for f in tail:
            f()

    @pl.when(step == 0)
    @jax.named_scope("prologue")
    def _():
        if ONLY:
            return
        nt1 = T // TA
        xgroups = XG
        cw = [pltpu.make_async_copy(src, dst, sems.at[j]) for j, (src, dst) in enumerate(
            [(wqkv_hbm, wqkv_ref), (wao_hbm, wao_ref), (wmi_hbm, wmi_ref), (wmo_hbm, wmo_ref), (wm_hbm, wm_ref),
             (dwc_hbm, dwc_ref), (dwm_hbm, dwm_ref)])]
        cx = [pltpu.make_async_copy(x_hbm.at[b, pl.ds(t0 * TA, (t1 - t0) * TA), :],
                                    x_ref.at[b, pl.ds(t0 * TA, (t1 - t0) * TA), :], sems.at[7 + j])
              for j, (b, t0, t1) in enumerate(xgroups)]
        dmas = {'w%d' % j: c for j, c in enumerate(cw)}
        dmas.update({'x%d' % j: c for j, c in enumerate(cx)})
        for name in DORD:
            dmas[name].start()
        z_s[...] = jnp.zeros(z_s.shape, z_s.dtype)
        for b in range(B):
            for lg in range(NLG):
                xa_b[b, lg, pl.ds(T, TP - T), :] = jnp.zeros((TP - T, 128), BF16)
                v_b[b, lg, pl.ds(T, TP - T), :] = jnp.zeros((TP - T, 128), BF16)
        for ring, nlg in ((g_s, NLG), (m_s, 2 * NLG)):
            for lg in range(nlg):
                for q in range(3):
                    seq_put(ring[0], q, lg, 0, jnp.zeros((8, 128), F32))
                ring[0][lg, 6, pl.ds(0, 8), :] = jnp.zeros((8, 128), F32)
        nodeps = [[] for _ in range(NTILE)]

        qs, mxs = {}, {0: None, 1: None, 2: None}

        def fold():
            wq = wqkv_ref[:, 0:D]
            wk = wqkv_ref[:, D:2 * D]
            wv = wqkv_ref[:, 2 * D:3 * D]
            wvo_s[...] = _pk(_dot(wv, wao_ref[...]).astype(BF16))
            wqk_s[...] = _pk((_dot_nt(wq, wk) * (D ** -0.5 * LOG2E)).astype(BF16))

        def taps():
            for src, dst, nlg, centre in ((dwc_ref, dwc_s, NLG, 0.0), (dwm_ref, dwm_s, 2 * NLG, 1.0)):
                for lg in range(nlg):
                    wl = src[:, pl.ds(lg * 128, 128)].astype(F32)
                    w = [wl[i:i + 1] for i in range(K)]
                    if centre:
                        w[K // 2] = w[K // 2] + centre
                    wa, wb = w[1::2], w[0::2]
                    ws = [wa[i] + wb[i] if i < len(wa) else wb[i] for i in range(len(wb))]
                    for q, ww in enumerate((ws, wb, wa)):
                        for i, wi in enumerate(ww):
                            dst[lg, pl.ds(8 * (16 * q + i), 8), :] = jnp.broadcast_to(wi, (8, 128))

        def jq(k):
            qs[k] = q_proj(k)

        def jc(ca, cb):
            for k in range(3):
                mxs[k] = q_chunks(k, k % U, qs[k], None, nodeps, mxs[k], ca, cb)

        def jp(k):
            never = z_s[...] != 0
            res = {('c1', lg, j): c1_job(k % U, lg, j, None, None) for lg in range(NLG) for j in range(NH)}
            deps = [[] for _ in range(NTILE)]
            place(deps, [v for key in res for v in res[key]], NTILE // 2, NTILE)
            stage_p(k, k % U, never, deps)
            c1_mm(k, k % U, gather(res, 'c1', NLG))

        for tok in PLAN.split():
            op, arg = tok[0], tok[1:]
            if op == '!':
                dmas[arg].wait()
            elif op == 'W':
                src, dst = {'2': (wmi_ref, wmi_s), '3': (wmo_ref, wmo_s), '4': (wm_ref, wm_s)}[arg]
                dst[...] = _pk(src[...])
            elif op == 'D':
                taps()
            elif op == 'F':
                fold()
            elif op == 'L':
                ln_tile(int(arg) // nt1, int(arg) % nt1)
            elif op == 'V':
                v_tile(int(arg) // nt1, int(arg) % nt1)
            elif op == 'Q':
                jq(int(arg))
            elif op == 'A':
                stage_a2(int(arg), int(arg) % U)
            elif op == 'C':
                ca, cb = arg.split('-')
                jc(int(ca), int(cb))
            elif op == 'P':
                jp(int(arg))
            else:
                raise ValueError(tok)

    @pl.when(step < NS - 1)
    @jax.named_scope("steady")
    def _():
        if ONLYP:
            return
        for i in range(UN):
            micro(step * UN + i, i)

    @pl.when(step == NS - 1)
    @jax.named_scope("last")
    def _():
        if ONLY or ONLYP:
            return
        for i in range(NKT - (NS - 1) * UN):
            micro((NS - 1) * UN + i, i)


@jax.jit
def pallas_standalone__conformer_family_e_branchformer__speech_kernel(
    x, w_qkv, w_att_out, w_mlp_in, dw_csgu, w_mlp_out, dw_merge, w_merge,
):
    B, T, D = x.shape
    K = dw_csgu.shape[0]
    R = 80
    U = UR
    TP = 4096
    NS = -(-(B * T // R) // UN)
    TH = -(-(R + 2 * PADR) // 32) * 32
    full = lambda a: pl.BlockSpec(a.shape, lambda s: (0,) * a.ndim)

    hbm = pl.BlockSpec(memory_space=pl.ANY)
    kern = functools.partial(_kernel, B=B, T=T, D=D, K=K, R=R, U=U, TP=TP)
    return pl.pallas_call(
        kern,
        grid=(NS,),
        in_specs=[hbm] * 8,
        out_specs=pl.BlockSpec((R * UN, D), lambda s: (s, 0)),
        out_shape=jax.ShapeDtypeStruct((B * T, D), x.dtype),
        scratch_shapes=[
            pltpu.VMEM(x.shape, BF16),
            pltpu.VMEM(w_qkv.shape, BF16),
            pltpu.VMEM(w_att_out.shape, BF16),
            pltpu.VMEM(w_mlp_in.shape, BF16),
            pltpu.VMEM(w_mlp_out.shape, BF16),
            pltpu.VMEM(w_merge.shape, BF16),
            pltpu.VMEM(dw_csgu.shape, BF16),
            pltpu.VMEM(dw_merge.shape, BF16),
            pltpu.SemaphoreType.DMA((7 + len(XG),)),
            pltpu.VMEM((D // 2, D), U32),
            pltpu.VMEM((D // 2, D), U32),
            pltpu.VMEM((D // 2, 2 * D), U32),
            pltpu.VMEM((D // 2, D), U32),
            pltpu.VMEM((D, D), U32),
            pltpu.VMEM((D // 128, 384, 128), F32),
            pltpu.VMEM((2 * D // 128, 384, 128), F32),
            pltpu.VMEM((B, D // 128, TP, 128), BF16),
            pltpu.VMEM((B, D // 128, TP, 128), BF16),
            pltpu.VMEM((U, R, D), F32),
            pltpu.VMEM((U, R, TP), F32),
            pltpu.VMEM((U, R, 128), F32),
            pltpu.VMEM((8, 128), jnp.int32),
        ] + [pltpu.VMEM((D // 128, 7, RR, 128), F32)] * U + [pltpu.VMEM((2 * D // 128, 7, RR, 128), F32)] * U,
        compiler_params=pltpu.CompilerParams(
            dimension_semantics=("arbitrary",),
            vmem_limit_bytes=100 * 1024 * 1024,
        ),
    )(x, w_qkv, w_att_out, w_mlp_in, dw_csgu, w_mlp_out, dw_merge, w_merge).reshape(B, T, D)
```

```python
import functools
import math

import jax
import jax.numpy as jnp
from jax import lax
import jax.experimental.pallas as pl
import jax.experimental.pallas.tpu as pltpu

F32 = jnp.float32
BF16 = jnp.bfloat16
U32 = jnp.uint32
EPS = 1e-5
LOG2E = 1.4426950408889634

R = 80
UN = 12
U = 6
TA = 400
CK = 256
CP = 512
RR = 72

PV0, NPVF, QK0, WIN = 40, 28, 12, 5
UA0, UA1, HA0, AW, AD = 16, 54, 36, 20, 8
THR, PPV0 = 3, 44

XG = [(0, 0, 2), (0, 2, 4), (0, 4, 6), (0, 6, 10), (1, 0, 5), (1, 5, 10)]
DORD = 'x0 w5 w6 w7 w1 w0 x1 w2 x2 x3 w3 w4 x4 x5'.split()
PLAN = ('!x0 L0 L1 '
        '!w5 !w6 !w7 !w0 !w1 D F V0 V1 Q0 Q1 Q2 C0-3 '
        '!x1 !w2 !x2 W2 L2 A0 A1 L3 A2 A3 L4 L5 V2 V3 V4 '
        '!x3 L6 V5 C3-5 L7 C5-7 L8 C7-9 L9 V6 V7 V8 '
        '!w3 !w4 !x4 W3 W4 V9 L10 C9-12 L11 C12-14 L12 C14-16 L13 L14 V10 V11 V12 V13 '
        '!x5 V14 L15 P0 L16 V15 L17 V16 P1 L18 V17 L19 V18 V19').split()


def _gelu(x):
    c = math.sqrt(2.0 / math.pi)
    return 0.5 * x * (1.0 + jnp.tanh(c * (x + 0.044715 * (x * x * x))))


def _dot(a, b):
    return jnp.dot(a, b, preferred_element_type=F32)


def _dot_nt(a, b):
    return lax.dot_general(a, b, (((1,), (1,)), ((), ())), preferred_element_type=F32)


def _cat(parts, axis=-1):
    return jnp.concatenate(parts, axis=axis)


def _pk(x):
    return pltpu.bitcast(x, U32)


def _upk(x):
    return pltpu.bitcast(x, BF16)


def _even_odd(xb):
    xu = _pk(xb)
    return pltpu.bitcast(xu << 16, F32), pltpu.bitcast(xu & jnp.uint32(0xFFFF0000), F32)


def _interleave_bf16(e, o):
    rb = lambda a: pltpu.bitcast(a.astype(BF16).astype(F32), U32)
    return _upk((rb(e) >> 16) | (rb(o) & jnp.uint32(0xFFFF0000)))


def _vregs(a):
    return [a[8 * r:8 * r + 8, l * 128:(l + 1) * 128]
            for r in range(a.shape[0] // 8) for l in range(a.shape[1] // 128)]


def _bc(a):
    return jnp.broadcast_to(a, (a.shape[0], 128))


def _anchored(t, never, deps):
    if not deps:
        return t
    pieces = [t[8 * j:8 * j + 8] for j in range(8)]
    for j, d in enumerate(deps):
        pieces[7 - j] = jnp.where(never, pltpu.bitcast(d, U32), pieces[7 - j])
    return _cat(pieces, axis=0)


def _ffa_chain(ring, lg, q, nj, w_ref, never, rel, init):
    nt = (16, 16, 15)[q]
    acc = init
    ks = [k for pair in zip(range(8), range(8, 16)) for k in pair if k < nt]
    for n_, k in enumerate(ks):
        win = ring[lg, 2 * q, pl.ds(k + 1, 8 * nj), :]
        w = w_ref[lg, pl.ds(8 * (16 * q + k), 8), :]
        if n_ == 0 and rel is not None:
            w = jnp.where(never, rel, w)
        w = _cat([w] * nj, axis=0)
        acc = win * w if acc is None else acc + win * w
    return acc


def _kernel(x_hbm, wqkv_hbm, wao_hbm, wmi_hbm, dwc_hbm, wmo_hbm, dwm_hbm, wm_hbm, o_ref,
            x_ref, wqkv_ref, wao_ref, wmi_ref, wmo_ref, wm_ref, dwc_ref, dwm_ref, sems,
            wqk_s, wvo_s, wmi_s, wmo_s, wm_s, dwc_s, dwm_s, xa_b, v_b, u_s, s_s, mx_s, z_s, *rings,
            B, T, D, K, TP):
    g_s, m_s = rings[:U], rings[U:]
    xa_s, v_s = xa_b.bitcast(U32), v_b.bitcast(U32)
    step = pl.program_id(0)
    NK = T // R
    NKT = B * NK
    NS = -(-NKT // UN)
    NLG = D // 128
    NC = TP // CK
    H = R // 2
    NH = H // 8
    NTILE = (TP // 128) * NLG

    def split(k):
        if isinstance(k, int):
            return k // NK, k % NK
        b = sum((k >= j * NK).astype(jnp.int32) for j in range(1, B))
        return b, k - b * NK

    def rows(i, n):
        r = i * n
        return pl.ds(r if isinstance(r, int) else pl.multiple_of(r, 8), n)

    def seq_put(ref, q, lg, r0, val):
        ref[lg, 2 * q, pl.ds(r0, val.shape[0]), :] = val

    def halo_store(ref, k, kmod, lg, val):
        cur, prv, nxt = ref[kmod % U], ref[(kmod - 1) % U], ref[(kmod + 1) % U]
        xe, xo = val[:H], val[H:]
        row0 = lax.broadcasted_iota(jnp.int32, (8, 128), 0) == 0
        rot = [pltpu.roll(xo[8 * i:8 * i + 8], 1, 0) for i in range(NH)]
        nxt[lg, 6, pl.ds(0, 8), :] = rot[-1]
        rot = [cur[lg, 6, pl.ds(0, 8), :]] + rot
        sh = _cat([jnp.where(row0, rot[i], rot[i + 1]) for i in range(NH)], axis=0)
        zero = jnp.zeros((8, 128), F32)
        if isinstance(k, int):
            first, last = k % NK == 0, k % NK == NK - 1
        else:
            first = (split(k)[1] == 0) if any((j * NK) % UN == kmod for j in range(B)) else False
            last = (split(k)[1] == NK - 1) if any((j * NK - 1) % UN == kmod for j in range(1, B + 1)) else False
        sh0 = sh[:8]
        if first is not False:
            cut = row0 if first is True else jnp.logical_and(row0, first)
            sh = _cat([jnp.where(cut, 0.0, sh0), sh[8:]], axis=0)
        seqs = [xe, sh - xe, xo - xe]
        for q, v in enumerate(seqs):
            seq_put(cur, q, lg, 8, v)
            top, bot = v[:8], v[H - 8:]
            if first is not False:
                edge = jnp.where(row0, sh0, 0.0) if q == 1 else zero
                top = None if (first is True and k == 0) else (edge if first is True else jnp.where(first, edge, top))
            if last is not False:
                bot = zero if last is True else jnp.where(last, 0.0, bot)
            if top is not None:
                seq_put(prv, q, lg, 8 + H, top)
            seq_put(nxt, q, lg, 0, bot)

    def tail_store(ref, nlg):
        row0 = lax.broadcasted_iota(jnp.int32, (8, 128), 0) == 0
        for lg in range(nlg):
            e = ref[NKT % U][lg, 6, pl.ds(0, 8), :]
            for q in range(3):
                seq_put(ref[(NKT - 1) % U], q, lg, 8 + H,
                        jnp.where(row0, e, 0.0) if q == 1 else jnp.zeros((8, 128), F32))

    def xa_rows(b, r):
        return _upk(_cat([xa_s[b, lg, r, :] for lg in range(NLG)]))

    def ln_tile(b, t):
        eo = _even_odd(x_ref[b, pl.ds(t * TA, TA), :])
        x = _cat([eo[par][i * H:(i + 1) * H] for i in range(TA // R) for par in range(2)], axis=0)
        xc = x - jnp.mean(x, axis=-1, keepdims=True)
        rs = lax.rsqrt(jnp.mean(xc * xc, axis=-1, keepdims=True) + EPS)
        xa = xc * rs
        for lg in range(NLG):
            xa_b[b, lg, pl.ds(t * TA, TA), :] = xa[:, lg * 128:(lg + 1) * 128].astype(BF16)

    def v_tile(b, t):
        w = wvo_s[...]
        v = _dot(xa_rows(b, rows(t, TA // 2)), _upk(w))
        for lg in range(NLG):
            v_b[b, lg, pl.ds(t * TA, TA), :] = v[:, lg * 128:(lg + 1) * 128].astype(BF16)

    def stage_a2(k, kmod):
        b, i = split(k)
        h = _gelu(_dot(xa_rows(b, rows(i, R // 2)), _upk(wmi_s[...])))
        u_s[kmod % U] = h[:, :D]
        hg = h[:, D:]
        mu = jnp.mean(hg, axis=-1, keepdims=True)
        xc = hg - mu
        rs = lax.rsqrt(jnp.mean(xc * xc, axis=-1, keepdims=True) + EPS)
        g = xc * rs
        for lg in range(NLG):
            halo_store(g_s, k, kmod, lg, g[:, lg * 128:(lg + 1) * 128])
        return _vregs(h[:, :D]), _vregs(hg), _vregs(_bc(mu)), _vregs(_bc(rs)), _vregs(g)

    def c1_mm(k, kmod, parts):
        loc = _dot(_cat(parts).astype(BF16), _upk(wmo_s[...]))
        for lg in range(NLG):
            halo_store(m_s, k, kmod, NLG + lg, loc[:, lg * 128:(lg + 1) * 128])

    def c2_mm(k, pos, parts):
        b, i = split(k)
        r0 = i * R
        r0 = r0 if isinstance(r0, int) else pl.multiple_of(r0, 16)
        y = _dot(_cat(parts).astype(BF16), _upk(wm_s[...]))
        xe, xo = _even_odd(x_ref[b, pl.ds(r0, R), :])
        o_ref[pl.ds(pos * R, R), :] = _interleave_bf16(y[:H] + xe, y[H:] + xo)

    def q_proj(k):
        b, i = split(k)
        return _dot(xa_rows(b, rows(i, R // 2)), _upk(wqk_s[...])).astype(BF16)

    def k_chunk(b, c, never, deps):
        blks = []
        for kt in range(CK // 128):
            blks.append(_cat([
                _anchored(xa_s[b, lg, pl.ds(c * CK // 2 + kt * 64, 64), :], never,
                          deps[(c * (CK // 128) + kt) * NLG + lg])
                for lg in range(NLG)]))
        return _upk(_cat(blks, axis=0))

    def q_chunks(k, kmod, q, never, deps, mx, ca, cb, hook=None):
        b, _ = split(k)
        for c in range(ca, cb):
            s = _dot_nt(q, k_chunk(b, c, never, deps))
            if hook is not None:
                hook(NC + c, s)
            for l in range(CK // 128):
                sl = s[:, l * 128:(l + 1) * 128]
                c0 = c * CK + l * 128
                if c0 + 128 > T:
                    col = lax.broadcasted_iota(jnp.int32, (R, 128), 1) + c0
                    sl = jnp.where(col < T, sl, -jnp.inf)
                s_s[kmod % U, :, pl.ds(c0, 128)] = sl
                mx = sl if mx is None else jnp.maximum(mx, sl)
        if cb == NC:
            mx_s[kmod % U] = jnp.broadcast_to(jnp.max(mx, axis=-1, keepdims=True), (R, 128))
        return mx

    def v_chunk(b, c, lg, never, deps):
        return _upk(_cat([
            _anchored(v_s[b, lg, pl.ds(c * CP // 2 + kt * 64, 64), :], never, deps[kt])
            for kt in range(CP // 128)], axis=0))

    def stage_p(k, kmod, never, deps, hook=None, thr=0):
        b, _ = split(k)
        m = mx_s[kmod % U]
        neverr = _cat([never] * (R // 8), axis=0)
        ncp = TP // CP
        tpc = CP // 128
        ls = None
        pbs, pvs, accs = [], [], []
        for lg in range(NLG):
            acc = None
            for c in range(ncp):
                gc = lg * ncp + c
                if lg == 0:
                    ps = []
                    if thr and c >= thr:
                        m = jnp.where(neverr, pvs[c - thr], m)
                    for l in range(tpc):
                        ps.append(jnp.exp2(s_s[kmod % U, :, pl.ds(c * CP + l * 128, 128)] - m))
                    for p in ps:
                        ls = p if ls is None else ls + p
                    pbs.append(_cat(ps).astype(BF16))
                pv = _dot(pbs[c], v_chunk(b, c, lg, never, deps[gc * tpc:(gc + 1) * tpc]))
                if hook is not None:
                    hook(gc, pv)
                pvs.append(pv)
                acc = pv if acc is None else acc + pv
            accs.append(acc)
        acc = _cat(accs)
        l = jnp.sum(ls, axis=-1, keepdims=True)
        glob = acc * (1.0 / l)
        for lg in range(NLG):
            halo_store(m_s, k, kmod, lg, glob[:, lg * 128:(lg + 1) * 128])

    def micro(n, pos):
        nmod = pos % U
        ok = lambda k: (not isinstance(k, int)) or 0 <= k < NKT
        never = z_s[...] != 0
        tpc = NTILE // NC
        hasp, hasq = ok(n + 2), ok(n + 3)
        lo = 0 if hasp else NTILE
        hi = 2 * NTILE if hasq else NTILE
        res = {}
        jobs = []
        if isinstance(n, int) and n + 4 == NKT:
            tail_store(g_s, NLG)
        if isinstance(n, int) and n + 2 == NKT:
            tail_store(m_s, 2 * NLG)

        def chain_jobs(name, ring, nlg, w_ref, fin):
            for lg in range(nlg):
                for q in range(3):
                    def fn(rel, lg=lg, q=q):
                        init = None if q == 0 else _cat(res[name, lg, 0], axis=0)
                        y = _ffa_chain(ring, lg, q, NH, w_ref, never, rel, init)
                        if q > 0:
                            y = fin(lg, q - 1, y)
                        return [y[8 * i:8 * i + 8] for i in range(NH)]
                    jobs.append(((name, lg, q), fn))

        chain_jobs('c2', m_s[nmod], 2 * NLG, dwm_s, lambda lg, par, y: y)
        if hasp:
            km = (nmod + 2) % U
            chain_jobs('c1', g_s[km], NLG, dwc_s,
                       lambda lg, par, y: y * u_s[km, pl.ds(par * H, H), pl.ds(lg * 128, 128)])

        def gather(name, nlg):
            return [_cat([v for q in (1, 2) for v in res[name, lg, q]], axis=0) for lg in range(nlg)]

        if hasp and hasq:
            npv = (NPVF * len(jobs)) // 100
        elif hasp:
            npv = len(jobs)
        else:
            npv = 0
        pv0 = PV0 if hasq else 0
        dls = [pv0 + (j * (NTILE - pv0)) // max(npv, 1) for j in range(npv)]
        nq = len(jobs) - npv
        dls += [NTILE + QK0 + (j * (NTILE - QK0)) // nq if hasq else None for j in range(nq)]
        slots = [[] for _ in range(2 * NTILE)]
        pending = {}

        def addslot(dl, vals):
            for v in vals:
                while len(slots[dl]) >= 8:
                    dl += 1
                slots[dl].append(v)

        for (key, fn), dl in zip(jobs, dls):
            rc = None if dl is None else dl // tpc - WIN
            if rc is None or rc < lo // tpc:
                res[key] = fn(None)
                if dl is not None:
                    addslot(dl, res[key])
            else:
                pending.setdefault(rc, []).append((key, fn, dl))

        def hook(gc, val):
            for j, (key, fn, dl) in enumerate(pending.pop(gc, [])):
                res[key] = fn(val[8 * j:8 * j + 8, :128])
                addslot(dl, res[key])

        def put(items, a, b):
            a, b = max(a, lo), min(b, hi)
            for j, it in enumerate(items):
                addslot(a + (j * (b - a)) // len(items), [it])

        if hasq:
            q = q_proj(n + 3)
        if ok(n + 4):
            uu, hh, mu, rs, gg = stage_a2(n + 4, (pos + 4) % UN)
            put(uu, UA0, UA1)
            put(hh, HA0, HA0 + AW)
            put(mu, HA0 + AD, HA0 + AD + AW)
            put(rs, HA0 + 2 * AD, HA0 + 2 * AD + AW)
            put(gg, HA0 + 2 * AD + 4, HA0 + 2 * AD + 4 + AW)
        if hasp:
            stage_p(n + 2, (pos + 2) % UN, never, slots[:NTILE], hook,
                    THR if (not hasq or pos == UN - 1) else 0)
        if hasq:
            q_chunks(n + 3, (pos + 3) % UN, q, never, slots[NTILE:], None, 0, NC, hook)
        assert not pending
        if hasp:
            c1_mm(n + 2, (pos + 2) % UN, gather('c1', NLG))
        c2_mm(n, pos, gather('c2', 2 * NLG))

    @pl.when(step == 0)
    def _():
        nt1 = T // TA
        cw = [pltpu.make_async_copy(src, dst, sems.at[j]) for j, (src, dst) in enumerate(
            [(wqkv_hbm.at[:, pl.ds(0, 2 * D)], wqkv_ref.at[:, pl.ds(0, 2 * D)]), (wao_hbm, wao_ref),
             (wmi_hbm, wmi_ref), (wmo_hbm, wmo_ref), (wm_hbm, wm_ref),
             (dwc_hbm, dwc_ref), (dwm_hbm, dwm_ref),
             (wqkv_hbm.at[:, pl.ds(2 * D, D)], wqkv_ref.at[:, pl.ds(2 * D, D)])])]
        cx = [pltpu.make_async_copy(x_hbm.at[b, pl.ds(t0 * TA, (t1 - t0) * TA), :],
                                    x_ref.at[b, pl.ds(t0 * TA, (t1 - t0) * TA), :], sems.at[8 + j])
              for j, (b, t0, t1) in enumerate(XG)]
        dmas = {'w%d' % j: c for j, c in enumerate(cw)}
        dmas.update({'x%d' % j: c for j, c in enumerate(cx)})
        for name in DORD:
            dmas[name].start()
        z_s[...] = jnp.zeros(z_s.shape, z_s.dtype)
        for b in range(B):
            for lg in range(NLG):
                xa_b[b, lg, pl.ds(T, TP - T), :] = jnp.zeros((TP - T, 128), BF16)
                v_b[b, lg, pl.ds(T, TP - T), :] = jnp.zeros((TP - T, 128), BF16)
        for ring, nlg in ((g_s, NLG), (m_s, 2 * NLG)):
            for lg in range(nlg):
                for q in range(3):
                    seq_put(ring[0], q, lg, 0, jnp.zeros((8, 128), F32))
                ring[0][lg, 6, pl.ds(0, 8), :] = jnp.zeros((8, 128), F32)
        nodeps = [[] for _ in range(NTILE)]
        qs, mxs = {}, {0: None, 1: None, 2: None}

        def fold():
            wvo_s[...] = _pk(_dot(wqkv_ref[:, 2 * D:3 * D], wao_ref[...]).astype(BF16))
            wqk_s[...] = _pk((_dot_nt(wqkv_ref[:, 0:D], wqkv_ref[:, D:2 * D])
                              * (D ** -0.5 * LOG2E)).astype(BF16))

        def taps():
            for src, dst, nlg, centre in ((dwc_ref, dwc_s, NLG, 0.0), (dwm_ref, dwm_s, 2 * NLG, 1.0)):
                for lg in range(nlg):
                    wl = src[:, pl.ds(lg * 128, 128)].astype(F32)
                    w = [wl[i:i + 1] for i in range(K)]
                    if centre:
                        w[K // 2] = w[K // 2] + centre
                    wa, wb = w[1::2], w[0::2]
                    ws = [wa[i] + wb[i] if i < len(wa) else wb[i] for i in range(len(wb))]
                    for q, ww in enumerate((ws, wb, wa)):
                        for i, wi in enumerate(ww):
                            dst[lg, pl.ds(8 * (16 * q + i), 8), :] = jnp.broadcast_to(wi, (8, 128))

        def warm_p(k):
            never = z_s[...] != 0
            deps = [[] for _ in range(NTILE)]
            parts, outs = [], []
            for lg in range(NLG):
                sc = _ffa_chain(g_s[k], lg, 0, NH, dwc_s, None, None, None)
                ys = [_ffa_chain(g_s[k], lg, q, NH, dwc_s, None, None, sc)
                      * u_s[k, pl.ds((q - 1) * H, H), pl.ds(lg * 128, 128)] for q in (1, 2)]
                parts.append(_cat(ys, axis=0))
                outs += [sc] + ys
            for j, y in enumerate(outs):
                deps[PPV0 + (j * (NTILE - PPV0)) // len(outs)] = [y[8 * i:8 * i + 8] for i in range(NH)]
            stage_p(k, k, never, deps)
            c1_mm(k, k, parts)

        for tok in PLAN:
            op, arg = tok[0], tok[1:]
            if op == '!':
                dmas[arg].wait()
            elif op == 'W':
                src, dst = {'2': (wmi_ref, wmi_s), '3': (wmo_ref, wmo_s), '4': (wm_ref, wm_s)}[arg]
                dst[...] = _pk(src[...])
            elif op == 'D':
                taps()
            elif op == 'F':
                fold()
            elif op == 'L':
                ln_tile(int(arg) // nt1, int(arg) % nt1)
            elif op == 'V':
                v_tile(int(arg) // nt1, int(arg) % nt1)
            elif op == 'Q':
                qs[int(arg)] = q_proj(int(arg))
            elif op == 'A':
                stage_a2(int(arg), int(arg))
            elif op == 'C':
                ca, cb = arg.split('-')
                for k in range(3):
                    mxs[k] = q_chunks(k, k, qs[k], None, nodeps, mxs[k], int(ca), int(cb))
            else:
                warm_p(int(arg))

    @pl.when(step < NS - 1)
    def _():
        for i in range(UN):
            micro(step * UN + i, i)

    @pl.when(step == NS - 1)
    def _():
        for i in range(NKT - (NS - 1) * UN):
            micro((NS - 1) * UN + i, i)


@jax.jit
def pallas_standalone__conformer_family_e_branchformer__speech_kernel(
    x: jax.Array,
    w_qkv: jax.Array,
    w_att_out: jax.Array,
    w_mlp_in: jax.Array,
    dw_csgu: jax.Array,
    w_mlp_out: jax.Array,
    dw_merge: jax.Array,
    w_merge: jax.Array,
):
    B, T, D = x.shape
    K = dw_csgu.shape[0]
    assert (B, T, D, K) == (2, 4000, 256, 31), "schedule tables are written for this shape"
    TP = 4096
    NS = -(-(B * T // R) // UN)
    nlg = D // 128
    kern = functools.partial(_kernel, B=B, T=T, D=D, K=K, TP=TP)
    out = pl.pallas_call(
        kern,
        grid=(NS,),
        in_specs=[pl.BlockSpec(memory_space=pl.ANY)] * 8,
        out_specs=pl.BlockSpec((R * UN, D), lambda s: (s, 0)),
        out_shape=jax.ShapeDtypeStruct((B * T, D), x.dtype),
        scratch_shapes=[
            pltpu.VMEM(x.shape, BF16),
            pltpu.VMEM(w_qkv.shape, BF16),
            pltpu.VMEM(w_att_out.shape, BF16),
            pltpu.VMEM(w_mlp_in.shape, BF16),
            pltpu.VMEM(w_mlp_out.shape, BF16),
            pltpu.VMEM(w_merge.shape, BF16),
            pltpu.VMEM(dw_csgu.shape, BF16),
            pltpu.VMEM(dw_merge.shape, BF16),
            pltpu.SemaphoreType.DMA((8 + len(XG),)),
            pltpu.VMEM((D // 2, D), U32),
            pltpu.VMEM((D // 2, D), U32),
            pltpu.VMEM((D // 2, 2 * D), U32),
            pltpu.VMEM((D // 2, D), U32),
            pltpu.VMEM((D, D), U32),
            pltpu.VMEM((nlg, 384, 128), F32),
            pltpu.VMEM((2 * nlg, 384, 128), F32),
            pltpu.VMEM((B, nlg, TP, 128), BF16),
            pltpu.VMEM((B, nlg, TP, 128), BF16),
            pltpu.VMEM((U, R, D), F32),
            pltpu.VMEM((U, R, TP), F32),
            pltpu.VMEM((U, R, 128), F32),
            pltpu.VMEM((8, 128), jnp.int32),
        ] + [pltpu.VMEM((nlg, 7, RR, 128), F32)] * U + [pltpu.VMEM((2 * nlg, 7, RR, 128), F32)] * U,
        compiler_params=pltpu.CompilerParams(
            dimension_semantics=("arbitrary",),
            vmem_limit_bytes=100 * 1024 * 1024,
        ),
    )(x, w_qkv, w_att_out, w_mlp_in, dw_csgu, w_mlp_out, dw_merge, w_merge)
    return out.reshape(B, T, D)
```

```python
import functools
import math

import jax
import jax.numpy as jnp
from jax import lax
import jax.experimental.pallas as pl
import jax.experimental.pallas.tpu as pltpu

F32 = jnp.float32
BF16 = jnp.bfloat16
U32 = jnp.uint32
EPS = 1e-5
LOG2E = 1.4426950408889634

R = 80
UN = 12
U = 6
TA = 400
CK = 256
CP = 512
RR = 56

PV0, NPVF, QK0, WIN = 40, 28, 12, 5
UA0, UA1, HA0, AW, AD = 16, 54, 36, 24, 7
THR, THRL, PPV0 = 2, 3, 44

XG = [(0, 0, 2), (0, 2, 4), (0, 4, 6), (0, 6, 10), (1, 0, 5), (1, 5, 10)]
DORD = 'x0 w5 w6 w7 w1 w0 x1 w2 x2 x3 w3 w4 x4 x5'.split()
PLAN = ('!x0 L0 L1 '
        '!w5 !w6 !w7 !w0 !w1 D F V0 V1 Q0 Q1 Q2 C0-3 '
        '!x1 !w2 !x2 W2 L2 A0 A1 L3 A2 A3 L4 L5 V2 V3 V4 '
        '!x3 L6 V5 C3-5 L7 C5-7 L8 C7-9 L9 V6 V7 V8 '
        '!w3 !w4 !x4 W3 W4 V9 L10 C9-12 L11 C12-14 L12 C14-16 L13 L14 V10 V11 V12 V13 '
        '!x5 V14 L15 P0 L16 V15 L17 V16 P1 L18 V17 L19 V18 V19').split()


def _gelu(x):
    c = math.sqrt(2.0 / math.pi)
    return 0.5 * x * (1.0 + jnp.tanh(c * (x + 0.044715 * (x * x * x))))


def _dot(a, b):
    return jnp.dot(a, b, preferred_element_type=F32)


def _dot_nt(a, b):
    return lax.dot_general(a, b, (((1,), (1,)), ((), ())), preferred_element_type=F32)


def _cat(parts, axis=-1):
    return jnp.concatenate(parts, axis=axis)


def _pk(x):
    return pltpu.bitcast(x, U32)


def _upk(x):
    return pltpu.bitcast(x, BF16)


def _even_odd(xb):
    xu = _pk(xb)
    return pltpu.bitcast(xu << 16, F32), pltpu.bitcast(xu & jnp.uint32(0xFFFF0000), F32)


def _interleave_bf16(e, o):
    rb = lambda a: pltpu.bitcast(a.astype(BF16).astype(F32), U32)
    return _upk((rb(e) >> 16) | (rb(o) & jnp.uint32(0xFFFF0000)))


def _vregs(a):
    return [a[8 * r:8 * r + 8, l * 128:(l + 1) * 128]
            for r in range(a.shape[0] // 8) for l in range(a.shape[1] // 128)]


def _bc(a):
    return jnp.broadcast_to(a, (a.shape[0], 128))


def _anchored(t, never, deps):
    if not deps:
        return t
    pieces = [t[8 * j:8 * j + 8] for j in range(8)]
    for j, d in enumerate(deps):
        pieces[7 - j] = jnp.where(never, pltpu.bitcast(d, U32), pieces[7 - j])
    return _cat(pieces, axis=0)


def _ffa_chain(ring, lg, q, nj, w_ref, never, rel, init):
    nt = (16, 16, 15)[q]
    acc = init
    ks = [k for pair in zip(range(8), range(8, 16)) for k in pair if k < nt]
    for n_, k in enumerate(ks):
        win = ring[lg, 2 * q, pl.ds(k + 1, 8 * nj), :]
        w = w_ref[lg, pl.ds(8 * (16 * q + k), 8), :]
        if n_ == 0 and rel is not None:
            w = jnp.where(never, rel, w)
        w = _cat([w] * nj, axis=0)
        acc = win * w if acc is None else acc + win * w
    return acc


def _kernel(x_hbm, wqkv_hbm, wao_hbm, wmi_hbm, dwc_hbm, wmo_hbm, dwm_hbm, wm_hbm, o_ref,
            x_ref, wqkv_ref, wao_ref, wmi_ref, wmo_ref, wm_ref, dwc_ref, dwm_ref, sems,
            wqk_s, wvo_s, wmi_s, wmo_s, wm_s, dwc_s, dwm_s, xa_s, v_s, u_s, s_s, mx_s, z_s, *rings,
            B, T, D, K, TP):
    g_s, m_s = rings[:U], rings[U:]
    step = pl.program_id(0)
    NK = T // R
    NKT = B * NK
    NS = -(-NKT // UN)
    NLG = D // 128
    NC = TP // CK
    H = R // 2
    NH = H // 8
    NTILE = (TP // 128) * NLG

    def split(k):
        if isinstance(k, int):
            return k // NK, k % NK
        b = sum((k >= j * NK).astype(jnp.int32) for j in range(1, B))
        return b, k - b * NK

    def rows(i, n):
        r = i * n
        return pl.ds(r if isinstance(r, int) else pl.multiple_of(r, 8), n)

    def seq_put(ref, q, lg, r0, val):
        ref[lg, 2 * q, pl.ds(r0, val.shape[0]), :] = val

    def halo_store(ref, k, kmod, lg, val):
        cur, prv, nxt = ref[kmod % U], ref[(kmod - 1) % U], ref[(kmod + 1) % U]
        xe, xo = val[:H], val[H:]
        row0 = lax.broadcasted_iota(jnp.int32, (8, 128), 0) == 0
        rot = [pltpu.roll(xo[8 * i:8 * i + 8], 1, 0) for i in range(NH)]
        nxt[lg, 6, pl.ds(0, 8), :] = rot[-1]
        rot = [cur[lg, 6, pl.ds(0, 8), :]] + rot
        sh = _cat([jnp.where(row0, rot[i], rot[i + 1]) for i in range(NH)], axis=0)
        zero = jnp.zeros((8, 128), F32)
        if isinstance(k, int):
            first, last = k % NK == 0, k % NK == NK - 1
        else:
            first = (split(k)[1] == 0) if any((j * NK) % UN == kmod for j in range(B)) else False
            last = (split(k)[1] == NK - 1) if any((j * NK - 1) % UN == kmod for j in range(1, B + 1)) else False
        sh0 = sh[:8]
        if first is not False:
            cut = row0 if first is True else jnp.logical_and(row0, first)
            sh = _cat([jnp.where(cut, 0.0, sh0), sh[8:]], axis=0)
        seqs = [xe, sh - xe, xo - xe]
        for q, v in enumerate(seqs):
            seq_put(cur, q, lg, 8, v)
            top, bot = v[:8], v[H - 8:]
            if first is not False:
                edge = jnp.where(row0, sh0, 0.0) if q == 1 else zero
                top = None if (first is True and k == 0) else (edge if first is True else jnp.where(first, edge, top))
            if last is not False:
                bot = zero if last is True else jnp.where(last, 0.0, bot)
            if top is not None:
                seq_put(prv, q, lg, 8 + H, top)
            seq_put(nxt, q, lg, 0, bot)

    def tail_store(ref, nlg):
        row0 = lax.broadcasted_iota(jnp.int32, (8, 128), 0) == 0
        for lg in range(nlg):
            e = ref[NKT % U][lg, 6, pl.ds(0, 8), :]
            for q in range(3):
                seq_put(ref[(NKT - 1) % U], q, lg, 8 + H,
                        jnp.where(row0, e, 0.0) if q == 1 else jnp.zeros((8, 128), F32))

    def xa_rows(b, r):
        return _upk(xa_s[b, r, :])

    def ln_tile(b, t):
        eo = _even_odd(x_ref[b, pl.ds(t * TA, TA), :])
        x = _cat([eo[par][i * H:(i + 1) * H] for i in range(TA // R) for par in range(2)], axis=0)
        xc = x - jnp.mean(x, axis=-1, keepdims=True)
        rs = lax.rsqrt(jnp.mean(xc * xc, axis=-1, keepdims=True) + EPS)
        xa = xc * rs
        xa_s[b, rows(t, TA // 2), :] = _pk(xa.astype(BF16))

    def v_tile(b, t):
        w = wvo_s[...]
        v = _dot(xa_rows(b, rows(t, TA // 2)), _upk(w))
        v_s[b, rows(t, TA // 2), :] = _pk(v.astype(BF16))

    def stage_a2(k, kmod):
        b, i = split(k)
        h = _gelu(_dot(xa_rows(b, rows(i, R // 2)), _upk(wmi_s[...])))
        u_s[kmod % U] = h[:, :D]
        hg = h[:, D:]
        mu = jnp.mean(hg, axis=-1, keepdims=True)
        xc = hg - mu
        rs = lax.rsqrt(jnp.mean(xc * xc, axis=-1, keepdims=True) + EPS)
        g = xc * rs
        for lg in range(NLG):
            halo_store(g_s, k, kmod, lg, g[:, lg * 128:(lg + 1) * 128])
        return _vregs(h[:, :D]), _vregs(hg), _vregs(_bc(mu)), _vregs(_bc(rs)), _vregs(g)

    def c1_mm(k, kmod, parts):
        loc = _dot(_cat(parts).astype(BF16), _upk(wmo_s[...]))
        for lg in range(NLG):
            halo_store(m_s, k, kmod, NLG + lg, loc[:, lg * 128:(lg + 1) * 128])

    def c2_mm(k, pos, parts):
        b, i = split(k)
        r0 = i * R
        r0 = r0 if isinstance(r0, int) else pl.multiple_of(r0, 16)
        y = _dot(_cat(parts).astype(BF16), _upk(wm_s[...]))
        xe, xo = _even_odd(x_ref[b, pl.ds(r0, R), :])
        o_ref[pl.ds(pos * R, R), :] = _interleave_bf16(y[:H] + xe, y[H:] + xo)

    def q_proj(k):
        b, i = split(k)
        return _dot(xa_rows(b, rows(i, R // 2)), _upk(wqk_s[...])).astype(BF16)

    def k_chunk(b, c, never, deps):
        blks = []
        for kt in range(CK // 128):
            blks.append(_cat([
                _anchored(xa_s[b, pl.ds(c * CK // 2 + kt * 64, 64), pl.ds(lg * 128, 128)], never,
                          deps[(c * (CK // 128) + kt) * NLG + lg])
                for lg in range(NLG)]))
        return _upk(_cat(blks, axis=0))

    def q_chunks(k, kmod, q, never, deps, mx, ca, cb, hook=None):
        b, _ = split(k)
        for c in range(ca, cb):
            s = _dot_nt(q, k_chunk(b, c, never, deps))
            if hook is not None:
                hook(NC + c, s)
            for l in range(CK // 128):
                sl = s[:, l * 128:(l + 1) * 128]
                c0 = c * CK + l * 128
                if c0 + 128 > T:
                    col = lax.broadcasted_iota(jnp.int32, (R, 128), 1) + c0
                    sl = jnp.where(col < T, sl, -jnp.inf)
                s_s[kmod % U, :, pl.ds(c0, 128)] = sl
                mx = sl if mx is None else jnp.maximum(mx, sl)
        if cb == NC:
            mx_s[kmod % U] = jnp.broadcast_to(jnp.max(mx, axis=-1, keepdims=True), (R, 128))
        return mx

    def v_chunk(b, c, lg, never, deps):
        return _upk(_cat([
            _anchored(v_s[b, pl.ds(c * CP // 2 + kt * 64, 64), pl.ds(lg * 128, 128)], never, deps[kt])
            for kt in range(CP // 128)], axis=0))

    def stage_p(k, kmod, never, deps, hook=None, thr=0):
        b, _ = split(k)
        m = mx_s[kmod % U]
        neverr = _cat([never] * (R // 8), axis=0)
        ncp = TP // CP
        tpc = CP // 128
        ls = None
        pbs, pvs, accs = [], [], []
        for lg in range(NLG):
            acc = None
            for c in range(ncp):
                gc = lg * ncp + c
                if lg == 0:
                    ps = []
                    if thr and c >= thr:
                        m = jnp.where(neverr, pvs[c - thr], m)
                    for l in range(tpc):
                        ps.append(jnp.exp2(s_s[kmod % U, :, pl.ds(c * CP + l * 128, 128)] - m))
                    for p in ps:
                        ls = p if ls is None else ls + p
                    pbs.append(_cat(ps).astype(BF16))
                pv = _dot(pbs[c], v_chunk(b, c, lg, never, deps[gc * tpc:(gc + 1) * tpc]))
                if hook is not None:
                    hook(gc, pv)
                pvs.append(pv)
                acc = pv if acc is None else acc + pv
            accs.append(acc)
        acc = _cat(accs)
        l = jnp.sum(ls, axis=-1, keepdims=True)
        glob = acc * (1.0 / l)
        for lg in range(NLG):
            halo_store(m_s, k, kmod, lg, glob[:, lg * 128:(lg + 1) * 128])

    def micro(n, pos):
        nmod = pos % U
        ok = lambda k: (not isinstance(k, int)) or 0 <= k < NKT
        never = z_s[...] != 0
        tpc = NTILE // NC
        hasp, hasq = ok(n + 2), ok(n + 3)
        lo = 0 if hasp else NTILE
        hi = 2 * NTILE if hasq else NTILE
        res = {}
        jobs = []
        if isinstance(n, int) and n + 4 == NKT:
            tail_store(g_s, NLG)
        if isinstance(n, int) and n + 2 == NKT:
            tail_store(m_s, 2 * NLG)

        def chain_jobs(name, ring, nlg, w_ref, fin):
            for lg in range(nlg):
                for q in range(3):
                    def fn(rel, lg=lg, q=q):
                        init = None if q == 0 else _cat(res[name, lg, 0], axis=0)
                        y = _ffa_chain(ring, lg, q, NH, w_ref, never, rel, init)
                        if q > 0:
                            y = fin(lg, q - 1, y)
                        return [y[8 * i:8 * i + 8] for i in range(NH)]
                    jobs.append(((name, lg, q), fn))

        chain_jobs('c2', m_s[nmod], 2 * NLG, dwm_s, lambda lg, par, y: y)
        if hasp:
            km = (nmod + 2) % U
            chain_jobs('c1', g_s[km], NLG, dwc_s,
                       lambda lg, par, y: y * u_s[km, pl.ds(par * H, H), pl.ds(lg * 128, 128)])

        def gather(name, nlg):
            return [_cat([v for q in (1, 2) for v in res[name, lg, q]], axis=0) for lg in range(nlg)]

        if hasp and hasq:
            npv = (NPVF * len(jobs)) // 100
        elif hasp:
            npv = len(jobs)
        else:
            npv = 0
        pv0 = PV0 if hasq else 0
        dls = [pv0 + (j * (NTILE - pv0)) // max(npv, 1) for j in range(npv)]
        nq = len(jobs) - npv
        dls += [NTILE + QK0 + (j * (NTILE - QK0)) // nq if hasq else None for j in range(nq)]
        slots = [[] for _ in range(2 * NTILE)]
        pending = {}

        def addslot(dl, vals):
            for v in vals:
                while len(slots[dl]) >= 8:
                    dl += 1
                slots[dl].append(v)

        for (key, fn), dl in zip(jobs, dls):
            rc = None if dl is None else dl // tpc - WIN
            if rc is None or rc < lo // tpc:
                res[key] = fn(None)
                if dl is not None:
                    addslot(dl, res[key])
            else:
                pending.setdefault(rc, []).append((key, fn, dl))

        def hook(gc, val):
            for j, (key, fn, dl) in enumerate(pending.pop(gc, [])):
                res[key] = fn(val[8 * j:8 * j + 8, :128])
                addslot(dl, res[key])

        def put(items, a, b):
            a, b = max(a, lo), min(b, hi)
            for j, it in enumerate(items):
                addslot(a + (j * (b - a)) // len(items), [it])

        if hasq:
            q = q_proj(n + 3)
        if ok(n + 4):
            uu, hh, mu, rs, gg = stage_a2(n + 4, (pos + 4) % UN)
            put(uu, UA0, UA1)
            put(hh, HA0, HA0 + AW)
            put(mu, HA0 + AD, HA0 + AD + AW)
            put(rs, HA0 + 2 * AD, HA0 + 2 * AD + AW)
            put(gg, HA0 + 2 * AD + 4, HA0 + 2 * AD + 4 + AW)
        if hasp:
            stage_p(n + 2, (pos + 2) % UN, never, slots[:NTILE], hook,
                    THRL if not hasq else (THR if pos == UN - 1 else 0))
        if hasq:
            q_chunks(n + 3, (pos + 3) % UN, q, never, slots[NTILE:], None, 0, NC, hook)
        assert not pending
        if hasp:
            c1_mm(n + 2, (pos + 2) % UN, gather('c1', NLG))
        c2_mm(n, pos, gather('c2', 2 * NLG))

    @pl.when(step == 0)
    def _():
        nt1 = T // TA
        cw = [pltpu.make_async_copy(src, dst, sems.at[j]) for j, (src, dst) in enumerate(
            [(wqkv_hbm.at[:, pl.ds(0, 2 * D)], wqkv_ref.at[:, pl.ds(0, 2 * D)]), (wao_hbm, wao_ref),
             (wmi_hbm, wmi_ref), (wmo_hbm, wmo_ref), (wm_hbm, wm_ref),
             (dwc_hbm, dwc_ref), (dwm_hbm, dwm_ref),
             (wqkv_hbm.at[:, pl.ds(2 * D, D)], wqkv_ref.at[:, pl.ds(2 * D, D)])])]
        cx = [pltpu.make_async_copy(x_hbm.at[b, pl.ds(t0 * TA, (t1 - t0) * TA), :],
                                    x_ref.at[b, pl.ds(t0 * TA, (t1 - t0) * TA), :], sems.at[8 + j])
              for j, (b, t0, t1) in enumerate(XG)]
        dmas = {'w%d' % j: c for j, c in enumerate(cw)}
        dmas.update({'x%d' % j: c for j, c in enumerate(cx)})
        for name in DORD:
            dmas[name].start()
        z_s[...] = jnp.zeros(z_s.shape, z_s.dtype)
        for b in range(B):
            xa_s[b, pl.ds(T // 2, (TP - T) // 2), :] = jnp.zeros(((TP - T) // 2, D), U32)
            v_s[b, pl.ds(T // 2, (TP - T) // 2), :] = jnp.zeros(((TP - T) // 2, D), U32)
        for ring, nlg in ((g_s, NLG), (m_s, 2 * NLG)):
            for lg in range(nlg):
                for q in range(3):
                    seq_put(ring[0], q, lg, 0, jnp.zeros((8, 128), F32))
                ring[0][lg, 6, pl.ds(0, 8), :] = jnp.zeros((8, 128), F32)
        nodeps = [[] for _ in range(NTILE)]
        qs, mxs = {}, {0: None, 1: None, 2: None}

        def fold():
            wvo_s[...] = _pk(_dot(wqkv_ref[:, 2 * D:3 * D], wao_ref[...]).astype(BF16))
            wqk_s[...] = _pk((_dot_nt(wqkv_ref[:, 0:D], wqkv_ref[:, D:2 * D])
                              * (D ** -0.5 * LOG2E)).astype(BF16))

        def taps():
            for src, dst, nlg, centre in ((dwc_ref, dwc_s, NLG, 0.0), (dwm_ref, dwm_s, 2 * NLG, 1.0)):
                for lg in range(nlg):
                    wl = src[:, pl.ds(lg * 128, 128)].astype(F32)
                    w = [wl[i:i + 1] for i in range(K)]
                    if centre:
                        w[K // 2] = w[K // 2] + centre
                    wa, wb = w[1::2], w[0::2]
                    ws = [wa[i] + wb[i] if i < len(wa) else wb[i] for i in range(len(wb))]
                    for q, ww in enumerate((ws, wb, wa)):
                        for i, wi in enumerate(ww):
                            dst[lg, pl.ds(8 * (16 * q + i), 8), :] = jnp.broadcast_to(wi, (8, 128))

        def warm_p(k):
            never = z_s[...] != 0
            deps = [[] for _ in range(NTILE)]
            parts, outs = [], []
            for lg in range(NLG):
                sc = _ffa_chain(g_s[k], lg, 0, NH, dwc_s, None, None, None)
                ys = [_ffa_chain(g_s[k], lg, q, NH, dwc_s, None, None, sc)
                      * u_s[k, pl.ds((q - 1) * H, H), pl.ds(lg * 128, 128)] for q in (1, 2)]
                parts.append(_cat(ys, axis=0))
                outs += [sc] + ys
            for j, y in enumerate(outs):
                deps[PPV0 + (j * (NTILE - PPV0)) // len(outs)] = [y[8 * i:8 * i + 8] for i in range(NH)]
            stage_p(k, k, never, deps)
            c1_mm(k, k, parts)

        for tok in PLAN:
            op, arg = tok[0], tok[1:]
            if op == '!':
                dmas[arg].wait()
            elif op == 'W':
                src, dst = {'2': (wmi_ref, wmi_s), '3': (wmo_ref, wmo_s), '4': (wm_ref, wm_s)}[arg]
                dst[...] = _pk(src[...])
            elif op == 'D':
                taps()
            elif op == 'F':
                fold()
            elif op == 'L':
                ln_tile(int(arg) // nt1, int(arg) % nt1)
            elif op == 'V':
                v_tile(int(arg) // nt1, int(arg) % nt1)
            elif op == 'Q':
                qs[int(arg)] = q_proj(int(arg))
            elif op == 'A':
                stage_a2(int(arg), int(arg))
            elif op == 'C':
                ca, cb = arg.split('-')
                for k in range(3):
                    mxs[k] = q_chunks(k, k, qs[k], None, nodeps, mxs[k], int(ca), int(cb))
            else:
                warm_p(int(arg))

    @pl.when(step < NS - 1)
    def _():
        for i in range(UN):
            micro(step * UN + i, i)

    @pl.when(step == NS - 1)
    def _():
        for i in range(NKT - (NS - 1) * UN):
            micro((NS - 1) * UN + i, i)


@jax.jit
def pallas_standalone__conformer_family_e_branchformer__speech_kernel(
    x: jax.Array,
    w_qkv: jax.Array,
    w_att_out: jax.Array,
    w_mlp_in: jax.Array,
    dw_csgu: jax.Array,
    w_mlp_out: jax.Array,
    dw_merge: jax.Array,
    w_merge: jax.Array,
):
    B, T, D = x.shape
    K = dw_csgu.shape[0]
    assert (B, T, D, K) == (2, 4000, 256, 31), "schedule tables are written for this shape"
    TP = 4096
    NS = -(-(B * T // R) // UN)
    nlg = D // 128
    kern = functools.partial(_kernel, B=B, T=T, D=D, K=K, TP=TP)
    out = pl.pallas_call(
        kern,
        grid=(NS,),
        in_specs=[pl.BlockSpec(memory_space=pl.ANY)] * 8,
        out_specs=pl.BlockSpec((R * UN, D), lambda s: (s, 0)),
        out_shape=jax.ShapeDtypeStruct((B * T, D), x.dtype),
        scratch_shapes=[
            pltpu.VMEM(x.shape, BF16),
            pltpu.VMEM(w_qkv.shape, BF16),
            pltpu.VMEM(w_att_out.shape, BF16),
            pltpu.VMEM(w_mlp_in.shape, BF16),
            pltpu.VMEM(w_mlp_out.shape, BF16),
            pltpu.VMEM(w_merge.shape, BF16),
            pltpu.VMEM(dw_csgu.shape, BF16),
            pltpu.VMEM(dw_merge.shape, BF16),
            pltpu.SemaphoreType.DMA((8 + len(XG),)),
            pltpu.VMEM((D // 2, D), U32),
            pltpu.VMEM((D // 2, D), U32),
            pltpu.VMEM((D // 2, 2 * D), U32),
            pltpu.VMEM((D // 2, D), U32),
            pltpu.VMEM((D, D), U32),
            pltpu.VMEM((nlg, 384, 128), F32),
            pltpu.VMEM((2 * nlg, 384, 128), F32),
            pltpu.VMEM((B, TP // 2, D), U32),
            pltpu.VMEM((B, TP // 2, D), U32),
            pltpu.VMEM((U, R, D), F32),
            pltpu.VMEM((U, R, TP), F32),
            pltpu.VMEM((U, R, 128), F32),
            pltpu.VMEM((8, 128), jnp.int32),
        ] + [pltpu.VMEM((nlg, 7, RR, 128), F32)] * U + [pltpu.VMEM((2 * nlg, 7, RR, 128), F32)] * U,
        compiler_params=pltpu.CompilerParams(
            dimension_semantics=("arbitrary",),
            vmem_limit_bytes=100 * 1024 * 1024,
        ),
    )(x, w_qkv, w_att_out, w_mlp_in, dw_csgu, w_mlp_out, dw_merge, w_merge)
    return out.reshape(B, T, D)
```

```python
import functools
import math

import jax
import jax.numpy as jnp
from jax import lax
import jax.experimental.pallas as pl
import jax.experimental.pallas.tpu as pltpu

F32 = jnp.float32
BF16 = jnp.bfloat16
U32 = jnp.uint32
EPS = 1e-5
LOG2E = 1.4426950408889634

R = 80
UN = 12
U = 6
TA = 400
CK = 256
CP = 512
RR = 72

GT = 13

PV0, NPVF, QK0, WIN = 42, 23, 4, 5
UA0, UA1, HA0, AW, AD = 12, 54, 38, 28, 8
THR, THRL, THRP, PPV0 = 3, 3, 2, 36

XG = [(0, 0, 2), (0, 2, 4), (0, 4, 6), (0, 6, 10), (1, 0, 5), (1, 5, 10)]
DORD = 'x0 w5 w6 w7 w1 w0 x1 w2 x2 x3 w3 w4 x4 x5'.split()
PLAN = ('!x0 L0 L1 '
        '!w5 !w6 !w7 !w0 !w1 D F V0 V1 G0 Q0 Q1 Q2 C0-3 '
        '!x1 !w2 !x2 W2 T00 Z3 L2 A0 A1 L3 A2 A3 L4 L5 V2 V3 V4 '
        '!x3 T01 T02 T03 L6 V5+ C3-5 L7 C5-7 L8 L9 V6+3 V7 V8 C7-9 '
        '!w3 !w4 !x4 W3 W4 V9+ L10 C9-12 L11 V10+ X0 C12-14 L12 C14-16 L13 L14 G1 V11 V12 V13 '
        '!x5 T10 T11 T12 T13 V14+ L15 P0 L16 V15+ L17 L18 V16 L19 V17+ V18+ Z X1 P1 V19').split()


def _gelu(x):
    c = math.sqrt(2.0 / math.pi)
    return 0.5 * x * (1.0 + jnp.tanh(c * (x + 0.044715 * (x * x * x))))


def _dot(a, b):
    return jnp.dot(a, b, preferred_element_type=F32)


def _dot_nt(a, b):
    return lax.dot_general(a, b, (((1,), (1,)), ((), ())), preferred_element_type=F32)


def _cat(parts, axis=-1):
    return jnp.concatenate(parts, axis=axis)


def _pk(x):
    return pltpu.bitcast(x, U32)


def _upk(x):
    return pltpu.bitcast(x, BF16)


def _even_odd(xb):
    xu = _pk(xb)
    return pltpu.bitcast(xu << 16, F32), pltpu.bitcast(xu & jnp.uint32(0xFFFF0000), F32)


def _interleave_bf16(e, o):
    rb = lambda a: pltpu.bitcast(a.astype(BF16).astype(F32), U32)
    return _upk((rb(e) >> 16) | (rb(o) & jnp.uint32(0xFFFF0000)))


def _vregs(a):
    return [a[8 * r:8 * r + 8, l * 128:(l + 1) * 128]
            for r in range(a.shape[0] // 8) for l in range(a.shape[1] // 128)]


def _bc(a):
    return jnp.broadcast_to(a, (a.shape[0], 128))


def _anchored(t, never, deps):
    if not deps:
        return t
    pieces = [t[8 * j:8 * j + 8] for j in range(8)]
    for j, d in enumerate(deps):
        pieces[7 - j] = jnp.where(never, pltpu.bitcast(d, U32), pieces[7 - j])
    return _cat(pieces, axis=0)


def _ffa_chain(ring, lg, q, nj, w_ref, never, rel, init):
    nt = (16, 16, 15)[q]
    acc = init
    ks = [k for pair in zip(range(8), range(8, 16)) for k in pair if k < nt]
    for n_, k in enumerate(ks):
        win = ring[lg, 2 * q, pl.ds(k + 1, 8 * nj), :]
        w = w_ref[lg, pl.ds(8 * (16 * q + k), 8), :]
        if n_ == 0 and rel is not None:
            w = jnp.where(never, rel, w)
        w = _cat([w] * nj, axis=0)
        acc = win * w if acc is None else acc + win * w
    return acc


def _kernel(x_hbm, wqkv_hbm, wao_hbm, wmi_hbm, dwc_hbm, wmo_hbm, dwm_hbm, wm_hbm, o_ref,
            x_ref, wqkv_ref, wao_ref, wmi_ref, wmo_ref, wm_ref, dwc_ref, dwm_ref, sems,
            wqk_s, wvo_s, wmi_s, wmo_s, wm_s, dwc_s, dwm_s, xa_s, v_s, u_s, s_s, mx_s, z_s, st_s, *rings,
            B, T, D, K, TP):
    g_s, m_s = rings[:U], rings[U:]
    step = pl.program_id(0)
    NK = T // R
    NKT = B * NK
    NS = -(-NKT // UN)
    NLG = D // 128
    NC = TP // CK
    H = R // 2
    NH = H // 8
    NTILE = (TP // 128) * NLG
    TM = (T // 128) * 128
    TK = T - TM

    def split(k):
        if isinstance(k, int):
            return k // NK, k % NK
        b = sum((k >= j * NK).astype(jnp.int32) for j in range(1, B))
        return b, k - b * NK

    def rows(i, n):
        r = i * n
        return pl.ds(r if isinstance(r, int) else pl.multiple_of(r, 8), n)

    def seq_put(ref, q, lg, r0, val):
        ref[lg, 2 * q, pl.ds(r0, val.shape[0]), :] = val

    def halo_store(ref, k, kmod, lg, val):
        cur, prv, nxt = ref[kmod % U], ref[(kmod - 1) % U], ref[(kmod + 1) % U]
        xe, xo = val[:H], val[H:]
        row0 = lax.broadcasted_iota(jnp.int32, (8, 128), 0) == 0
        rot = [pltpu.roll(xo[8 * i:8 * i + 8], 1, 0) for i in range(NH)]
        nxt[lg, 6, pl.ds(0, 8), :] = rot[-1]
        rot = [cur[lg, 6, pl.ds(0, 8), :]] + rot
        sh = _cat([jnp.where(row0, rot[i], rot[i + 1]) for i in range(NH)], axis=0)
        zero = jnp.zeros((8, 128), F32)
        if isinstance(k, int):
            first, last = k % NK == 0, k % NK == NK - 1
        else:
            first = (split(k)[1] == 0) if any((j * NK) % UN == kmod for j in range(B)) else False
            last = (split(k)[1] == NK - 1) if any((j * NK - 1) % UN == kmod for j in range(1, B + 1)) else False
        sh0 = sh[:8]
        if first is not False:
            cut = row0 if first is True else jnp.logical_and(row0, first)
            sh = _cat([jnp.where(cut, 0.0, sh0), sh[8:]], axis=0)
        seqs = [xe, sh - xe, xo - xe]
        for q, v in enumerate(seqs):
            seq_put(cur, q, lg, 8, v)
            top, bot = v[:8], v[H - 8:]
            if first is not False:
                edge = jnp.where(row0, sh0, 0.0) if q == 1 else zero
                top = None if (first is True and k == 0) else (edge if first is True else jnp.where(first, edge, top))
            if last is not False:
                bot = zero if last is True else jnp.where(last, 0.0, bot)
            if top is not None:
                seq_put(prv, q, lg, 8 + H, top)
            seq_put(nxt, q, lg, 0, bot)

    def tail_store(ref, nlg):
        row0 = lax.broadcasted_iota(jnp.int32, (8, 128), 0) == 0
        for lg in range(nlg):
            e = ref[NKT % U][lg, 6, pl.ds(0, 8), :]
            for q in range(3):
                seq_put(ref[(NKT - 1) % U], q, lg, 8 + H,
                        jnp.where(row0, e, 0.0) if q == 1 else jnp.zeros((8, 128), F32))

    def xa_rows(b, r):
        return _upk(xa_s[b, r, :])

    def ln_tile(b, t):
        eo = _even_odd(x_ref[b, pl.ds(t * TA, TA), :])
        x = _cat([eo[par][i * H:(i + 1) * H] for i in range(TA // R) for par in range(2)], axis=0)
        xc = x - jnp.mean(x, axis=-1, keepdims=True)
        ve = jnp.mean(xc * xc, axis=-1, keepdims=True) + EPS
        rs = jnp.exp2(jnp.log(ve) * (-0.5 * LOG2E))
        xa = xc * rs
        xa_s[b, rows(t, TA // 2), :] = _pk(xa.astype(BF16))

    def v_tile(b, t, extra=None):
        n = TA if extra is None else R
        for j in range(TA // n):
            w = wvo_s[...]
            r = pl.ds((t * TA + j * n) // 2, n // 2)
            vp = _pk(_dot(xa_rows(b, r), _upk(w)).astype(BF16))
            v_s[b, r, :] = vp
            if t == 0 and j == 0:
                for a in range(128 // TK):
                    v_s[b, pl.ds((T + a * TK) // 2, TK // 2), :] = vp[:TK // 2]
            if extra:
                extra.pop(0)()

    def stage_a2(k, kmod):
        b, i = split(k)
        h = _gelu(_dot(xa_rows(b, rows(i, R // 2)), _upk(wmi_s[...])))
        u_s[kmod % U] = h[:, :D]
        hg = h[:, D:]
        mu = jnp.mean(hg, axis=-1, keepdims=True)
        xc = hg - mu
        rs = lax.rsqrt(jnp.mean(xc * xc, axis=-1, keepdims=True) + EPS)
        g = xc * rs
        for lg in range(NLG):
            halo_store(g_s, k, kmod, lg, g[:, lg * 128:(lg + 1) * 128])
        return _vregs(h[:, :D]), _vregs(hg), _vregs(_bc(mu)), _vregs(_bc(rs)), _vregs(g)

    def c1_mm(k, kmod, parts):
        loc = _dot(_cat(parts).astype(BF16), _upk(wmo_s[...]))
        for lg in range(NLG):
            halo_store(m_s, k, kmod, NLG + lg, loc[:, lg * 128:(lg + 1) * 128])

    def c2_mm(k, pos, parts):
        b, i = split(k)
        r0 = i * R
        r0 = r0 if isinstance(r0, int) else pl.multiple_of(r0, 16)
        y = _dot(_cat(parts).astype(BF16), _upk(wm_s[...]))
        xe, xo = _even_odd(x_ref[b, pl.ds(r0, R), :])
        o_ref[pl.ds(pos * R, R), :] = _interleave_bf16(y[:H] + xe, y[H:] + xo)

    def q_proj(k):
        b, i = split(k)
        return _dot(xa_rows(b, rows(i, R // 2)), _upk(wqk_s[...])).astype(BF16)

    def k_chunk(b, c, never, deps):
        blks = []
        for kt in range(min(CK, TM - c * CK) // 128):
            blks.append(_cat([
                _anchored(xa_s[b, pl.ds((TK + c * CK) // 2 + kt * 64, 64), pl.ds(lg * 128, 128)], never,
                          deps[(c * (CK // 128) + kt) * NLG + lg])
                for lg in range(NLG)]))
        return _upk(_cat(blks, axis=0))

    def q_chunks(k, kmod, q, never, deps, mx, ca, cb, hook=None):
        b, _ = split(k)
        for c in range(ca, cb):
            s = _dot_nt(q, k_chunk(b, c, never, deps))
            if hook is not None:
                hook(NC + c, s)
            for l in range(CK // 128):
                c0 = c * CK + l * 128
                if c0 < TM:
                    sl = s[:, l * 128:(l + 1) * 128]
                else:
                    i = split(k)[1]
                    a = i // GT if isinstance(i, int) else sum((i >= j * GT).astype(jnp.int32) for j in range(1, 4))
                    grp = lax.broadcasted_iota(jnp.int32, (R, 128), 1) // TK
                    sl = jnp.where(grp == a, st_s[b, rows(i - a * GT, R), :], -jnp.inf)
                s_s[kmod % U, :, pl.ds(c0, 128)] = sl
                mx = sl if mx is None else jnp.maximum(mx, sl)
        if cb == NC:
            mx_s[kmod % U] = jnp.broadcast_to(jnp.max(mx, axis=-1, keepdims=True), (R, 128))
        return mx

    def v_chunk(b, c, lg, never, deps):
        return _upk(_cat([
            _anchored(v_s[b, pl.ds((TK + c * CP) // 2 + kt * 64, 64), pl.ds(lg * 128, 128)], never, deps[kt])
            for kt in range(CP // 128)], axis=0))

    def stage_p(k, kmod, never, deps, hook=None, thr=0):
        b, _ = split(k)
        m = mx_s[kmod % U]
        neverr = _cat([never] * (R // 8), axis=0)
        ncp = TP // CP
        tpc = CP // 128
        ls = None
        pbs, pvs, accs = [], [], []
        for lg in range(NLG):
            acc = None
            for c in range(ncp):
                gc = lg * ncp + c
                if lg == 0:
                    ps = []
                    if thr and c >= thr:
                        m = jnp.where(neverr, pvs[c - thr], m)
                    for l in range(tpc):
                        ps.append(jnp.exp2(s_s[kmod % U, :, pl.ds(c * CP + l * 128, 128)] - m))
                    for p in ps:
                        ls = p if ls is None else ls + p
                    pbs.append(_cat(ps).astype(BF16))
                pv = _dot(pbs[c], v_chunk(b, c, lg, never, deps[gc * tpc:(gc + 1) * tpc]))
                if hook is not None:
                    hook(gc, pv)
                pvs.append(pv)
                acc = pv if acc is None else acc + pv
            accs.append(acc)
        acc = _cat(accs)
        l = jnp.sum(ls, axis=-1, keepdims=True)
        glob = acc * (1.0 / l)
        for lg in range(NLG):
            halo_store(m_s, k, kmod, lg, glob[:, lg * 128:(lg + 1) * 128])

    def micro(n, pos):
        nmod = pos % U
        ok = lambda k: (not isinstance(k, int)) or 0 <= k < NKT
        never = z_s[...] != 0
        tpc = NTILE // NC
        hasp, hasq = ok(n + 2), ok(n + 3)
        lo = 0 if hasp else NTILE
        hi = 2 * NTILE if hasq else NTILE
        res = {}
        jobs = []
        if isinstance(n, int) and n + 4 == NKT:
            tail_store(g_s, NLG)
        if isinstance(n, int) and n + 2 == NKT:
            tail_store(m_s, 2 * NLG)

        def chain_jobs(name, ring, nlg, w_ref, fin):
            for lg in range(nlg):
                for q in range(3):
                    def fn(rel, lg=lg, q=q):
                        init = None if q == 0 else _cat(res[name, lg, 0], axis=0)
                        y = _ffa_chain(ring, lg, q, NH, w_ref, never, rel, init)
                        if q > 0:
                            y = fin(lg, q - 1, y)
                        return [y[8 * i:8 * i + 8] for i in range(NH)]
                    jobs.append(((name, lg, q), fn))

        chain_jobs('c2', m_s[nmod], 2 * NLG, dwm_s, lambda lg, par, y: y)
        if hasp:
            km = (nmod + 2) % U
            chain_jobs('c1', g_s[km], NLG, dwc_s,
                       lambda lg, par, y: y * u_s[km, pl.ds(par * H, H), pl.ds(lg * 128, 128)])

        def gather(name, nlg):
            return [_cat([v for q in (1, 2) for v in res[name, lg, q]], axis=0) for lg in range(nlg)]

        if hasp and hasq:
            npv = (NPVF * len(jobs)) // 100
        elif hasp:
            npv = len(jobs)
        else:
            npv = 0
        pv0 = PV0 if hasq else 0
        dls = [pv0 + (j * (NTILE - pv0)) // max(npv, 1) for j in range(npv)]
        nq = len(jobs) - npv
        dls += [NTILE + QK0 + (j * (NTILE - NLG - QK0)) // nq if hasq else None for j in range(nq)]
        slots = [[] for _ in range(2 * NTILE)]
        pending = {}

        def addslot(dl, vals):
            for v in vals:
                while len(slots[dl]) >= 8:
                    dl += 1
                slots[dl].append(v)

        for (key, fn), dl in zip(jobs, dls):
            rc = None if dl is None else dl // tpc - WIN
            if rc is None or rc < lo // tpc:
                res[key] = fn(None)
                if dl is not None:
                    addslot(dl, res[key])
            else:
                pending.setdefault(rc, []).append((key, fn, dl))

        def hook(gc, val):
            for j, (key, fn, dl) in enumerate(pending.pop(gc, [])):
                res[key] = fn(val[8 * j:8 * j + 8, :128])
                addslot(dl, res[key])

        def put(items, a, b):
            a, b = max(a, lo), min(b, hi)
            for j, it in enumerate(items):
                addslot(a + (j * (b - a)) // len(items), [it])

        if hasq:
            q = q_proj(n + 3)
        if ok(n + 4):
            uu, hh, mu, rs, gg = stage_a2(n + 4, (pos + 4) % UN)
            put(uu, UA0, UA1)
            put(hh, HA0, HA0 + AW)
            put(mu, HA0 + AD, HA0 + AD + AW)
            put(rs, HA0 + 2 * AD, HA0 + 2 * AD + AW)
            put(gg, HA0 + 2 * AD + 4, HA0 + 2 * AD + 4 + AW)
        if hasp:
            stage_p(n + 2, (pos + 2) % UN, never, slots[:NTILE], hook,
                    THRL if not hasq else (THR if pos == UN - 1 else 0))
        if hasq:
            q_chunks(n + 3, (pos + 3) % UN, q, never, slots[NTILE:], None, 0, NC, hook)
        assert not pending
        if hasp:
            c1_mm(n + 2, (pos + 2) % UN, gather('c1', NLG))
        c2_mm(n, pos, gather('c2', 2 * NLG))

    @pl.when(step == 0)
    def _():
        nt1 = T // TA
        cw = [pltpu.make_async_copy(src, dst, sems.at[j]) for j, (src, dst) in enumerate(
            [(wqkv_hbm.at[:, pl.ds(0, 2 * D)], wqkv_ref.at[:, pl.ds(0, 2 * D)]), (wao_hbm, wao_ref),
             (wmi_hbm, wmi_ref), (wmo_hbm, wmo_ref), (wm_hbm, wm_ref),
             (dwc_hbm, dwc_ref), (dwm_hbm, dwm_ref),
             (wqkv_hbm.at[:, pl.ds(2 * D, D)], wqkv_ref.at[:, pl.ds(2 * D, D)])])]
        cx = [pltpu.make_async_copy(x_hbm.at[b, pl.ds(t0 * TA, (t1 - t0) * TA), :],
                                    x_ref.at[b, pl.ds(t0 * TA, (t1 - t0) * TA), :], sems.at[8 + j])
              for j, (b, t0, t1) in enumerate(XG)]
        dmas = {'w%d' % j: c for j, c in enumerate(cw)}
        dmas.update({'x%d' % j: c for j, c in enumerate(cx)})
        for name in DORD:
            dmas[name].start()
        z_s[...] = jnp.zeros(z_s.shape, z_s.dtype)
        for b in range(B):
            xa_s[b, pl.ds(T // 2, (TP - T) // 2), :] = jnp.zeros(((TP - T) // 2, D), U32)
        for ring, nlg in ((g_s, NLG), (m_s, 2 * NLG)):
            for lg in range(nlg):
                for q in range(3):
                    seq_put(ring[0], q, lg, 0, jnp.zeros((8, 128), F32))
                ring[0][lg, 6, pl.ds(0, 8), :] = jnp.zeros((8, 128), F32)
        nodeps = [[] for _ in range(NTILE)]
        qs, mxs = {}, {0: None, 1: None, 2: None}

        def fold():
            wvo_s[...] = _pk(_dot(wqkv_ref[:, 2 * D:3 * D], wao_ref[...]).astype(BF16))
            wqk_s[...] = _pk((_dot_nt(wqkv_ref[:, 0:D], wqkv_ref[:, D:2 * D])
                              * (D ** -0.5 * LOG2E)).astype(BF16))

        def taps():
            for src, dst, nlg, centre in ((dwc_ref, dwc_s, NLG, 0.0), (dwm_ref, dwm_s, 2 * NLG, 1.0)):
                for lg in range(nlg):
                    wl = src[:, pl.ds(lg * 128, 128)].astype(F32)
                    w = [wl[i:i + 1] for i in range(K)]
                    if centre:
                        w[K // 2] = w[K // 2] + centre
                    wa, wb = w[1::2], w[0::2]
                    ws = [wa[i] + wb[i] if i < len(wa) else wb[i] for i in range(len(wb))]
                    for q, ww in enumerate((ws, wb, wa)):
                        for i, wi in enumerate(ww):
                            dst[lg, pl.ds(8 * (16 * q + i), 8), :] = jnp.broadcast_to(wi, (8, 128))

        gts, sts = {}, {}

        def tail_g(b):
            gts[b] = _dot_nt(xa_rows(b, pl.ds(0, TK // 2)), _upk(wqk_s[...])).astype(BF16)

        def tail_units(b, a):
            nb = -(-min(GT * R, T - a * GT * R) // 128)
            jobs = []
            for i in range(0, nb, 2):
                def job(i=i, n=min(2, nb - i)):
                    st = _dot_nt(gts[b], xa_rows(b, pl.ds(a * GT * R // 2 + i * 64, n * 64)))
                    for j in range(n):
                        sts[b, a, i + j] = st[:, j * 128:(j + 1) * 128]
                jobs.append(job)
            return jobs

        def tail_transpose(b):
            for i in range(9):
                blk = [sts.get((b, a, i), jnp.zeros((TK, 128), F32)) for a in range(4)]
                st_s[b, pl.ds(i * 128, 128), :] = _cat(blk, axis=0).T

        def warm_p(k):
            never = z_s[...] != 0
            deps = [[] for _ in range(NTILE)]
            parts, outs = [], []
            for lg in range(NLG):
                sc = _ffa_chain(g_s[k], lg, 0, NH, dwc_s, None, None, None)
                ys = [_ffa_chain(g_s[k], lg, q, NH, dwc_s, None, None, sc)
                      * u_s[k, pl.ds((q - 1) * H, H), pl.ds(lg * 128, 128)] for q in (1, 2)]
                parts.append(_cat(ys, axis=0))
                outs += [sc] + ys
            for j, y in enumerate(outs):
                deps[PPV0 + (j * (NTILE - PPV0)) // len(outs)] = [y[8 * i:8 * i + 8] for i in range(NH)]
            stage_p(k, k, never, deps, None, THRP)
            c1_mm(k, k, parts)

        queue = []
        for tok in PLAN:
            op, arg = tok[0], tok[1:]
            if op == '!':
                dmas[arg].wait()
            elif op == 'W':
                src, dst = {'2': (wmi_ref, wmi_s), '3': (wmo_ref, wmo_s), '4': (wm_ref, wm_s)}[arg]
                dst[...] = _pk(src[...])
            elif op == 'D':
                taps()
            elif op == 'F':
                fold()
            elif op == 'L':
                ln_tile(int(arg) // nt1, int(arg) % nt1)
            elif op == 'V':
                t, plus, cnt = arg.partition('+')
                extra = [queue.pop(0) for _ in range(min(len(queue), int(cnt or TA // R)))] if plus else None
                v_tile(int(t) // nt1, int(t) % nt1, extra)
            elif op == 'Q':
                qs[int(arg)] = q_proj(int(arg))
            elif op == 'A':
                stage_a2(int(arg), int(arg))
            elif op == 'C':
                ca, cb = arg.split('-')
                for k in range(3):
                    mxs[k] = q_chunks(k, k, qs[k], None, nodeps, mxs[k], int(ca), int(cb))
            elif op == 'G':
                tail_g(int(arg))
            elif op == 'T':
                queue += tail_units(int(arg[0]), int(arg[1]))
            elif op == 'Z':
                for _ in range(int(arg) if arg else len(queue)):
                    queue.pop(0)()
            elif op == 'X':
                assert not queue
                tail_transpose(int(arg))
            else:
                warm_p(int(arg))

    @pl.when(step < NS - 1)
    def _():
        for i in range(UN):
            micro(step * UN + i, i)

    @pl.when(step == NS - 1)
    def _():
        for i in range(NKT - (NS - 1) * UN):
            micro((NS - 1) * UN + i, i)


@jax.jit
def pallas_standalone__conformer_family_e_branchformer__speech_kernel(
    x: jax.Array,
    w_qkv: jax.Array,
    w_att_out: jax.Array,
    w_mlp_in: jax.Array,
    dw_csgu: jax.Array,
    w_mlp_out: jax.Array,
    dw_merge: jax.Array,
    w_merge: jax.Array,
):
    B, T, D = x.shape
    K = dw_csgu.shape[0]
    assert (B, T, D, K) == (2, 4000, 256, 31), "schedule tables are written for this shape"
    TP = 4096
    NS = -(-(B * T // R) // UN)
    nlg = D // 128
    kern = functools.partial(_kernel, B=B, T=T, D=D, K=K, TP=TP)
    out = pl.pallas_call(
        kern,
        grid=(NS,),
        in_specs=[pl.BlockSpec(memory_space=pl.ANY)] * 8,
        out_specs=pl.BlockSpec((R * UN, D), lambda s: (s, 0)),
        out_shape=jax.ShapeDtypeStruct((B * T, D), x.dtype),
        scratch_shapes=[
            pltpu.VMEM(x.shape, BF16),
            pltpu.VMEM(w_qkv.shape, BF16),
            pltpu.VMEM(w_att_out.shape, BF16),
            pltpu.VMEM(w_mlp_in.shape, BF16),
            pltpu.VMEM(w_mlp_out.shape, BF16),
            pltpu.VMEM(w_merge.shape, BF16),
            pltpu.VMEM(dw_csgu.shape, BF16),
            pltpu.VMEM(dw_merge.shape, BF16),
            pltpu.SemaphoreType.DMA((8 + len(XG),)),
            pltpu.VMEM((D // 2, D), U32),
            pltpu.VMEM((D // 2, D), U32),
            pltpu.VMEM((D // 2, 2 * D), U32),
            pltpu.VMEM((D // 2, D), U32),
            pltpu.VMEM((D, D), U32),
            pltpu.VMEM((nlg, 384, 128), F32),
            pltpu.VMEM((2 * nlg, 384, 128), F32),
            pltpu.VMEM((B, TP // 2, D), U32),
            pltpu.VMEM((B, TP // 2 + 32, D), U32),
            pltpu.VMEM((U, R, D), F32),
            pltpu.VMEM((U, R, TP), F32),
            pltpu.VMEM((U, R, 128), F32),
            pltpu.VMEM((8, 128), jnp.int32),
            pltpu.VMEM((B, 9 * 128, 128), F32),
        ] + [pltpu.VMEM((nlg, 7, RR, 128), F32)] * U + [pltpu.VMEM((2 * nlg, 7, RR, 128), F32)] * U,
        compiler_params=pltpu.CompilerParams(
            dimension_semantics=("arbitrary",),
            vmem_limit_bytes=100 * 1024 * 1024,
        ),
    )(x, w_qkv, w_att_out, w_mlp_in, dw_csgu, w_mlp_out, dw_merge, w_merge)
    return out.reshape(B, T, D)
```
